```python
import jax
import jax.numpy as jnp

def _softmax(x, axis=-1):
    return jax.nn.softmax(x, axis=axis)

def _gelu(x):
    return jax.nn.gelu(x, approximate=True)

def _silu(x):
    return jax.nn.silu(x)

def _sigmoid(x):
    return jax.nn.sigmoid(x)

def _layernorm(x, axis=-1, eps=1e-05):
    m = jnp.mean(x, axis=axis, keepdims=True)
    v = jnp.var(x, axis=axis, keepdims=True)
    return (x - m) / jnp.sqrt(v + eps)

def _scatter_add(tgt, idx, src, axis=0):
    return tgt.at[idx].add(src)

def _segment_sum(src, seg, n):
    return jax.ops.segment_sum(src, seg, n)

class _Rng:

    def __init__(self, key):
        self._k = key

    def _next(self):
        self._k, sub = jax.random.split(self._k)
        return sub

    def normal(self, shape):
        return jax.random.normal(self._next(), shape, dtype=jnp.bfloat16)

    def randint(self, lo, hi, shape):
        return jax.random.randint(self._next(), shape, lo, hi, dtype=jnp.int32)

    def uniform(self, shape, lo=0.0, hi=1.0):
        return jax.random.uniform(self._next(), shape, jnp.bfloat16, lo, hi)

    def permutation(self, n):
        return jax.random.permutation(self._next(), n)
kernel_name = 'adaLN_cond__linear_kernel_hedgehog__moe_arch_mod__prompt'

def setup_inputs():
    _rng = _Rng(jax.random.key(int.from_bytes(__import__("os").urandom(4), "little")))
    _w = lambda a: (lambda t: t.astype(jnp.bfloat16) if jnp.issubdtype(t.dtype, jnp.floating) else t)(jnp.asarray(a))

    def _A_setup():
        B, S, D, H = (1, 2048, 1024, 32)
        Dh = D // H
        return {'x': _w((lambda *s: _rng.normal(s) * 0.05)(B, S, D)), 'wqkv': _w((lambda *s: _rng.normal(s) * 0.05)(D, 3 * D)), 'w_phi': _w((lambda *s: _rng.normal(s) * 0.05)(H, Dh, Dh) * Dh ** (-0.5)), 'wo': _w((lambda *s: _rng.normal(s) * 0.05)(D, D))}
    _A_in = _A_setup()

    def _B_setup():
        B, S, D, F, C = (1, 2048, 1024, 3584, 2)
        return {'x': _w((lambda *s: _rng.normal(s) * 0.05)(B, S, D)), 'w_r': _w((lambda *s: _rng.normal(s) * 0.05)(D)), 'w_gate': _w((lambda *s: _rng.normal(s) * 0.05)(D, F)), 'w_up': _w((lambda *s: _rng.normal(s) * 0.05)(D, F)), 'w_down': _w((lambda *s: _rng.normal(s) * 0.05)(F, D))}
    _B_in = _B_setup()
    return {'A_x': _A_in['x'], 'A_wqkv': _A_in['wqkv'], 'A_w_phi': _A_in['w_phi'], 'A_wo': _A_in['wo'], 'B_x': _B_in['x'], 'B_w_r': _B_in['w_r'], 'B_w_gate': _B_in['w_gate'], 'B_w_up': _B_in['w_up'], 'B_w_down': _B_in['w_down'], 'c': _w((lambda *s: _rng.normal(s) * 0.05)(1, 1024)), 'w_mod': _w((lambda *s: _rng.normal(s) * 0.05)(1024, 6 * 1024) * 1024 ** (-0.5))}

def reference(A_x, A_wqkv, A_w_phi, A_wo, B_x, B_w_r, B_w_gate, B_w_up, B_w_down, c, w_mod):

    def _A_ref(x, wqkv, w_phi, wo):
        B, S, D = x.shape
        H = 32
        Dh = D // H
        qkv = (lambda x, *d: x.transpose(*d))((x @ wqkv).reshape(B, S, 3, H, Dh), 2, 0, 3, 1, 4)
        q, k, v = (qkv[0], qkv[1], qkv[2])
        pq = jnp.einsum('bhsd,hdf->bhsf', q, w_phi)
        pk = jnp.einsum('bhsd,hdf->bhsf', k, w_phi)
        phi_q = jnp.concatenate([_softmax(pq, axis=-1), _softmax(-pq, axis=-1)], axis=-1)
        phi_k = jnp.concatenate([_softmax(pk, axis=-1), _softmax(-pk, axis=-1)], axis=-1)
        kv = jnp.einsum('bhsf,bhsd->bhfd', phi_k, v)
        z = jnp.einsum('bhsf->bhf', phi_k)
        num = jnp.einsum('bhqf,bhfd->bhqd', phi_q, kv)
        den = jnp.einsum('bhqf,bhf->bhq', phi_q, z)[..., None] + 1e-06
        o = num / den
        return (lambda x, *d: x.transpose(*d))(o, 0, 2, 1, 3).reshape(B, S, D) @ wo

    def _B_ref(x, w_r, w_gate, w_up, w_down):
        B, S, D = x.shape
        C = 2
        r = x @ w_r
        idx = jnp.argsort(-r, axis=-1)[:, :C]
        idx_e = jnp.repeat(idx.reshape(B, C, 1), D, axis=2)
        x_sel = jnp.take_along_axis(x, idx_e, axis=1)
        g = _silu(x_sel @ w_gate)
        u = x_sel @ w_up
        y = g * u @ w_down
        r_sel = _sigmoid(jnp.take_along_axis(r, idx, axis=1))
        y = y * r_sel.reshape(B, C, 1)
        b_off = (jnp.arange(B) * S).reshape(B, 1)
        flat_idx = (idx + b_off).reshape(B * C)
        zero = (x * 0.0).reshape(B * S, D)
        upd = _scatter_add(zero, flat_idx, y.reshape(B * C, D), axis=0)
        return x + upd.reshape(B, S, D)
    x = A_x
    mod = (_silu(c) @ w_mod).reshape(c.shape[0], 6, 1, -1)
    sa, ca, ga, sb, cb, gb = (mod[:, 0].copy(), mod[:, 1].copy(), mod[:, 2].copy(), mod[:, 3].copy(), mod[:, 4].copy(), mod[:, 5].copy())
    h = _layernorm(x, axis=-1) * (1 + ca) + sa
    x = x + ga * _A_ref(h, A_wqkv, A_w_phi, A_wo)
    h = _layernorm(x, axis=-1) * (1 + cb) + sb
    x = x + gb * _B_ref(h, B_w_r, B_w_gate, B_w_up, B_w_down)
    return x
```

```python
import functools

import jax
import jax.numpy as jnp
from jax import lax
from jax.experimental import pallas as pl
from jax.experimental.pallas import tpu as pltpu

S, D, H, DH, F = 2048, 1024, 32, 32, 3584
LOG2E = 1.4426950408889634
NN = (((1,), (0,)), ((), ()))
NT = (((1,), (1,)), ((), ()))
TN = (((0,), (0,)), ((), ()))
BF = jnp.bfloat16
F32 = jnp.float32


def _dot(a, b, dims):
    return lax.dot_general(a, b, dims, preferred_element_type=F32)


def _layernorm(x):
    m = jnp.mean(x, axis=-1, keepdims=True)
    xc = x - m
    v = jnp.mean(xc * xc, axis=-1, keepdims=True)
    return xc * lax.rsqrt(v + 1e-5)


def _pair_reduce(x, op):
    r = x[0:8]
    for i in range(1, 8):
        r = op(r, x[8 * i:8 * i + 8])
    r = op(r, pltpu.roll(r, 4, 0))
    return op(r, pltpu.roll(r, 2, 0))


def _tile8(r, n):
    return jnp.concatenate([r] * n, axis=0)


def _hedgehog(p):
    mx = _tile8(_pair_reduce(p, jnp.maximum), 8)
    mn = _tile8(_pair_reduce(p, jnp.minimum), 8)
    ep = jnp.exp2(p - mx)
    en = jnp.exp2(mn - p)
    rp = _tile8(1.0 / _pair_reduce(ep, jnp.add), 8)
    rn = _tile8(1.0 / _pair_reduce(en, jnp.add), 8)
    return ep * rp, en * rn


def _kernel(x_hbm, wqkv_hbm, wphi_hbm, wo_hbm, wr_hbm, wg_hbm, wu_hbm, wd_hbm, c_hbm, wmod_hbm,
            out_hbm,
            x_v, wqkv_v, wphi_v, wo_v, wr_v, wg_v, wu_v, wd_v, c_v, wmod_v,
            wqT, wkT, wvT, h_v, x1_v, out_v, kv_acc, z_acc, kvT, zb, mod_v, top_v, slab_v,
            sems, osems, *, T, CH):
    NTILE = S // T
    NPAIR = H // 2

    def cp(src, dst, i):
        return pltpu.make_async_copy(src, dst, sems.at[i])

    def col(ref, j, w=D):
        return ref.at[:, pl.ds(j * w, w)]

    copies = {}
    order = [("c", c_hbm, c_v), ("wphi", wphi_hbm, wphi_v), ("wr", wr_hbm, wr_v),
             ("sa", col(wmod_hbm, 0), wmod_v.at[0]), ("ca", col(wmod_hbm, 1), wmod_v.at[1]),
             ("x0", x_hbm.at[pl.ds(0, T)], x_v.at[pl.ds(0, T)]),
             ("wk", col(wqkv_hbm, 1), wqkv_v.at[1]), ("wv", col(wqkv_hbm, 2), wqkv_v.at[2]),
             ("xr", x_hbm.at[pl.ds(T, S - T)], x_v.at[pl.ds(T, S - T)]),
             ("wq", col(wqkv_hbm, 0), wqkv_v.at[0]),
             ("ga", col(wmod_hbm, 2), wmod_v.at[2]), ("sb", col(wmod_hbm, 3), wmod_v.at[3]),
             ("cb", col(wmod_hbm, 4), wmod_v.at[4]), ("gb", col(wmod_hbm, 5), wmod_v.at[5]),
             ("wo", wo_hbm, wo_v), ("wg", wg_hbm, wg_v), ("wu", wu_hbm, wu_v), ("wd", wd_hbm, wd_v)]
    for i, (name, src, dst) in enumerate(order):
        copies[name] = cp(src, dst, i)
        copies[name].start()

    copies["c"].wait()
    copies["wphi"].wait()
    copies["wr"].wait()
    cf = c_v[...].astype(F32)
    sc = jnp.broadcast_to(cf * jax.nn.sigmoid(cf), (16, D)).astype(BF)

    row = lax.broadcasted_iota(jnp.int32, (128, DH), 0)
    lane = lax.broadcasted_iota(jnp.int32, (128, DH), 1)
    expand = jnp.where(((row % 64) // 2) == lane, 1.0, 0.0).astype(BF)
    bdt = _dot(expand, wphi_v[...].reshape(H * DH, DH), NT)
    row = lax.broadcasted_iota(jnp.int32, (128, D), 0)
    lane = lax.broadcasted_iota(jnp.int32, (128, D), 1)
    bdt = jnp.where(2 * (row // 64) + (row % 2) == (lane % 128) // DH, bdt, 0.0).astype(BF)

    def mod_row(j):
        return _dot(sc, wmod_v[j], NN)[0:8]

    copies["sa"].wait()
    mod_v[0] = mod_row(0)
    copies["ca"].wait()
    mod_v[1] = 1.0 + mod_row(1)

    def ln1(t):
        rows = pl.ds(pl.multiple_of(t * T, T), T)
        xn = _layernorm(x_v[rows, :].astype(F32))
        h_v[rows, :] = (xn * mod_v[1, 0:1, :] + mod_v[0, 0:1, :]).astype(BF)

    copies["x0"].wait()
    ln1(0)

    def fold(j, dst):
        for g in range(D // 128):
            w = wqkv_v[j, :, g * 128:(g + 1) * 128]
            dst[g * 128:(g + 1) * 128, :] = (_dot(bdt[:, g * 128:(g + 1) * 128], w, NT) * LOG2E).astype(BF)

    copies["wk"].wait()
    fold(1, wkT)
    copies["wv"].wait()
    for g in range(D // 128):
        wvT[g * 128:(g + 1) * 128, :] = wqkv_v[2, :, g * 128:(g + 1) * 128].T
    copies["xr"].wait()

    kv_acc[...] = jnp.zeros_like(kv_acc)
    z_acc[...] = jnp.zeros_like(z_acc)

    def phase1(t, carry):
        rows = pl.ds(pl.multiple_of(t * T, T), T)
        h = h_v[rows, :]
        for c in range(D // CH):
            pk = _dot(wkT[c * CH:(c + 1) * CH, :], h, NT)
            vt = _dot(wvT[c * CH:(c + 1) * CH, :], h, NT).astype(BF)
            for q in range(CH // 64):
                pair = c * (CH // 64) + q
                fp, fn = _hedgehog(pk[q * 64:(q + 1) * 64])
                phi = jnp.concatenate([fp, fn], axis=0)
                zs = phi[:, 0:128]
                for l in range(1, T // 128):
                    zs = zs + phi[:, l * 128:(l + 1) * 128]
                z_acc[pair] += zs
                kv_acc[pair] += _dot(vt[q * 64:(q + 1) * 64], phi.astype(BF), NT)
        ln1(jnp.minimum(t + 1, NTILE - 1))
        return carry

    lax.fori_loop(0, NTILE, phase1, 0)

    copies["wq"].wait()
    fold(0, wqT)
    for j, name in ((2, "ga"), (3, "sb"), (4, "cb"), (5, "gb")):
        copies[name].wait()
        mod_v[j] = mod_row(j) + (1.0 if name == "cb" else 0.0)
    row = lax.broadcasted_iota(jnp.int32, (64, 128), 0)
    lane = lax.broadcasted_iota(jnp.int32, (64, 128), 1)
    same_head = (row // DH) == (lane % 2)
    for pair in range(NPAIR):
        kvT[pair] = jnp.where(same_head, kv_acc[pair], 0.0).astype(BF)
        zb[pair] = jnp.broadcast_to(jnp.sum(z_acc[pair], axis=-1, keepdims=True), (128, 128))
    copies["wo"].wait()

    wr = wr_v[...].astype(F32)
    wr_row = jnp.concatenate([wr[j:j + 1, :] for j in range(8)], axis=1)

    def ln2(x1):
        h2 = _layernorm(x1) * mod_v[4, 0:1, :] + mod_v[3, 0:1, :]
        return h2, x1 + mod_v[5, 0:1, :] * h2

    neg = jnp.full((8, 128), -jnp.inf, F32)
    top_v[0] = neg
    top_v[1] = neg
    top_v[2] = jnp.zeros((8, 128), F32)
    top_v[3] = jnp.zeros((8, 128), F32)

    def out_copy(t):
        rows = pl.ds(pl.multiple_of(t * T, T), T)
        return pltpu.make_async_copy(out_v.at[rows], out_hbm.at[rows], osems.at[t])

    def phase2(t, carry):
        rows = pl.ds(pl.multiple_of(t * T, T), T)
        h = h_v[rows, :]
        even = (lax.broadcasted_iota(jnp.int32, (8, T), 0) % 2) == 0
        ots = []
        for c in range(D // CH):
            pq = _dot(wqT[c * CH:(c + 1) * CH, :], h, NT)
            for q in range(CH // 64):
                pair = c * (CH // 64) + q
                fp, fn = _hedgehog(pq[q * 64:(q + 1) * 64])
                phi = jnp.concatenate([fp, fn], axis=0)
                num = _dot(kvT[pair], phi.astype(BF), NN)
                w = phi * jnp.concatenate([zb[pair]] * (T // 128), axis=1)
                den = _pair_reduce(w[0:64] + w[64:128], jnp.add) + 1e-6
                inv = 1.0 / den
                swapped = pltpu.roll(inv, 1, 0)
                inv_a = jnp.where(even, inv, swapped)
                inv_b = jnp.where(even, swapped, inv)
                scale = jnp.concatenate([inv_a] * 4 + [inv_b] * 4, axis=0)
                ots.append((num * scale).astype(BF))
        ot = jnp.concatenate(ots, axis=0)
        attn = _dot(ot, wo_v[...], TN)
        x1 = x_v[rows, :].astype(F32) + mod_v[2, 0:1, :] * attn
        x1_v[rows, :] = x1
        h2, out = ln2(x1)
        out_v[rows, :] = out.astype(BF)
        out_copy(t).start()
        r = jnp.sum(h2 * wr_row, axis=-1, keepdims=True)
        m1, m2, i1, i2 = top_v[0], top_v[1], top_v[2], top_v[3]
        base = (t * T).astype(F32) + lax.broadcasted_iota(jnp.int32, (8, 128), 0).astype(F32)
        for g in range(T // 8):
            rg = jnp.broadcast_to(r[g * 8:(g + 1) * 8], (8, 128))
            ig = base + float(g * 8)
            gt1 = rg > m1
            gt2 = rg > m2
            m2 = jnp.where(gt1, m1, jnp.where(gt2, rg, m2))
            i2 = jnp.where(gt1, i1, jnp.where(gt2, ig, i2))
            m1 = jnp.where(gt1, rg, m1)
            i1 = jnp.where(gt1, ig, i1)
        top_v[0], top_v[1], top_v[2], top_v[3] = m1, m2, i1, i2
        return carry

    lax.fori_loop(0, NTILE, phase2, 0)

    m1, m2, i1, i2 = top_v[0], top_v[1], top_v[2], top_v[3]
    big = float(2 * S)
    best = jnp.max(m1, axis=0, keepdims=True)
    ia = jnp.min(jnp.where(m1 == best, i1, big), axis=0, keepdims=True)
    taken = i1 == ia
    cm = jnp.where(taken, m2, m1)
    ci = jnp.where(taken, i2, i1)
    second = jnp.max(cm, axis=0, keepdims=True)
    ib = jnp.min(jnp.where(cm == second, ci, big), axis=0, keepdims=True)
    idx_a = jnp.clip(ia.astype(jnp.int32)[0, 0], 0, S - 1)
    idx_b = jnp.clip(ib.astype(jnp.int32)[0, 0], 0, S - 1)

    sub = lax.broadcasted_iota(jnp.int32, (16, D), 0)
    xa = jnp.broadcast_to(x1_v[pl.ds(idx_a, 1), :], (16, D))
    xb = jnp.broadcast_to(x1_v[pl.ds(idx_b, 1), :], (16, D))
    hsel, _ = ln2(jnp.where(sub == 0, xa, xb))
    gate_r = jax.nn.sigmoid(jnp.sum(hsel * wr_row, axis=-1, keepdims=True))
    hb = hsel.astype(BF)
    copies["wg"].wait()
    copies["wu"].wait()
    copies["wd"].wait()
    g = _dot(hb, wg_v[...], NN)
    u = _dot(hb, wu_v[...], NN)
    act = (g * jax.nn.sigmoid(g) * u).astype(BF)
    y = _dot(act, wd_v[...], NN) * gate_r * mod_v[5, 0:1, :]

    for t in range(NTILE):
        out_copy(t).wait()

    def fix(idx, slot):
        base = pl.multiple_of((idx // 16) * 16, 16)
        _, o = ln2(x1_v[pl.ds(base, 16), :])
        o = o + jnp.where(sub + base == idx_a, y[0:1], 0.0) + jnp.where(sub + base == idx_b, y[1:2], 0.0)
        slab_v[slot] = o.astype(BF)
        return pltpu.make_async_copy(slab_v.at[slot], out_hbm.at[pl.ds(base, 16)], osems.at[slot])

    fa = fix(idx_a, 0)
    fa.start()

    @pl.when(idx_a // 16 != idx_b // 16)
    def _():
        fb = fix(idx_b, 1)
        fb.start()
        fb.wait()

    fa.wait()


def make(T=512, CH=256):
    def run(A_x, A_wqkv, A_w_phi, A_wo, B_x, B_w_r, B_w_gate, B_w_up, B_w_down, c, w_mod):
        del B_x
        any_spec = pl.BlockSpec(memory_space=pl.ANY)
        scratch = [
            pltpu.VMEM((S, D), BF), pltpu.VMEM((3, D, D), BF), pltpu.VMEM((H, DH, DH), BF),
            pltpu.VMEM((D, D), BF), pltpu.VMEM((8, 128), BF),
            pltpu.VMEM((D, F), BF), pltpu.VMEM((D, F), BF), pltpu.VMEM((F, D), BF),
            pltpu.VMEM((1, D), BF), pltpu.VMEM((6, D, D), BF),
            pltpu.VMEM((D, D), BF), pltpu.VMEM((D, D), BF), pltpu.VMEM((D, D), BF),
            pltpu.VMEM((S, D), BF), pltpu.VMEM((S, D), F32), pltpu.VMEM((S, D), BF),
            pltpu.VMEM((H // 2, 64, 128), F32), pltpu.VMEM((H // 2, 128, 128), F32),
            pltpu.VMEM((H // 2, 64, 128), BF), pltpu.VMEM((H // 2, 128, 128), F32),
            pltpu.VMEM((6, 8, D), F32), pltpu.VMEM((4, 8, 128), F32), pltpu.VMEM((2, 16, D), BF),
            pltpu.SemaphoreType.DMA((18,)), pltpu.SemaphoreType.DMA((max(S // T, 2),)),
        ]
        out = pl.pallas_call(
            functools.partial(_kernel, T=T, CH=CH),
            out_shape=jax.ShapeDtypeStruct((S, D), BF),
            in_specs=[any_spec] * 10,
            out_specs=any_spec,
            scratch_shapes=scratch,
            compiler_params=pltpu.CompilerParams(vmem_limit_bytes=120 * 2**20),
            name="fused_block",
        )(A_x.reshape(S, D), A_wqkv, A_w_phi, A_wo, B_w_r.reshape(8, 128), B_w_gate, B_w_up, B_w_down, c, w_mod)
        return out.reshape(1, S, D)
    return run


_run = make(**dict(T=512, CH=256))


@jax.jit
def pallas_adaLN_cond__linear_kernel_hedgehog__moe_arch_mod__prompt_kernel(
    A_x: jax.Array,
    A_wqkv: jax.Array,
    A_w_phi: jax.Array,
    A_wo: jax.Array,
    B_x: jax.Array,
    B_w_r: jax.Array,
    B_w_gate: jax.Array,
    B_w_up: jax.Array,
    B_w_down: jax.Array,
    c: jax.Array,
    w_mod: jax.Array,
):
    return _run(A_x, A_wqkv, A_w_phi, A_wo, B_x, B_w_r, B_w_gate, B_w_up, B_w_down, c, w_mod)
```

```python
import functools

import jax
import jax.numpy as jnp
from jax import lax
from jax.experimental import pallas as pl
from jax.experimental.pallas import tpu as pltpu

S, D, H, DH, F = 2048, 1024, 32, 32, 3584
T = 512
TH = T // 2
DHALF = D // 2
NTILE = S // T
NCH = D // 256
LOG2E = 1.4426950408889634
NN = (((1,), (0,)), ((), ()))
NT = (((1,), (1,)), ((), ()))
TN = (((0,), (0,)), ((), ()))
BF = jnp.bfloat16
F32 = jnp.float32
I32 = jnp.int32


def _dot(a, b, dims):
    return lax.dot_general(a, b, dims, preferred_element_type=F32)


def _center(x, order=None):
    s = jnp.sum(x, axis=-1, keepdims=True)
    if order is not None:
        s = order.after(s)
    xc = x - s * (1.0 / D)
    rs = lax.rsqrt(jnp.sum(xc * xc, axis=-1, keepdims=True) * (1.0 / D) + 1e-5)
    if order is not None:
        order.link = rs
    return xc, rs


def _pair_reduce(x, op):
    r = x[0:8]
    for i in range(1, 8):
        r = op(r, x[8 * i:8 * i + 8])
    r = op(r, pltpu.roll(r, 4, 0))
    return op(r, pltpu.roll(r, 2, 0))


def _tile8(r, n):
    return jnp.concatenate([r] * n, axis=0)


def _hedgehog(p):
    mx = _tile8(_pair_reduce(p, jnp.maximum), 8)
    mn = _tile8(_pair_reduce(p, jnp.minimum), 8)
    ep = jnp.exp2(p - mx)
    en = jnp.exp2(mn - p)
    rp = _tile8(1.0 / _pair_reduce(ep, jnp.add), 8)
    rn = _tile8(1.0 / _pair_reduce(en, jnp.add), 8)
    return jnp.concatenate([ep * rp, en * rn], axis=0)


def _lhs_terms(a11, a12, a21, a22):
    return (a11 + a22, a21 + a22, a11, a22, a11 + a12, a21 - a11, a12 - a22)


def _rhs_terms(b11, b12, b21, b22):
    return (b11 + b22, b11, b12 - b22, b21 - b11, b22, b11 + b12, b21 + b22)


def _block_product(product, fill, lower_done=None):
    m0 = product(0)
    fill(0, m0)
    m1 = product(1)
    fill(1, m1)
    c22 = m0 - m1
    m3 = product(3)
    fill(2, m3)
    c21 = m1 + m3
    c11 = m0 + m3
    m2 = product(2)
    fill(3, m2)
    c22 = c22 + m2
    m5 = product(5)
    fill(4, m5)
    lower = jnp.concatenate([c21, c22 + m5], axis=1)
    if lower_done is not None:
        lower_done(lower)
    m4 = product(4)
    fill(5, m4)
    c12 = m2 + m4
    c11 = c11 - m4
    m6 = product(6)
    fill(6, m6)
    return jnp.concatenate([c11 + m6, c12], axis=1), lower


def _pack(x):
    return pltpu.bitcast(x.astype(BF), I32)


def _unpack(x):
    return pltpu.bitcast(x, BF)


class _Order:
    def __init__(self, never):
        self.never = never
        self.link = None
        self.release = None

    def after(self, v):
        for dep in (self.link, self.release):
            if dep is not None:
                v = jnp.where(self.never, dep[:v.shape[0], :v.shape[1]], v)
        return v


def _kernel(x_hbm, wqkv_hbm, wphi_hbm, wo_hbm, wr_hbm, wg_hbm, wu_hbm, wd_hbm, c_hbm, wmod_hbm,
            out_hbm,
            x_v, wqkv_v, wphi_v, wo_v, wr_v, wg_v, wu_v, wd_v, c_v, wmod_v,
            wkv_c, wq_c, wo_c, hc_v, oc_v, x1_v, kv_acc, z_acc, kvT, zb, mod_v, slab_v, idle_sem,
            sems, osems, *, cfg):
    R1, R2 = cfg.get("R1", 16), cfg.get("R2", 16)

    def col(ref, j, w=D):
        return ref.at[:, pl.ds(j * w, w)]

    def x_copy(t):
        return ("x%d" % t, x_hbm.at[pl.ds(t * T, T)], x_v.at[pl.ds(t * T, T)])

    def w_copy(name, j, c):
        return ("%s%d" % (name, c), col(wqkv_hbm, j * NCH + c, 256), wqkv_v.at[j * NCH + c])

    def mod_copy(name, j):
        return (name, col(wmod_hbm, j), wmod_v.at[j, :, pl.ds(0, D)])

    order = [("c", c_hbm, c_v), ("wphi", wphi_hbm, wphi_v), ("wr", wr_hbm, wr_v),
             x_copy(0), w_copy("wk", 1, 0), w_copy("wv", 2, 0), mod_copy("sa", 0), mod_copy("ca", 1),
             w_copy("wk", 1, 1), w_copy("wv", 2, 1), x_copy(1),
             w_copy("wk", 1, 2), w_copy("wv", 2, 2), w_copy("wk", 1, 3), w_copy("wv", 2, 3),
             x_copy(2), x_copy(3)]
    order += [w_copy("wq", 0, c) for c in range(NCH)]
    order += [("wo", wo_hbm, wo_v), mod_copy("ga", 2), mod_copy("sb", 3), mod_copy("cb", 4), mod_copy("gb", 5),
              ("wg", wg_hbm, wg_v), ("wu", wu_hbm, wu_v), ("wd", wd_hbm, wd_v.at[:, pl.ds(0, D)])]
    copies = {}
    for i, (name, src, dst) in enumerate(order):
        copies[name] = pltpu.make_async_copy(src, dst, sems.at[i])
        copies[name].start()

    waited, started = set(), []

    def wait(*names):
        for name in names:
            copies[name].wait()
            waited.add(name)

    never = pl.semaphore_read(idle_sem) != 0
    order1, order2 = _Order(never), _Order(never)

    wait("c", "wphi", "wr")
    cf = c_v[...].astype(F32)
    sc = jnp.broadcast_to(cf * jax.nn.sigmoid(cf), (16, D)).astype(BF)

    row = lax.broadcasted_iota(I32, (128, DH), 0)
    lane = lax.broadcasted_iota(I32, (128, DH), 1)
    expand = jnp.where(((row % 64) // 2) == lane, 1.0, 0.0).astype(BF)
    bdt = _dot(expand, wphi_v[...].reshape(H * DH, DH), NT)
    row = lax.broadcasted_iota(I32, (128, D), 0)
    lane = lax.broadcasted_iota(I32, (128, D), 1)
    bdt = jnp.where(2 * (row // 64) + (row % 2) == (lane % 128) // DH, bdt, 0.0).astype(BF)

    def mod_row(j):
        return _dot(sc, wmod_v[j, :, pl.ds(0, D)], NN)[0:8]

    def mod_part(j, n, half):
        part = _dot(sc[:, half * DHALF:(half + 1) * DHALF],
                    wmod_v[j, pl.ds(half * DHALF, DHALF), pl.ds(n * 128, 128)], NN)[0:8]
        if half == 0:
            mod_v[j, :, pl.ds(n * 128, 128)] = part
        else:
            mod_v[j, :, pl.ds(n * 128, 128)] += part

    def finish_mod():
        wr = wr_v[...].astype(F32)
        wr_row = jnp.concatenate([jnp.broadcast_to(wr[j:j + 1, :], (8, 128)) for j in range(8)], axis=1)
        shift, scale, gate = mod_v[3], 1.0 + mod_v[4], mod_v[5]
        mod_v[4] = scale
        mod_v[6] = gate * scale
        mod_v[7] = gate * shift
        mod_v[8] = wr_row * scale
        mod_v[9] = jnp.broadcast_to(jnp.sum(wr_row * shift, axis=-1, keepdims=True), (8, D))

    def rows_of(j, n):
        return _tile8(mod_v[j], n // 8)

    def h_term(t, i, r0=0, n=TH):
        return (t, i // 2, pl.ds(r0, n), pl.ds((i % 2) * DHALF, DHALF))

    def store_h_terms(t, r0, n, a, b):
        h1 = a * rows_of(1, n) + rows_of(0, n)
        h2 = b * rows_of(1, n) + rows_of(0, n)
        terms = _rhs_terms(h1[:, :DHALF], h2[:, :DHALF], h1[:, DHALF:], h2[:, DHALF:])
        for i, term in enumerate(terms):
            hc_v[h_term(t, i, r0, n)] = term.astype(BF)

    def normalized(tok, n, order=None):
        xc, rs = _center(x_v[pl.ds(tok, n), :].astype(F32), order)
        return xc * rs

    def ln1_piece(t, r0):
        store_h_terms(t, r0, R1, normalized(t * T + r0, R1, order1), normalized(t * T + TH + r0, R1, order1))

    def store_lhs_terms(top, bot, dst, c, r0):
        terms = _lhs_terms(top[:, :DHALF], top[:, DHALF:], bot[:, :DHALF], bot[:, DHALF:])
        for i, term in enumerate(terms):
            dst[c, i, pl.ds(r0, 64), :] = _pack(term)

    def fold(j, c, dst):
        halves = []
        for g in range(2):
            w = wqkv_v[j * NCH + c, :, g * 128:(g + 1) * 128]
            gg = 2 * c + g
            halves.append(_dot(bdt[:, gg * 128:(gg + 1) * 128], w, NT) * LOG2E)
        store_lhs_terms(halves[0], halves[1], dst, c, 0)

    def prep_v(c):
        halves = [wqkv_v[2 * NCH + c, :, g * 128:(g + 1) * 128].T.astype(F32) for g in range(2)]
        store_lhs_terms(halves[0], halves[1], wkv_c, c, 64)

    def prep_wo(c, r0):
        top = wo_v[pl.ds(c * 256 + r0, 32), :].astype(F32)
        bot = wo_v[pl.ds(c * 256 + 128 + r0, 32), :].astype(F32)
        terms = _rhs_terms(top[:, :DHALF], top[:, DHALF:], bot[:, :DHALF], bot[:, DHALF:])
        for i, term in enumerate(terms):
            wo_c[i, pl.ds(c * 64 + r0 // 2, 16), :] = _pack(term)

    def kv_pair(t, c, res, k):
        g, q = divmod(k, 2)
        pair = 4 * c + k
        phi = _hedgehog(res[g][q * 64:(q + 1) * 64])
        vt = res[g][128 + q * 64:128 + (q + 1) * 64].astype(BF)
        zs = phi[:, 0:128]
        for l in range(1, T // 128):
            zs = zs + phi[:, l * 128:(l + 1) * 128]
        kv = _dot(vt, phi.astype(BF), NT)
        if t > 0:
            zs = zs + z_acc[pair]
            kv = kv + kv_acc[pair]
        if t < NTILE - 1:
            z_acc[pair] = zs
            kv_acc[pair] = kv
        else:
            row = lax.broadcasted_iota(I32, (64, 128), 0)
            lane = lax.broadcasted_iota(I32, (64, 128), 1)
            kvT[pair] = jnp.where((row // DH) == (lane % 2), kv, 0.0).astype(BF)
            zb[pair] = jnp.broadcast_to(jnp.sum(zs, axis=-1, keepdims=True), (128, 128))

    def q_pair(c, res, k):
        g, q = divmod(k, 2)
        pair = 4 * c + k
        even = (lax.broadcasted_iota(I32, (8, T), 0) % 2) == 0
        phi = _hedgehog(res[g][q * 64:(q + 1) * 64])
        num = _dot(kvT[pair], phi.astype(BF), NN)
        w = phi * jnp.concatenate([zb[pair]] * (T // 128), axis=1)
        inv = 1.0 / (_pair_reduce(w[0:64] + w[64:128], jnp.add) + 1e-6)
        swapped = pltpu.roll(inv, 1, 0)
        inv_a = jnp.where(even, inv, swapped)
        inv_b = jnp.where(even, swapped, inv)
        return num * jnp.concatenate([inv_a] * 4 + [inv_b] * 4, axis=0)

    held = {}

    def q_lower(c, res, q):
        held[q] = q_pair(c, res, 2 + q)

    def q_upper(t, c, res, q):
        o1, o2 = q_pair(c, res, q), held.pop(q)
        terms = _lhs_terms(o1[:, :TH], o2[:, :TH], o1[:, TH:], o2[:, TH:])
        for i, term in enumerate(terms):
            oc_v[t, i, pl.ds(c * 128 + q * 64, 64), :] = term.astype(BF)

    def residual(tok, attn):
        rows = pl.ds(tok, 128)
        x1_v[rows, :] = x_v[rows, :].astype(F32) + rows_of(2, 128) * attn

    def block_out(x1, xc, rs):
        n = x1.shape[0]
        return xc * (rs * rows_of(6, n)) + (x1 + rows_of(7, n))

    def router(xc, rs):
        n = xc.shape[0]
        return jnp.sum(xc * rows_of(8, n), axis=-1, keepdims=True) * rs + rows_of(9, n)[:, 0:1]

    neg = jnp.full((8, 128), -jnp.inf, F32)
    top = [neg, neg, jnp.zeros((8, 128), F32), jnp.zeros((8, 128), F32)]

    def ln2_piece(tok, order):
        x1 = x1_v[pl.ds(tok, R2), :]
        xc, rs = _center(x1, order)
        t, r0 = divmod(tok, T)
        hc_v[t, r0 // TH, pl.ds(r0 % TH, R2), :] = block_out(x1, xc, rs).astype(BF)
        r = router(xc, rs)
        sub = lax.broadcasted_iota(I32, (8, 128), 0).astype(F32)
        m1, m2, i1, i2 = top
        for g in range(R2 // 8):
            rg = jnp.broadcast_to(r[g * 8:(g + 1) * 8], (8, 128))
            ig = sub + float(tok + g * 8)
            gt1 = (rg > m1) | ((rg == m1) & (ig < i1))
            gt2 = (rg > m2) | ((rg == m2) & (ig < i2))
            m2 = jnp.where(gt1, m1, jnp.where(gt2, rg, m2))
            i2 = jnp.where(gt1, i1, jnp.where(gt2, ig, i2))
            m1 = jnp.where(gt1, rg, m1)
            i1 = jnp.where(gt1, ig, i1)
        top[:] = m1, m2, i1, i2

    def out_copy(t, half):
        return pltpu.make_async_copy(hc_v.at[t, half], out_hbm.at[pl.ds(t * T + half * TH, TH)],
                                     osems.at[2 * t + half])

    def start_out(t):
        for half in range(2):
            out_copy(t, half).start()
        started.append(t)

    wait("x0")
    for r0 in range(0, T, 32):
        x1_v[pl.ds(r0, 32), :] = normalized(r0, 32)
    wait("wk0", "wv0")
    fold(1, 0, wkv_c)
    prep_v(0)
    wait("sa")
    mod_v[0] = mod_row(0)
    wait("ca")
    mod_v[1] = 1.0 + mod_row(1)
    for r0 in range(0, TH, 32):
        store_h_terms(0, r0, 32, x1_v[pl.ds(r0, 32), :], x1_v[pl.ds(TH + r0, 32), :])

    P = functools.partial

    def spread(slots, lo, hi, works):
        for n, work in enumerate(works):
            slots[lo + n * (hi - lo) // len(works)].append(work)

    steps = [("kv", t, c) for t in range(NTILE) for c in range(NCH)]
    steps += [("q", t, c) for t in range(NTILE) for c in range(NCH)]
    steps += [("o", t, s) for t in range(NTILE) for s in range(2)]
    if cfg.get("only"):
        steps = [steps[i] for i in cfg["only"]]
    mod_parts = [P(mod_part, j, n, half) for j in range(2, 6) for half in range(2) for n in range(8)]
    prev = None
    for step, (kind, t, c) in enumerate(steps):
        slots = [[] for _ in range(7)]
        lower_done = None
        if prev is not None:
            pkind, pt, pc, pres = prev
            if pkind == "kv":
                for slot, k in zip(cfg.get("ks", (0, 1, 2, 3)), (2, 3, 0, 1)):
                    slots[slot].append(P(kv_pair, pt, pc, pres, k))
            elif pkind == "q":
                qs = cfg.get("qs", (0, 1, 3, 5))
                slots[qs[0]].append(P(q_lower, pc, pres, 0))
                slots[qs[1]].append(P(q_lower, pc, pres, 1))
                slots[qs[2]].append(P(q_upper, pt, pc, pres, 0))
                slots[qs[3]].append(P(q_upper, pt, pc, pres, 1))
            else:
                tok = pt * T + pc * 128
                slots[0].append(P(residual, tok, pres[0]))
                lo, hi = cfg.get("l2a", (0, 4))
                spread(slots, lo, hi, [P(ln2_piece, tok + r0, order2) for r0 in range(0, 128, R2)])
                if pc == 1:
                    slots[hi].append(P(start_out, pt))
        if kind == "kv":
            if t == 0:
                if c == 0:
                    slots[3].insert(0, P(wait, "wk1", "wv1"))
                if c == 1:
                    slots[3].insert(0, P(wait, "x1", "wk2", "wv2", "wk3", "wv3"))
                if c == NCH - 1:
                    slots[3].insert(0, P(wait, "x2", "x3", "wq0", "wq1", "wq2", "wq3"))
                if c + 1 < NCH:
                    slots[4].append(P(fold, 1, c + 1, wkv_c))
                    slots[5].append(P(prep_v, c + 1))
            if t + 1 < NTILE:
                chunks = (2, 3) if t == 0 else (0, 1, 2, 3)
                if c in chunks:
                    pieces = list(range(0, TH, R1))
                    k = chunks.index(c)
                    mine = pieces[k * len(pieces) // len(chunks):(k + 1) * len(pieces) // len(chunks)]
                    spread(slots, 0, 6, [P(ln1_piece, t + 1, r0) for r0 in mine])
            if t == cfg.get("foldq", 1):
                slots[5].append(P(fold, 0, c, wq_c))
            if t == 3:
                if c == 0:
                    slots[0].insert(0, P(wait, "wo", "ga", "sb", "cb", "gb"))
                spread(slots, 1, 7, [P(prep_wo, c, r0) for r0 in range(0, 128, 32)])
                if not cfg.get("modparts"):
                    slots[5].append(lambda j=2 + c: mod_v.__setitem__(j, mod_row(j)))
        if cfg.get("modparts") and mod_parts and (kind, t) >= ("kv", 3) and kind != "o":
            for k in range(1 if (kind, t, c) == ("kv", 3, 0) else 0, 7):
                if mod_parts:
                    slots[k].insert(0, mod_parts.pop(0))
        if (kind, t, c) == ("q", 2, 0):
            slots[6].append(finish_mod)
        if kind == "o":
            last = step == len(steps) - 1
            tok2 = t * T + TH + c * 128
            lower_done = P(residual, tok2)
            lo, hi = (5, 6) if last else cfg.get("l2b", (5, 7))
            spread(slots, lo, hi, [P(ln2_piece, tok2 + r0, None if last else order2) for r0 in range(0, 128, R2)])

        def fill(k, m, slots=slots):
            if cfg.get("tie", True):
                order1.release = order2.release = m
            for work in slots[k]:
                work()

        if kind == "kv":
            res = _block_product(lambda i: _dot(_unpack(wkv_c[c, i]), hc_v[h_term(t, i)], NT), fill)
        elif kind == "q":
            res = _block_product(lambda i: _dot(_unpack(wq_c[c, i]), hc_v[h_term(t, i)], NT), fill)
        else:
            res = _block_product(
                lambda i: _dot(oc_v[t, i, :, pl.ds(c * 128, 128)], _unpack(wo_c[i]), TN), fill, lower_done)
        if kind == "kv" and c == NCH - 1:
            order1.link = None
        prev = (kind, t, c, res)

    if cfg.get("only"):
        for name in copies:
            if name not in waited:
                wait(name)
        a, b = prev[3]
        x1_v[0:128, 0:256] = a[0:128, 0:256] + b[0:128, 0:256] + a[0:128, 256:512] + b[0:128, 256:512]
        x1_v[128:136, 0:128] = top[0] + top[1] + top[2] + top[3]
        for t in started:
            out_copy(t, 0).wait()
            out_copy(t, 1).wait()
        return

    _, pt, pc, pres = prev
    tok = pt * T + pc * 128
    residual(tok, pres[0])
    for r0 in range(0, 128, R2):
        ln2_piece(tok + r0, None)
    start_out(pt)

    m1, m2, i1, i2 = top
    big = float(2 * S)
    best = jnp.max(m1, axis=0, keepdims=True)
    ia = jnp.min(jnp.where(m1 == best, i1, big), axis=0, keepdims=True)
    taken = i1 == ia
    cm = jnp.where(taken, m2, m1)
    ci = jnp.where(taken, i2, i1)
    second = jnp.max(cm, axis=0, keepdims=True)
    ib = jnp.min(jnp.where(cm == second, ci, big), axis=0, keepdims=True)
    idx_a = jnp.clip(ia.astype(I32)[0, 0], 0, S - 1)
    idx_b = jnp.clip(ib.astype(I32)[0, 0], 0, S - 1)

    sub = lax.broadcasted_iota(I32, (16, D), 0)
    xa = jnp.broadcast_to(x1_v[pl.ds(idx_a, 1), :], (16, D))
    xb = jnp.broadcast_to(x1_v[pl.ds(idx_b, 1), :], (16, D))
    xc, rs = _center(jnp.where(sub == 0, xa, xb))
    gate_r = jax.nn.sigmoid(router(xc, rs))
    hb = (xc * rs * rows_of(4, 16) + rows_of(3, 16)).astype(BF)
    wait("wg", "wu", "wd")
    g = _dot(hb, wg_v[...], NN)
    u = _dot(hb, wu_v[...], NN)
    act = (g * jax.nn.sigmoid(g) * u).astype(BF)
    y = _dot(act, wd_v[:, pl.ds(0, D)], NN) * gate_r * rows_of(5, 16)

    for t in range(NTILE):
        out_copy(t, 0).wait()
        out_copy(t, 1).wait()

    def fix(idx, slot):
        start = pl.multiple_of((idx // 16) * 16, 16)
        x1 = x1_v[pl.ds(start, 16), :]
        o = block_out(x1, *_center(x1))
        o = o + jnp.where(sub + start == idx_a, y[0:1], 0.0) + jnp.where(sub + start == idx_b, y[1:2], 0.0)
        slab_v[slot] = o.astype(BF)
        return pltpu.make_async_copy(slab_v.at[slot], out_hbm.at[pl.ds(start, 16)], osems.at[slot])

    fa = fix(idx_a, 0)
    fb = fix(idx_b, 1)
    fa.start()

    @pl.when(idx_a // 16 != idx_b // 16)
    def _():
        fb.start()
        fb.wait()

    fa.wait()


def make(flags=None, **cfg):
    if cfg.get("ev", True):
        flags = dict(flags or {}, XLA_TPU_EVENLY_DISTRIBUTE_CRITICAL_NODES=True)
    pad = cfg.get("pad", 128)

    def run(A_x, A_wqkv, A_w_phi, A_wo, B_x, B_w_r, B_w_gate, B_w_up, B_w_down, c, w_mod):
        del B_x
        any_spec = pl.BlockSpec(memory_space=pl.ANY)
        scratch = [
            pltpu.VMEM((S, D), BF), pltpu.VMEM((3 * NCH, D, 256), BF), pltpu.VMEM((H, DH, DH), BF),
            pltpu.VMEM((D, D), BF), pltpu.VMEM((8, 128), BF),
            pltpu.VMEM((D, F), BF), pltpu.VMEM((D, F), BF), pltpu.VMEM((F, D + pad), BF),
            pltpu.VMEM((1, D), BF), pltpu.VMEM((6, D, D + pad), BF),
            pltpu.VMEM((NCH, 7, 128, DHALF), I32), pltpu.VMEM((NCH, 7, 64, DHALF), I32),
            pltpu.VMEM((7, DHALF // 2, DHALF), I32),
            pltpu.VMEM((NTILE, 4, TH, D), BF), pltpu.VMEM((NTILE, 7, DHALF, TH), BF), pltpu.VMEM((S, D), F32),
            pltpu.VMEM((H // 2, 64, 128), F32), pltpu.VMEM((H // 2, 128, 128), F32),
            pltpu.VMEM((H // 2, 64, 128), BF), pltpu.VMEM((H // 2, 128, 128), F32),
            pltpu.VMEM((10, 8, D), F32), pltpu.VMEM((2, 16, D), BF), pltpu.SemaphoreType.REGULAR,
            pltpu.SemaphoreType.DMA((32,)), pltpu.SemaphoreType.DMA((2 * NTILE,)),
        ]
        out = pl.pallas_call(
            functools.partial(_kernel, cfg=cfg),
            out_shape=jax.ShapeDtypeStruct((S, D), BF),
            in_specs=[any_spec] * 10,
            out_specs=any_spec,
            scratch_shapes=scratch,
            compiler_params=pltpu.CompilerParams(vmem_limit_bytes=120 * 2**20, flags=flags),
            name="fused_block",
        )(A_x.reshape(S, D), A_wqkv, A_w_phi, A_wo, B_w_r.reshape(8, 128), B_w_gate, B_w_up, B_w_down, c, w_mod)
        return out.reshape(1, S, D)
    return run


_run = make(**dict(tie=False))


@jax.jit
def pallas_adaLN_cond__linear_kernel_hedgehog__moe_arch_mod__prompt_kernel(
    A_x: jax.Array,
    A_wqkv: jax.Array,
    A_w_phi: jax.Array,
    A_wo: jax.Array,
    B_x: jax.Array,
    B_w_r: jax.Array,
    B_w_gate: jax.Array,
    B_w_up: jax.Array,
    B_w_down: jax.Array,
    c: jax.Array,
    w_mod: jax.Array,
):
    return _run(A_x, A_wqkv, A_w_phi, A_wo, B_x, B_w_r, B_w_gate, B_w_up, B_w_down, c, w_mod)
```

```python
import functools

import jax
import jax.numpy as jnp
from jax import lax
from jax.experimental import pallas as pl
from jax.experimental.pallas import tpu as pltpu

S, D, H, DH, F = 2048, 1024, 32, 32, 3584
T = 512
TH = T // 2
DHALF = D // 2
NTILE = S // T
NCH = D // 256
EARLY = 2
LOG2E = 1.4426950408889634
NN = (((1,), (0,)), ((), ()))
NT = (((1,), (1,)), ((), ()))
TN = (((0,), (0,)), ((), ()))
BF = jnp.bfloat16
F32 = jnp.float32
I32 = jnp.int32


def _dot(a, b, dims):
    return lax.dot_general(a, b, dims, preferred_element_type=F32)


def _center(x, order=None):
    s = jnp.sum(x, axis=-1, keepdims=True)
    if order is not None:
        s = order.after(s)
    xc = x - s * (1.0 / D)
    rs = lax.rsqrt(jnp.sum(xc * xc, axis=-1, keepdims=True) * (1.0 / D) + 1e-5)
    if order is not None:
        order.link = rs
    return xc, rs


def _pair_reduce(x, op):
    r = x[0:8]
    for i in range(1, 8):
        r = op(r, x[8 * i:8 * i + 8])
    r = op(r, pltpu.roll(r, 4, 0))
    return op(r, pltpu.roll(r, 2, 0))


def _tile8(r, n):
    return jnp.concatenate([r] * n, axis=0)


def _hedgehog(p):
    mx = _tile8(_pair_reduce(p, jnp.maximum), 8)
    mn = _tile8(_pair_reduce(p, jnp.minimum), 8)
    ep = jnp.exp2(p - mx)
    en = jnp.exp2(mn - p)
    rp = _tile8(1.0 / _pair_reduce(ep, jnp.add), 8)
    rn = _tile8(1.0 / _pair_reduce(en, jnp.add), 8)
    return jnp.concatenate([ep * rp, en * rn], axis=0)


def _lhs_terms(a11, a12, a21, a22):
    return (a11 + a22, a21 + a22, a11, a22, a11 + a12, a21 - a11, a12 - a22)


def _rhs_terms(b11, b12, b21, b22):
    return (b11 + b22, b11, b12 - b22, b21 - b11, b22, b11 + b12, b21 + b22)


def _block_product(product, fill, lower_done=None):
    m0 = product(0)
    fill(0, m0)
    m1 = product(1)
    fill(1, m1)
    c22 = m0 - m1
    m3 = product(3)
    fill(2, m3)
    c21 = m1 + m3
    c11 = m0 + m3
    m2 = product(2)
    fill(3, m2)
    c22 = c22 + m2
    m5 = product(5)
    fill(4, m5)
    lower = jnp.concatenate([c21, c22 + m5], axis=1)
    if lower_done is not None:
        lower_done(lower)
    m4 = product(4)
    fill(5, m4)
    c12 = m2 + m4
    c11 = c11 - m4
    m6 = product(6)
    fill(6, m6)
    return jnp.concatenate([c11 + m6, c12], axis=1), lower


def _pack(x):
    return pltpu.bitcast(x.astype(BF), I32)


def _unpack(x):
    return pltpu.bitcast(x, BF)


class _Order:
    def __init__(self, never):
        self.never = never
        self.link = None
        self.release = None

    def after(self, v):
        for dep in (self.link, self.release):
            if dep is not None:
                probe = self.never[:v.shape[0], :v.shape[1]]
                v = jnp.where(probe != probe, dep[:v.shape[0], :v.shape[1]], v)
        return v


def _kernel(x_hbm, wqkv_hbm, wphi_hbm, wo_hbm, wr_hbm, wg_hbm, wu_hbm, wd_hbm, c_hbm, wmod_hbm,
            out_hbm,
            x_v, wqkv_v, wphi_v, wo_v, wr_v, wg_v, wu_v, wd_v, c_v, wmod_v,
            wkv_c, wq_c, wo_c, hc_v, oc_v, x1_v, kv_acc, z_acc, kvT, zb, mod_v, sb_v, bias_v, slab_v, idle_sem,
            sems, osems, *, cfg):
    R1, R2 = cfg.get("R1", 16), cfg.get("R2", 16)

    def col(ref, j, w=D):
        return ref.at[:, pl.ds(j * w, w)]

    def x_copy(t):
        return ("x%d" % t, x_hbm.at[pl.ds(t * T, T)], x_v.at[pl.ds(t * T, T)])

    def w_copy(name, j, c):
        return ("%s%d" % (name, c), col(wqkv_hbm, j * NCH + c, 256), wqkv_v.at[j * NCH + c])

    def mod_copy(name, j):
        return (name, col(wmod_hbm, j), wmod_v.at[j, :, pl.ds(0, D)])

    order = [("c", c_hbm, c_v), x_copy(0), ("wphi", wphi_hbm, wphi_v),
             w_copy("wk", 1, 0), w_copy("wv", 2, 0), mod_copy("ca", 1),
             w_copy("wk", 1, 1), w_copy("wv", 2, 1), mod_copy("sa", 0),
             w_copy("wk", 1, 2), w_copy("wv", 2, 2), x_copy(1), w_copy("wk", 1, 3), w_copy("wv", 2, 3),
             x_copy(2), x_copy(3)]
    order += [w_copy("wq", 0, c) for c in range(NCH)]
    order += [("wr", wr_hbm, wr_v), ("wo", wo_hbm, wo_v), mod_copy("ga", 2), mod_copy("sb", 3), mod_copy("cb", 4), mod_copy("gb", 5),
              ("wg", wg_hbm, wg_v), ("wu", wu_hbm, wu_v), ("wd", wd_hbm, wd_v.at[:, pl.ds(0, D)])]
    copies = {}
    for i, (name, src, dst) in enumerate(order):
        copies[name] = pltpu.make_async_copy(src, dst, sems.at[i])
        copies[name].start()

    waited, started = set(), []

    def wait(*names):
        for name in names:
            copies[name].wait()
            waited.add(name)


    wait("c", "x0")
    cf = c_v[...].astype(F32)
    never = jnp.broadcast_to(cf[:, 0:128], (32, 128))
    order1, order2, order3, order4 = [_Order(never) for _ in range(4)]
    sc = jnp.broadcast_to(cf * jax.nn.sigmoid(cf), (16, D)).astype(BF)

    def normalized(tok, n, order=None):
        xc, rs = _center(x_v[pl.ds(tok, n), :].astype(F32), order)
        return xc * rs

    for r0 in range(0, T, 32):
        x1_v[pl.ds(r0, 32), :] = normalized(r0, 32)

    wait("wphi")
    row = lax.broadcasted_iota(I32, (128, DH), 0)
    lane = lax.broadcasted_iota(I32, (128, DH), 1)
    expand = jnp.where(((row % 64) // 2) == lane, 1.0, 0.0).astype(BF)
    bdt = _dot(expand, wphi_v[...].reshape(H * DH, DH), NT)
    row = lax.broadcasted_iota(I32, (128, D), 0)
    lane = lax.broadcasted_iota(I32, (128, D), 1)
    bdt = jnp.where(2 * (row // 64) + (row % 2) == (lane % 128) // DH, bdt, 0.0).astype(BF)

    def mod_row(j):
        return _dot(sc, wmod_v[j, :, pl.ds(0, D)], NN)[0:8]

    def mod_part(j, n, half):
        part = _dot(sc[:, half * DHALF:(half + 1) * DHALF],
                    wmod_v[j, pl.ds(half * DHALF, DHALF), pl.ds(n * 128, 128)], NN)[0:8]
        if half == 0:
            mod_v[j, :, pl.ds(n * 128, 128)] = part
        else:
            mod_v[j, :, pl.ds(n * 128, 128)] += part

    for k0 in range(0, D, 128):
        sb_v[pl.ds(k0, 128), :] = jnp.broadcast_to(sc[0:1, k0:k0 + 128].astype(F32), (128, 128)).T

    partial_mod = {}

    def mod_piece(j, k0, nk):
        acc = partial_mod.pop(j, None)
        for k in range(k0, k0 + nk, 16):
            s_col = sb_v[pl.ds(k, 16), :]
            if k == k0 and cfg.get("chain3"):
                s_col = order3.after(s_col)
            term = wmod_v[j, pl.ds(k, 16), pl.ds(0, D)].astype(F32) * jnp.concatenate([s_col] * (D // 128), axis=1)
            term = term[0:8] + term[8:16]
            acc = term if acc is None else acc + term
        if cfg.get("chain3"):
            link = acc[:, 0:128]
            for _ in range(cfg["chain3"]):
                link = jnp.broadcast_to(jnp.max(link, axis=-1, keepdims=True), (8, 128))
            order3.link = jnp.concatenate([link, link], axis=0)
        if k0 + nk < D:
            partial_mod[j] = acc
        else:
            mod_v[j] = jnp.broadcast_to(jnp.sum(acc, axis=0, keepdims=True), (8, D))

    def finish_mod():
        wr = wr_v[...].astype(F32)
        wr_row = jnp.concatenate([jnp.broadcast_to(wr[j:j + 1, :], (8, 128)) for j in range(8)], axis=1)
        shift, scale, gate = mod_v[3], 1.0 + mod_v[4], mod_v[5]
        mod_v[4] = scale
        mod_v[6] = gate * scale
        mod_v[7] = gate * shift
        mod_v[8] = wr_row * scale
        mod_v[9] = jnp.broadcast_to(jnp.sum(wr_row * shift, axis=-1, keepdims=True), (8, D))

    def rows_of(j, n):
        return _tile8(mod_v[j], n // 8)

    def h_term(t, i, r0=0, n=TH):
        return (t, i // 2, pl.ds(r0, n), pl.ds((i % 2) * DHALF, DHALF))

    def store_h_terms(t, r0, n, a, b, shift=True):
        h1, h2 = a * rows_of(1, n), b * rows_of(1, n)
        if shift:
            h1, h2 = h1 + rows_of(0, n), h2 + rows_of(0, n)
        terms = _rhs_terms(h1[:, :DHALF], h2[:, :DHALF], h1[:, DHALF:], h2[:, DHALF:])
        for i, term in enumerate(terms):
            hc_v[h_term(t, i, r0, n)] = term.astype(BF)

    def ln1_piece(t, r0):
        store_h_terms(t, r0, R1, normalized(t * T + r0, R1, order1), normalized(t * T + TH + r0, R1, order1))

    def store_lhs_terms(top, bot, dst, c, r0):
        terms = _lhs_terms(top[:, :DHALF], top[:, DHALF:], bot[:, :DHALF], bot[:, DHALF:])
        for i, term in enumerate(terms):
            if dst.dtype == I32:
                dst[c, i] = _pack(term)
            else:
                dst[c, i, pl.ds(r0, 128), :] = term.astype(BF)

    def keep_weights(c, r0, halves):
        if c < EARLY:
            for g in range(2):
                x1_v[pl.ds(T + c * 512 + g * 256 + r0, 128), :] = halves[g]

    def early_bias(r0, n):
        b = jnp.sum(x1_v[pl.ds(T + r0, n), :] * rows_of(0, n), axis=-1, keepdims=True)
        bias_v[pl.ds(r0, n), :] = jnp.broadcast_to(b, (n, 128))

    def first_tile_terms(slot, r0, shift):
        store_h_terms(slot, r0, 32, x1_v[pl.ds(r0, 32), :], x1_v[pl.ds(TH + r0, 32), :], shift)

    def fold(j, c, dst):
        halves = []
        for g in range(2):
            w = wqkv_v[j * NCH + c, :, g * 128:(g + 1) * 128]
            gg = 2 * c + g
            halves.append(_dot(bdt[:, gg * 128:(gg + 1) * 128], w, NT) * LOG2E)
        store_lhs_terms(halves[0], halves[1], dst, c, 0)
        if j == 1:
            keep_weights(c, 0, halves)

    def prep_v(c):
        halves = [wqkv_v[2 * NCH + c, :, g * 128:(g + 1) * 128].T.astype(F32) for g in range(2)]
        store_lhs_terms(halves[0], halves[1], wkv_c, c, 128)
        keep_weights(c, 128, halves)

    def prep_wo(c, r0):
        def rows(r):
            w = wo_v[pl.ds(r, 16), :].astype(F32)
            return jnp.concatenate([order3.after(w[:, l:l + 128]) for l in range(0, D, 128)], axis=1)
        top, bot = rows(c * 256 + r0), wo_v[pl.ds(c * 256 + 128 + r0, 16), :].astype(F32)
        terms = _rhs_terms(top[:, :DHALF], top[:, DHALF:], bot[:, :DHALF], bot[:, DHALF:])
        for i, term in enumerate(terms):
            wo_c[i, pl.ds(c * 64 + r0 // 2, 8), :] = _pack(term)
        order3.link = jnp.broadcast_to(jnp.max(terms[0][:, 0:128], axis=-1, keepdims=True), (16, 128))

    def kv_pair(t, c, res, k):
        g, q = divmod(k, 2)
        pair = 4 * c + k

        def rows(r0):
            val = res[g][r0:r0 + 64]
            if t == 0 and c < EARLY:
                val = val + jnp.concatenate([bias_v[pl.ds(c * 512 + g * 256 + r0, 64), :]] * (T // 128), axis=1)
            return val

        phi = _hedgehog(rows(q * 64))
        vt = rows(128 + q * 64).astype(BF)
        zs = phi[:, 0:128]
        for l in range(1, T // 128):
            zs = zs + phi[:, l * 128:(l + 1) * 128]
        kv = _dot(vt, phi.astype(BF), NT)
        if t > 0:
            zs = zs + z_acc[pair]
            kv = kv + kv_acc[pair]
        if t < NTILE - 1:
            z_acc[pair] = zs
            kv_acc[pair] = kv
        else:
            row = lax.broadcasted_iota(I32, (64, 128), 0)
            lane = lax.broadcasted_iota(I32, (64, 128), 1)
            kvT[pair] = jnp.where((row // DH) == (lane % 2), kv, 0.0).astype(BF)
            zb[pair] = jnp.broadcast_to(jnp.sum(zs, axis=-1, keepdims=True), (128, 128))

    def q_pair(c, res, k):
        g, q = divmod(k, 2)
        pair = 4 * c + k
        even = (lax.broadcasted_iota(I32, (8, T), 0) % 2) == 0
        phi = _hedgehog(res[g][q * 64:(q + 1) * 64])
        num = _dot(kvT[pair], phi.astype(BF), NN)
        w = phi * jnp.concatenate([zb[pair]] * (T // 128), axis=1)
        inv = 1.0 / (_pair_reduce(w[0:64] + w[64:128], jnp.add) + 1e-6)
        swapped = pltpu.roll(inv, 1, 0)
        inv_a = jnp.where(even, inv, swapped)
        inv_b = jnp.where(even, swapped, inv)
        return num * jnp.concatenate([inv_a] * 4 + [inv_b] * 4, axis=0)

    held = {}

    def q_step(t, c, res, k):
        held[k] = q_pair(c, res, k)
        if k == 3:
            held["lower"] = jnp.concatenate([held.pop(2), held.pop(3)], axis=0).T
        if k == 1:
            o1, o2 = jnp.concatenate([held.pop(0), held.pop(1)], axis=0).T, held.pop("lower")
            for i, term in enumerate(_lhs_terms(o1[:TH], o2[:TH], o1[TH:], o2[TH:])):
                oc_v[t, i, :, pl.ds(c * 128, 128)] = term.astype(BF)

    def residual(tok, attn):
        rows = pl.ds(tok, 128)
        x1_v[rows, :] = x_v[rows, :].astype(F32) + rows_of(2, 128) * attn

    def block_out(x1, xc, rs):
        n = x1.shape[0]
        return xc * (rs * rows_of(6, n)) + (x1 + rows_of(7, n))

    def router(xc, rs):
        n = xc.shape[0]
        return jnp.sum(xc * rows_of(8, n), axis=-1, keepdims=True) * rs + rows_of(9, n)[:, 0:1]

    neg = jnp.full((8, 128), -jnp.inf, F32)
    top = [neg, neg, jnp.zeros((8, 128), F32), jnp.zeros((8, 128), F32)]

    def ln2_piece(tok, order):
        x1 = x1_v[pl.ds(tok, R2), :]
        xc, rs = _center(x1, order)
        t, r0 = divmod(tok, T)
        hc_v[t, r0 // TH, pl.ds(r0 % TH, R2), :] = block_out(x1, xc, rs).astype(BF)
        r = router(xc, rs)
        sub = lax.broadcasted_iota(I32, (8, 128), 0).astype(F32)
        m1, m2, i1, i2 = top
        for g in range(R2 // 8):
            rg = jnp.broadcast_to(r[g * 8:(g + 1) * 8], (8, 128))
            ig = sub + float(tok + g * 8)
            gt1 = (rg > m1) | ((rg == m1) & (ig < i1))
            gt2 = (rg > m2) | ((rg == m2) & (ig < i2))
            m2 = jnp.where(gt1, m1, jnp.where(gt2, rg, m2))
            i2 = jnp.where(gt1, i1, jnp.where(gt2, ig, i2))
            m1 = jnp.where(gt1, rg, m1)
            i1 = jnp.where(gt1, ig, i1)
        top[:] = m1, m2, i1, i2

    def out_copy(t, half):
        return pltpu.make_async_copy(hc_v.at[t, half], out_hbm.at[pl.ds(t * T + half * TH, TH)],
                                     osems.at[2 * t + half])

    def start_out(t):
        for half in range(2):
            out_copy(t, half).start()
        started.append(t)

    wait("wk0", "wv0")
    fold(1, 0, wkv_c)
    prep_v(0)
    wait("ca")
    mod_v[1] = 1.0 + mod_row(1)
    for r0 in range(0, TH, 32):
        first_tile_terms(NTILE, r0, False)

    P = functools.partial

    def spread(slots, lo, hi, works):
        for n, work in enumerate(works):
            slots[lo + n * (hi - lo) // len(works)].append(work)

    steps = [("kv", t, c) for t in range(NTILE) for c in range(NCH)]
    steps += [("q", t, c) for t in range(NTILE) for c in range(NCH)]
    steps += [("o", t, s) for t in range(NTILE) for s in range(2)]
    if cfg.get("only"):
        steps = [steps[i] for i in cfg["only"]]
    mod_parts = [P(mod_part, j, n, half) for j in range(2, 6) for half in range(2) for n in range(8)]
    prev = None
    for step, (kind, t, c) in enumerate(steps):
        slots = [[] for _ in range(7)]
        lower_done = None
        if prev is not None:
            pkind, pt, pc, pres = prev
            if pkind == "kv":
                works = [P(kv_pair, pt, pc, pres, k) for k in (2, 3, 0, 1)]
                if (pt, pc) == (0, 0):
                    late, works = works[:2], works[2:]
                    delayed = works
                elif (pt, pc) == (0, 1):
                    for slot, work in enumerate(delayed + works):
                        slots[slot].append(work)
                else:
                    for slot, work in zip(cfg.get("ks", (0, 1, 2, 3)), works):
                        slots[slot].append(work)
            elif pkind == "q":
                qs = cfg.get("qs", (0, 1, 3, 5))
                for slot, k in zip(qs, (2, 3, 0, 1)):
                    slots[slot].append(P(q_step, pt, pc, pres, k))
            else:
                tok = pt * T + pc * 128
                slots[0].append(P(residual, tok, pres[0]))
                lo, hi = cfg.get("l2a", (0, 4))
                group = _Order(never) if cfg.get("groups", 1) == 1 else order2
                spread(slots, lo, hi, [P(ln2_piece, tok + r0, group) for r0 in range(0, 128, R2)])
                if pc == 1:
                    slots[hi].append(P(start_out, pt))
        if kind == "kv":
            if t == 0:
                if c == 0:
                    slots[cfg.get("w1", 2)] += [P(wait, "wk1", "wv1"), P(prep_v, 1), P(fold, 1, 1, wkv_c)]
                if c == 1:
                    slots[2] += [P(wait, "sa"), lambda: mod_v.__setitem__(0, mod_row(0))]
                    slots[3] += [P(early_bias, r0, 32) for r0 in range(0, 512 * EARLY, 32)]
                    slots[3] += [P(first_tile_terms, 0, r0, True) for r0 in range(0, TH, 32)]
                    slots[cfg.get("w2", 4)] += [P(wait, "wk2", "wv2"), P(prep_v, 2), P(fold, 1, 2, wkv_c)]
                    slots[5].append(late[0])
                    slots[6].append(late[1])
                if c == 2:
                    w3 = cfg.get("w3", 3)
                    slots[w3] = [P(wait, "x1", "wk3", "wv3"), P(prep_v, 3), P(fold, 1, 3, wkv_c)] + slots[w3]
            if (t, c) == (1, 2):
                slots[0].insert(0, P(wait, "x2", "x3", "wq0", "wq1", "wq2", "wq3", "wr", "wo"))
            if t + 1 < NTILE:
                chunks = ((3,), (2, 3), (0, 1, 2, 3))[t]
                if c in chunks:
                    pieces = list(range(0, TH, R1))
                    k = chunks.index(c)
                    mine = pieces[k * len(pieces) // len(chunks):(k + 1) * len(pieces) // len(chunks)]
                    spread(slots, 0, 6, [P(ln1_piece, t + 1, r0) for r0 in mine])
            if t == 2:
                slots[5].append(P(fold, 0, c, wq_c))
                spread(slots, 1, 7, [P(prep_wo, c, r0) for r0 in range(0, 128, 16)])
            if t == 3:
                if c == 0:
                    slots[0].insert(0, P(wait, "ga", "sb", "cb", "gb"))
                if cfg.get("vmod"):
                    nk = cfg["vmod"]
                    spread(slots, 1, 7, [P(mod_piece, 2 + c, k0, nk) for k0 in range(0, D, nk)])
                else:
                    slots[5].append(lambda j=2 + c: mod_v.__setitem__(j, mod_row(j)))
        if cfg.get("modparts") and mod_parts and (kind, t) >= ("kv", 3) and kind != "o":
            for k in range(1 if (kind, t, c) == ("kv", 3, 0) else 0, 7):
                if mod_parts:
                    slots[k].insert(0, mod_parts.pop(0))
        if (kind, t, c) == ("q", 0, 0):
            slots[0].insert(0, P(wait, "wg"))
            slots[6].append(finish_mod)
        if kind == "o":
            last = step == len(steps) - 1
            tok2 = t * T + TH + c * 128
            lower_done = P(residual, tok2)
            lo, hi = (5, 6) if last else cfg.get("l2b", (5, 7))
            group = _Order(never) if cfg.get("groups", 1) == 1 else order4
            spread(slots, lo, hi, [P(ln2_piece, tok2 + r0, None if last else group) for r0 in range(0, 128, R2)])

        def fill(k, m, slots=slots):
            if cfg.get("tie", True):
                order1.release = order2.release = m
            for work in slots[k]:
                work()

        if kind == "kv":
            slot = NTILE if t == 0 and c < EARLY else t
            res = _block_product(lambda i: _dot(wkv_c[c, i], hc_v[h_term(slot, i)], NT), fill)
        elif kind == "q":
            res = _block_product(lambda i: _dot(_unpack(wq_c[c, i]), hc_v[h_term(t, i)], NT), fill)
        else:
            res = _block_product(
                lambda i: _dot(oc_v[t, i, pl.ds(c * 128, 128), :], _unpack(wo_c[i]), NN), fill, lower_done)
        if kind == "kv" and c == NCH - 1:
            order1.link = None
        prev = (kind, t, c, res)

    if cfg.get("only"):
        for name in copies:
            if name not in waited:
                wait(name)
        a, b = prev[3]
        x1_v[0:128, 0:256] = a[0:128, 0:256] + b[0:128, 0:256] + a[0:128, 256:512] + b[0:128, 256:512]
        x1_v[128:136, 0:128] = top[0] + top[1] + top[2] + top[3]
        z = pl.semaphore_read(idle_sem)
        x1_v[136:144, :] = mod_v[z]
        x1_v[144:160, 0:512] = oc_v[z, z, 0:16, :].astype(F32) + hc_v[z, z, 0:16, 0:512].astype(F32) + (
            wo_c[z, 0:16, :] + wq_c[z, z, 0:16, :] + wkv_c[z, z, 0:16, :]).astype(F32)
        x1_v[160:176, 0:128] = kvT[z, 0:16, :].astype(F32) + zb[z, 0:16, :] + kv_acc[z, 0:16, :] + z_acc[z, 0:16, :]
        slab_v[0] = x1_v[pl.ds(pl.multiple_of(z * 16, 16), 16), :].astype(BF)
        cpy = pltpu.make_async_copy(slab_v.at[0], out_hbm.at[pl.ds(0, 16)], osems.at[0])
        cpy.start()
        cpy.wait()
        for t in started:
            out_copy(t, 0).wait()
            out_copy(t, 1).wait()
        return

    _, pt, pc, pres = prev
    tok = pt * T + pc * 128
    residual(tok, pres[0])
    for r0 in range(0, 128, R2):
        ln2_piece(tok + r0, None)
    start_out(pt)

    m1, m2, i1, i2 = top
    big = float(2 * S)
    best = jnp.max(m1, axis=0, keepdims=True)
    ia = jnp.min(jnp.where(m1 == best, i1, big), axis=0, keepdims=True)
    taken = i1 == ia
    cm = jnp.where(taken, m2, m1)
    ci = jnp.where(taken, i2, i1)
    second = jnp.max(cm, axis=0, keepdims=True)
    ib = jnp.min(jnp.where(cm == second, ci, big), axis=0, keepdims=True)
    idx_a = jnp.clip(ia.astype(I32)[0, 0], 0, S - 1)
    idx_b = jnp.clip(ib.astype(I32)[0, 0], 0, S - 1)

    sub = lax.broadcasted_iota(I32, (16, D), 0)
    xa = jnp.broadcast_to(x1_v[pl.ds(idx_a, 1), :], (16, D))
    xb = jnp.broadcast_to(x1_v[pl.ds(idx_b, 1), :], (16, D))
    xc, rs = _center(jnp.where(sub == 0, xa, xb))
    gate_r = jax.nn.sigmoid(router(xc, rs))
    hb = (xc * rs * rows_of(4, 16) + rows_of(3, 16)).astype(BF)
    wait("wu", "wd")
    g = _dot(hb, wg_v[...], NN)
    u = _dot(hb, wu_v[...], NN)
    act = (g * jax.nn.sigmoid(g) * u).astype(BF)
    y = _dot(act, wd_v[:, pl.ds(0, D)], NN) * gate_r * rows_of(5, 16)

    for t in range(NTILE):
        out_copy(t, 0).wait()
        out_copy(t, 1).wait()

    def fix(idx, slot):
        start = pl.multiple_of((idx // 16) * 16, 16)
        x1 = x1_v[pl.ds(start, 16), :]
        o = block_out(x1, *_center(x1))
        o = o + jnp.where(sub + start == idx_a, y[0:1], 0.0) + jnp.where(sub + start == idx_b, y[1:2], 0.0)
        slab_v[slot] = o.astype(BF)
        return pltpu.make_async_copy(slab_v.at[slot], out_hbm.at[pl.ds(start, 16)], osems.at[slot])

    fa = fix(idx_a, 0)
    fb = fix(idx_b, 1)
    fa.start()

    @pl.when(idx_a // 16 != idx_b // 16)
    def _():
        fb.start()
        fb.wait()

    fa.wait()


def make(flags=None, **cfg):
    cfg = dict(dict(tie=False, vmod=32, chain3=1, w1=1, w2=2, w3=1), **cfg)
    if cfg.get("ev", True):
        flags = dict(flags or {}, XLA_TPU_EVENLY_DISTRIBUTE_CRITICAL_NODES=True)
    pad = cfg.get("pad", 128)

    def run(A_x, A_wqkv, A_w_phi, A_wo, B_x, B_w_r, B_w_gate, B_w_up, B_w_down, c, w_mod):
        del B_x
        any_spec = pl.BlockSpec(memory_space=pl.ANY)
        scratch = [
            pltpu.VMEM((S, D), BF), pltpu.VMEM((3 * NCH, D, 256), BF), pltpu.VMEM((H, DH, DH), BF),
            pltpu.VMEM((D, D), BF), pltpu.VMEM((8, 128), BF),
            pltpu.VMEM((D, F), BF), pltpu.VMEM((D, F), BF), pltpu.VMEM((F, D + pad), BF),
            pltpu.VMEM((1, D), BF), pltpu.VMEM((6, D, D + pad), BF),
            pltpu.VMEM((NCH, 7, 256, DHALF), BF), pltpu.VMEM((NCH, 7, 64, DHALF), I32),
            pltpu.VMEM((7, DHALF // 2, DHALF), I32),
            pltpu.VMEM((NTILE + 1, 4, TH, D), BF), pltpu.VMEM((NTILE, 7, TH, DHALF), BF), pltpu.VMEM((S, D), F32),
            pltpu.VMEM((H // 2, 64, 128), F32), pltpu.VMEM((H // 2, 128, 128), F32),
            pltpu.VMEM((H // 2, 64, 128), BF), pltpu.VMEM((H // 2, 128, 128), F32),
            pltpu.VMEM((10, 8, D), F32), pltpu.VMEM((D, 128), F32), pltpu.VMEM((512 * EARLY, 128), F32), pltpu.VMEM((2, 16, D), BF), pltpu.SemaphoreType.REGULAR,
            pltpu.SemaphoreType.DMA((32,)), pltpu.SemaphoreType.DMA((2 * NTILE,)),
        ]
        out = pl.pallas_call(
            functools.partial(_kernel, cfg=cfg),
            out_shape=jax.ShapeDtypeStruct((S, D), BF),
            in_specs=[any_spec] * 10,
            out_specs=any_spec,
            scratch_shapes=scratch,
            compiler_params=pltpu.CompilerParams(vmem_limit_bytes=120 * 2**20, flags=flags),
            name="fused_block",
        )(A_x.reshape(S, D), A_wqkv, A_w_phi, A_wo, B_w_r.reshape(8, 128), B_w_gate, B_w_up, B_w_down, c, w_mod)
        return out.reshape(1, S, D)
    return run


_run = make(**dict())


@jax.jit
def pallas_adaLN_cond__linear_kernel_hedgehog__moe_arch_mod__prompt_kernel(
    A_x: jax.Array,
    A_wqkv: jax.Array,
    A_w_phi: jax.Array,
    A_wo: jax.Array,
    B_x: jax.Array,
    B_w_r: jax.Array,
    B_w_gate: jax.Array,
    B_w_up: jax.Array,
    B_w_down: jax.Array,
    c: jax.Array,
    w_mod: jax.Array,
):
    return _run(A_x, A_wqkv, A_w_phi, A_wo, B_x, B_w_r, B_w_gate, B_w_up, B_w_down, c, w_mod)
```

```python
import functools

import jax
import jax.numpy as jnp
from jax import lax
from jax.experimental import pallas as pl
from jax.experimental.pallas import tpu as pltpu

S, D, H, DH, F = 2048, 1024, 32, 32, 3584
T = 512
TH = T // 2
DHALF = D // 2
NTILE = S // T
NCH = D // 256
EARLY = 2
LOG2E = 1.4426950408889634
NN = (((1,), (0,)), ((), ()))
NT = (((1,), (1,)), ((), ()))
TN = (((0,), (0,)), ((), ()))
BF = jnp.bfloat16
F32 = jnp.float32
I32 = jnp.int32


def _dot(a, b, dims):
    return lax.dot_general(a, b, dims, preferred_element_type=F32)


def _recip(x):
    return pltpu.reciprocal(x, approx=False, full_range=False)


def _center(x, order=None):
    s = jnp.sum(x, axis=-1, keepdims=True)
    if order is not None:
        s = order.after(s)
    xc = x - s * (1.0 / D)
    rs = lax.rsqrt(jnp.sum(xc * xc, axis=-1, keepdims=True) * (1.0 / D) + 1e-5)
    if order is not None:
        order.link = rs
    return xc, rs


def _pair_reduce(x, op):
    r = x[0:8]
    for i in range(1, 8):
        r = op(r, x[8 * i:8 * i + 8])
    r = op(r, pltpu.roll(r, 4, 0))
    return op(r, pltpu.roll(r, 2, 0))


def _tile8(r, n):
    return jnp.concatenate([r] * n, axis=0)


def _hedgehog(p):
    mx = _tile8(_pair_reduce(p, jnp.maximum), 8)
    mn = _tile8(_pair_reduce(p, jnp.minimum), 8)
    ep = jnp.exp2(p - mx)
    en = jnp.exp2(mn - p)
    rp = _tile8(_recip(_pair_reduce(ep, jnp.add)), 8)
    rn = _tile8(_recip(_pair_reduce(en, jnp.add)), 8)
    return jnp.concatenate([ep * rp, en * rn], axis=0)


def _hedgehog_scaled(p):
    mx = _tile8(_pair_reduce(p, jnp.maximum), 8)
    mn = _tile8(_pair_reduce(p, jnp.minimum), 8)
    ep = jnp.exp2(p - mx)
    en = jnp.exp2(mn - p)
    sp = _pair_reduce(ep, jnp.add)
    ratio = _tile8(sp * _recip(_pair_reduce(en, jnp.add)), 8)
    return jnp.concatenate([ep, en * ratio], axis=0), sp


def _lhs_terms(a11, a12, a21, a22):
    return (a11 + a22, a21 + a22, a11, a22, a11 + a12, a21 - a11, a12 - a22)


def _rhs_terms(b11, b12, b21, b22):
    return (b11 + b22, b11, b12 - b22, b21 - b11, b22, b11 + b12, b21 + b22)


def _block_product(product, fill, lower_done=None):
    m0 = product(0)
    fill(0, m0)
    m1 = product(1)
    fill(1, m1)
    c22 = m0 - m1
    m3 = product(3)
    fill(2, m3)
    c21 = m1 + m3
    c11 = m0 + m3
    m2 = product(2)
    fill(3, m2)
    c22 = c22 + m2
    m5 = product(5)
    fill(4, m5)
    lower = jnp.concatenate([c21, c22 + m5], axis=1)
    if lower_done is not None:
        lower_done(lower)
    m4 = product(4)
    fill(5, m4)
    c12 = m2 + m4
    c11 = c11 - m4
    m6 = product(6)
    fill(6, m6)
    return jnp.concatenate([c11 + m6, c12], axis=1), lower


def _pack(x):
    return pltpu.bitcast(x.astype(BF), I32)


def _unpack(x):
    return pltpu.bitcast(x, BF)


class _Order:
    def __init__(self, never):
        self.never = never
        self.link = None
        self.release = None

    def after(self, v):
        for dep in (self.link, self.release):
            if dep is not None:
                probe = self.never[:v.shape[0], :v.shape[1]]
                v = jnp.where(probe != probe, dep[:v.shape[0], :v.shape[1]], v)
        return v


def _kernel(x_hbm, wqkv_hbm, wphi_hbm, wo_hbm, wr_hbm, wg_hbm, wu_hbm, wd_hbm, c_hbm, wmod_hbm,
            out_hbm,
            x_v, wqkv_v, wphi_v, wo_v, wr_v, wg_v, wu_v, wd_v, c_v, wmod_v,
            wkv_c, wq_c, wo_c, hc_v, oc_v, x1_v, kv_acc, z_acc, kvT, mod_v, sb_v, bias_v, slab_v, idle_sem,
            sems, osems, *, cfg):
    R1, R2 = cfg.get("R1", 16), cfg.get("R2", 16)
    NCA = cfg.get("nca", 4)

    def col(ref, j, w=D):
        return ref.at[:, pl.ds(j * w, w)]

    def x_copy(t):
        return ("x%d" % t, x_hbm.at[pl.ds(t * T, T)], x_v.at[pl.ds(t * T, T)])

    def w_copy(name, j, c):
        return ("%s%d" % (name, c), col(wqkv_hbm, j * NCH + c, 256), wqkv_v.at[j * NCH + c])

    def mod_copy(name, j):
        return (name, col(wmod_hbm, j), wmod_v.at[j, :, pl.ds(0, D)])

    def scale_copy(k):
        rows = pl.ds(k * (D // NCA), D // NCA)
        return ("ca%d" % k, wmod_hbm.at[rows, pl.ds(D, D)], wmod_v.at[1, rows, pl.ds(0, D)])

    order = [("c", c_hbm, c_v), x_copy(0), ("wphi", wphi_hbm, wphi_v),
             w_copy("wk", 1, 0), w_copy("wv", 2, 0), *[scale_copy(k) for k in range(NCA)],
             w_copy("wk", 1, 1), w_copy("wv", 2, 1), mod_copy("sa", 0),
             w_copy("wk", 1, 2), w_copy("wv", 2, 2), x_copy(1), w_copy("wk", 1, 3), w_copy("wv", 2, 3),
             x_copy(2), x_copy(3)]
    order += [w_copy("wq", 0, c) for c in range(NCH)]
    order += [("wr", wr_hbm, wr_v), ("wo", wo_hbm, wo_v), mod_copy("ga", 2), mod_copy("sb", 3), mod_copy("cb", 4), mod_copy("gb", 5),
              ("wg", wg_hbm, wg_v), ("wu", wu_hbm, wu_v), ("wd", wd_hbm, wd_v.at[:, pl.ds(0, D)])]
    copies = {}
    for i, (name, src, dst) in enumerate(order):
        copies[name] = pltpu.make_async_copy(src, dst, sems.at[i])
        copies[name].start()

    waited, started = set(), []

    scope = []

    def mark(name):
        if cfg.get("marks"):
            if scope:
                scope.pop().__exit__(None, None, None)
            if name:
                scope.append(jax.named_scope(name))
                scope[0].__enter__()

    def wait(*names):
        mark("w_" + names[0])
        for name in names:
            copies[name].wait()
            waited.add(name)
        mark("r_" + names[0])


    wait("c", "x0")
    cf = c_v[...].astype(F32)
    never = jnp.broadcast_to(cf[:, 0:128], (32, 128))
    order1, order2, order3, order4 = [_Order(never) for _ in range(4)]
    sc = jnp.broadcast_to(cf * jax.nn.sigmoid(cf), (16, D)).astype(BF)

    def normalized(tok, n, order=None):
        xc, rs = _center(x_v[pl.ds(tok, n), :].astype(F32), order)
        return xc * rs

    for r0 in range(0, T, 32):
        x1_v[pl.ds(r0, 32), :] = normalized(r0, 32)

    wait("wphi")
    row = lax.broadcasted_iota(I32, (128, DH), 0)
    lane = lax.broadcasted_iota(I32, (128, DH), 1)
    expand = jnp.where(((row % 64) // 2) == lane, 1.0, 0.0).astype(BF)
    bdt = _dot(expand, wphi_v[...].reshape(H * DH, DH), NT)
    row = lax.broadcasted_iota(I32, (128, D), 0)
    lane = lax.broadcasted_iota(I32, (128, D), 1)
    bdt = jnp.where(2 * (row // 64) + (row % 2) == (lane % 128) // DH, bdt, 0.0).astype(BF)

    def mod_row(j):
        return _dot(sc, wmod_v[j, :, pl.ds(0, D)], NN)[0:8]

    def mod_part(j, n, half):
        part = _dot(sc[:, half * DHALF:(half + 1) * DHALF],
                    wmod_v[j, pl.ds(half * DHALF, DHALF), pl.ds(n * 128, 128)], NN)[0:8]
        if half == 0:
            mod_v[j, :, pl.ds(n * 128, 128)] = part
        else:
            mod_v[j, :, pl.ds(n * 128, 128)] += part

    for k0 in range(0, D, 128):
        sb_v[pl.ds(k0, 128), :] = jnp.broadcast_to(sc[0:1, k0:k0 + 128].astype(F32), (128, 128)).T

    partial_mod = {}

    def mod_piece(j, k0, nk):
        acc = partial_mod.pop(j, None)
        for k in range(k0, k0 + nk, 16):
            s_col = sb_v[pl.ds(k, 16), :]
            if k == k0 and cfg.get("chain3"):
                s_col = order3.after(s_col)
            term = wmod_v[j, pl.ds(k, 16), pl.ds(0, D)].astype(F32) * jnp.concatenate([s_col] * (D // 128), axis=1)
            term = term[0:8] + term[8:16]
            acc = term if acc is None else acc + term
        if cfg.get("chain3"):
            link = acc[:, 0:128]
            for _ in range(cfg["chain3"]):
                link = jnp.broadcast_to(jnp.max(link, axis=-1, keepdims=True), (8, 128))
            order3.link = jnp.concatenate([link, link], axis=0)
        if k0 + nk < D:
            partial_mod[j] = acc
        else:
            mod_v[j] = jnp.broadcast_to(jnp.sum(acc, axis=0, keepdims=True), (8, D))

    def finish_mod():
        wr = wr_v[...].astype(F32)
        wr_row = jnp.concatenate([jnp.broadcast_to(wr[j:j + 1, :], (8, 128)) for j in range(8)], axis=1)
        shift, scale, gate = mod_v[3], 1.0 + mod_v[4], mod_v[5]
        mod_v[4] = scale
        mod_v[6] = gate * scale
        mod_v[7] = gate * shift
        mod_v[8] = wr_row * scale
        mod_v[9] = jnp.broadcast_to(jnp.sum(wr_row * shift, axis=-1, keepdims=True), (8, D))

    def rows_of(j, n):
        return _tile8(mod_v[j], n // 8)

    def h_term(t, i, r0=0, n=TH):
        return (t, i // 2, pl.ds(r0, n), pl.ds((i % 2) * DHALF, DHALF))

    def store_h_terms(t, r0, n, a, b):
        h1 = a * rows_of(1, n) + rows_of(0, n)
        h2 = b * rows_of(1, n) + rows_of(0, n)
        terms = _rhs_terms(h1[:, :DHALF], h2[:, :DHALF], h1[:, DHALF:], h2[:, DHALF:])
        for i, term in enumerate(terms):
            hc_v[h_term(t, i, r0, n)] = term.astype(BF)

    def ln1_piece(t, r0):
        store_h_terms(t, r0, R1, normalized(t * T + r0, R1, order1), normalized(t * T + TH + r0, R1, order1))

    def store_lhs_terms(top, bot, dst, c, r0):
        terms = _lhs_terms(top[:, :DHALF], top[:, DHALF:], bot[:, :DHALF], bot[:, DHALF:])
        for i, term in enumerate(terms):
            if dst.dtype == I32:
                dst[c, i] = _pack(term)
            else:
                dst[c, i, pl.ds(r0, 128), :] = term.astype(BF)

    def keep_weights(c, r0, halves):
        if c < EARLY:
            for g in range(2):
                x1_v[pl.ds(T + c * 512 + g * 256 + r0, 128), :] = halves[g]

    def early_bias(r0, n):
        b = jnp.sum(x1_v[pl.ds(T + r0, n), :] * rows_of(0, n), axis=-1, keepdims=True)
        bias_v[pl.ds(r0, n), :] = jnp.broadcast_to(b, (n, 128))

    def first_tile_terms(r0):
        store_h_terms(0, r0, 32, x1_v[pl.ds(r0, 32), :], x1_v[pl.ds(TH + r0, 32), :])

    def fold(j, c, dst):
        halves = []
        for g in range(2):
            w = wqkv_v[j * NCH + c, :, g * 128:(g + 1) * 128]
            gg = 2 * c + g
            halves.append(_dot(bdt[:, gg * 128:(gg + 1) * 128], w, NT) * LOG2E)
        store_lhs_terms(halves[0], halves[1], dst, c, 0)
        if j == 1:
            keep_weights(c, 0, halves)

    def prep_v(c):
        halves = [wqkv_v[2 * NCH + c, :, g * 128:(g + 1) * 128].T.astype(F32) for g in range(2)]
        store_lhs_terms(halves[0], halves[1], wkv_c, c, 128)
        keep_weights(c, 128, halves)

    def prep_wo(c, r0):
        def rows(r):
            w = wo_v[pl.ds(r, 16), :].astype(F32)
            return jnp.concatenate([order4.after(w[:, l:l + 128]) for l in range(0, D, 128)], axis=1)
        top, bot = rows(c * 256 + r0), wo_v[pl.ds(c * 256 + 128 + r0, 16), :].astype(F32)
        terms = _rhs_terms(top[:, :DHALF], top[:, DHALF:], bot[:, :DHALF], bot[:, DHALF:])
        for i, term in enumerate(terms):
            wo_c[i, pl.ds(c * 64 + r0 // 2, 8), :] = _pack(term)
        order4.link = jnp.broadcast_to(jnp.max(terms[0][:, 0:128], axis=-1, keepdims=True), (16, 128))

    def kv_pair(t, c, res, k):
        g, q = divmod(k, 2)
        pair = 4 * c + k

        def rows(r0):
            val = res[g][r0:r0 + 64]
            if t == 0 and c < EARLY:
                val = val + jnp.concatenate([bias_v[pl.ds(c * 512 + g * 256 + r0, 64), :]] * (T // 128), axis=1)
            return val

        phi = _hedgehog(rows(q * 64))
        vt = rows(128 + q * 64).astype(BF)
        zs = phi[:, 0:128]
        for l in range(1, T // 128):
            zs = zs + phi[:, l * 128:(l + 1) * 128]
        kv = _dot(vt, phi.astype(BF), NT)
        if t > 0:
            zs = zs + z_acc[pair]
            kv = kv + kv_acc[pair]
        if t < NTILE - 1:
            z_acc[pair] = zs
            kv_acc[pair] = kv
        else:
            z = jnp.broadcast_to(jnp.sum(zs.T, axis=0, keepdims=True), (16, 128))
            row = lax.broadcasted_iota(I32, (80, 128), 0)
            lane = lax.broadcasted_iota(I32, (80, 128), 1)
            head = jnp.where(row < 64, row // DH, (row - 64) // 8)
            kvT[pair] = jnp.where(head == lane % 2, jnp.concatenate([kv, z], axis=0), 0.0).astype(BF)

    def q_pair(c, res, k):
        g, q = divmod(k, 2)
        pair = 4 * c + k
        even = (lax.broadcasted_iota(I32, (8, T), 0) % 2) == 0
        phi, scale = _hedgehog_scaled(res[g][q * 64:(q + 1) * 64])
        nd = _dot(kvT[pair], phi.astype(BF), NN)
        swapped = pltpu.roll(scale, 1, 0)
        inv_a = _recip(nd[64:72] + 1e-6 * jnp.where(even, scale, swapped))
        inv_b = _recip(nd[72:80] + 1e-6 * jnp.where(even, swapped, scale))
        return nd[0:64] * jnp.concatenate([inv_a] * 4 + [inv_b] * 4, axis=0)

    held = {}

    def q_step(t, c, res, k):
        held[k] = q_pair(c, res, k)
        if k == 3:
            held["lower"] = jnp.concatenate([held.pop(2), held.pop(3)], axis=0).T
        if k == 1:
            o1, o2 = jnp.concatenate([held.pop(0), held.pop(1)], axis=0).T, held.pop("lower")
            for i, term in enumerate(_lhs_terms(o1[:TH], o2[:TH], o1[TH:], o2[TH:])):
                oc_v[t, i, :, pl.ds(c * 128, 128)] = term.astype(BF)

    def residual(tok, attn):
        rows = pl.ds(tok, 128)
        x1_v[rows, :] = x_v[rows, :].astype(F32) + rows_of(2, 128) * attn

    def block_out(x1, xc, rs):
        n = x1.shape[0]
        return xc * (rs * rows_of(6, n)) + (x1 + rows_of(7, n))

    def router(xc, rs):
        n = xc.shape[0]
        return jnp.sum(xc * rows_of(8, n), axis=-1, keepdims=True) * rs + rows_of(9, n)[:, 0:1]

    neg = jnp.full((8, 128), -jnp.inf, F32)
    top = [neg, neg, jnp.zeros((8, 128), F32), jnp.zeros((8, 128), F32)]

    def ln2_piece(tok, order):
        x1 = x1_v[pl.ds(tok, R2), :]
        xc, rs = _center(x1, order)
        t, r0 = divmod(tok, T)
        hc_v[t, r0 // TH, pl.ds(r0 % TH, R2), :] = block_out(x1, xc, rs).astype(BF)
        r = router(xc, rs)
        sub = lax.broadcasted_iota(I32, (8, 128), 0).astype(F32)
        m1, m2, i1, i2 = top
        for g in range(R2 // 8):
            rg = jnp.broadcast_to(r[g * 8:(g + 1) * 8], (8, 128))
            ig = sub + float(tok + g * 8)
            gt1 = (rg > m1) | ((rg == m1) & (ig < i1))
            gt2 = (rg > m2) | ((rg == m2) & (ig < i2))
            m2 = jnp.where(gt1, m1, jnp.where(gt2, rg, m2))
            i2 = jnp.where(gt1, i1, jnp.where(gt2, ig, i2))
            m1 = jnp.where(gt1, rg, m1)
            i1 = jnp.where(gt1, ig, i1)
        top[:] = m1, m2, i1, i2

    def out_copy(t, half):
        return pltpu.make_async_copy(hc_v.at[t, half], out_hbm.at[pl.ds(t * T + half * TH, TH)],
                                     osems.at[2 * t + half])

    def start_out(t):
        for half in range(2):
            out_copy(t, half).start()
        started.append(t)

    wait("wk0", "wv0")
    fold(1, 0, wkv_c)
    prep_v(0)
    scale = 1.0
    for k in range(NCA):
        wait("ca%d" % k)
        n = D // NCA
        scale = scale + _dot(sc[:, k * n:(k + 1) * n], wmod_v[1, pl.ds(k * n, n), pl.ds(0, D)], NN)[0:8]
    mod_v[1] = scale

    def scaled(half, d):
        cols = slice(d * DHALF, (d + 1) * DHALF)
        return lambda r0: x1_v[pl.ds(half * TH + r0, 64), cols] * _tile8(scale[:, cols], 8)

    b11, b12, b21, b22 = scaled(0, 0), scaled(1, 0), scaled(0, 1), scaled(1, 1)
    for group in cfg.get("tg", ((0,), (1, 2, 3, 4, 5, 6))):
        for r0 in range(0, TH, 64):
            terms = _rhs_terms(b11(r0), b12(r0), b21(r0), b22(r0))
            for i in group:
                hc_v[h_term(NTILE, i, r0, 64)] = terms[i].astype(BF)

    P = functools.partial

    def spread(slots, lo, hi, works):
        for n, work in enumerate(works):
            slots[lo + n * (hi - lo) // len(works)].append(work)

    steps = [("kv", t, c) for t in range(NTILE) for c in range(NCH)]
    steps += [("q", t, c) for t in range(NTILE) for c in range(NCH)]
    steps += [("o", t, s) for t in range(NTILE) for s in range(2)]
    if cfg.get("only"):
        steps = [steps[i] for i in cfg["only"]]
    mod_parts = [P(mod_part, j, n, half) for j in range(2, 6) for half in range(2) for n in range(8)]
    prev = None
    for step, (kind, t, c) in enumerate(steps):
        slots = [[] for _ in range(7)]
        lower_done = None
        if prev is not None:
            pkind, pt, pc, pres = prev
            if pkind == "kv":
                works = [P(kv_pair, pt, pc, pres, k) for k in (2, 3, 0, 1)]
                if (pt, pc) == (0, 0):
                    late, works = works[:2], works[2:]
                    delayed = works
                elif (pt, pc) == (0, 1):
                    for slot, work in enumerate(delayed + works):
                        slots[slot].append(work)
                else:
                    for slot, work in zip(cfg.get("ks", (0, 1, 2, 3)), works):
                        slots[slot].append(work)
            elif pkind == "q":
                qs = cfg.get("qs", (0, 1, 3, 5))
                for slot, k in zip(qs, (2, 3, 0, 1)):
                    slots[slot].append(P(q_step, pt, pc, pres, k))
            else:
                tok = pt * T + pc * 128
                slots[0].append(P(residual, tok, pres[0]))
                lo, hi = cfg.get("l2a", (0, 4))
                group = _Order(never) if cfg.get("groups", 1) == 1 else order2
                spread(slots, lo, hi, [P(ln2_piece, tok + r0, group) for r0 in range(0, 128, R2)])
                if pc == 1:
                    slots[hi].append(P(start_out, pt))
        if kind == "kv":
            if t == 0:
                if c == 0:
                    slots[cfg.get("w1", 2)] += [P(wait, "wk1", "wv1"), P(prep_v, 1), P(fold, 1, 1, wkv_c)]
                if c == 1:
                    sa = cfg.get("sa", 2)
                    slots[sa] += [P(wait, "sa", "wk2", "wv2"), lambda: mod_v.__setitem__(0, mod_row(0)),
                                  P(prep_v, 2), P(fold, 1, 2, wkv_c)]
                    slots[sa] += [P(first_tile_terms, r0) for r0 in range(0, TH, 32)]
                    slots[sa] += [P(early_bias, r0, 32) for r0 in range(0, 512 * EARLY, 32)]
                    slots[5].append(late[0])
                    slots[6].append(late[1])
                if c == 2:
                    w3 = cfg.get("w3", 3)
                    slots[w3] = [P(wait, "x1", "wk3", "wv3"), P(prep_v, 3), P(fold, 1, 3, wkv_c)] + slots[w3]
            if (t, c) == (1, 0):
                slots[0].insert(0, P(wait, "x2", "x3", "wq0", "wq1", "wq2", "wq3"))
            if t + 1 < NTILE:
                chunks = ((3,), (0, 1, 2, 3), (0, 1, 2, 3))[t]
                if c in chunks:
                    pieces = list(range(0, TH, R1))
                    k = chunks.index(c)
                    mine = pieces[k * len(pieces) // len(chunks):(k + 1) * len(pieces) // len(chunks)]
                    spread(slots, 0, 6, [P(ln1_piece, t + 1, r0) for r0 in mine])
            if t == cfg.get("foldq", 2):
                slots[5].append(P(fold, 0, c, wq_c))
            if t == 3:
                if c == 0:
                    slots[0].insert(0, P(wait, "wr", "wo", "ga", "sb", "cb", "gb"))
                spread(slots, 1, 7, [P(prep_wo, c, r0) for r0 in range(0, 128, 16)])
                if cfg.get("vmod"):
                    nk = cfg["vmod"]
                    spread(slots, 1, 7, [P(mod_piece, 2 + c, k0, nk) for k0 in range(0, D, nk)])
                else:
                    slots[5].append(lambda j=2 + c: mod_v.__setitem__(j, mod_row(j)))
        if cfg.get("modparts") and mod_parts and (kind, t) >= ("kv", 3) and kind != "o":
            for k in range(1 if (kind, t, c) == ("kv", 3, 0) else 0, 7):
                if mod_parts:
                    slots[k].insert(0, mod_parts.pop(0))
        if (kind, t, c) == ("q", 0, 0):
            slots[0].insert(0, P(wait, "wg"))
            slots[6].append(finish_mod)
        if kind == "o":
            last = step == len(steps) - 1
            tok2 = t * T + TH + c * 128
            lower_done = P(residual, tok2)
            lo, hi = (5, 6) if last else cfg.get("l2b", (5, 7))
            group = _Order(never) if cfg.get("groups", 1) == 1 else order4
            spread(slots, lo, hi, [P(ln2_piece, tok2 + r0, None if last else group) for r0 in range(0, 128, R2)])

        def fill(k, m, slots=slots):
            if cfg.get("tie", True):
                order1.release = order2.release = m
            for work in slots[k]:
                work()

        if kind == "kv":
            slot = NTILE if t == 0 and c < EARLY else t
            res = _block_product(lambda i: _dot(wkv_c[c, i], hc_v[h_term(slot, i)], NT), fill)
        elif kind == "q":
            res = _block_product(lambda i: _dot(_unpack(wq_c[c, i]), hc_v[h_term(t, i)], NT), fill)
        else:
            res = _block_product(
                lambda i: _dot(oc_v[t, i, pl.ds(c * 128, 128), :], _unpack(wo_c[i]), NN), fill, lower_done)
        if kind == "kv" and c == NCH - 1:
            order1.link = None
        prev = (kind, t, c, res)

    if cfg.get("only"):
        for name in copies:
            if name not in waited:
                wait(name)
        a, b = prev[3]
        x1_v[0:128, 0:256] = a[0:128, 0:256] + b[0:128, 0:256] + a[0:128, 256:512] + b[0:128, 256:512]
        x1_v[128:136, 0:128] = top[0] + top[1] + top[2] + top[3]
        z = pl.semaphore_read(idle_sem)
        x1_v[136:144, :] = mod_v[z]
        x1_v[144:160, 0:512] = oc_v[z, z, 0:16, :].astype(F32) + hc_v[z, z, 0:16, 0:512].astype(F32) + (
            wo_c[z, 0:16, :] + wq_c[z, z, 0:16, :] + wkv_c[z, z, 0:16, :]).astype(F32)
        x1_v[160:176, 0:128] = kvT[z, 0:16, :].astype(F32) + kv_acc[z, 0:16, :] + z_acc[z, 0:16, :]
        slab_v[0] = x1_v[pl.ds(pl.multiple_of(z * 16, 16), 16), :].astype(BF)
        cpy = pltpu.make_async_copy(slab_v.at[0], out_hbm.at[pl.ds(0, 16)], osems.at[0])
        cpy.start()
        cpy.wait()
        for t in started:
            out_copy(t, 0).wait()
            out_copy(t, 1).wait()
        return

    _, pt, pc, pres = prev
    tok = pt * T + pc * 128
    residual(tok, pres[0])
    for r0 in range(0, 128, R2):
        ln2_piece(tok + r0, None)
    start_out(pt)

    m1, m2, i1, i2 = top
    big = float(2 * S)
    best = jnp.max(m1, axis=0, keepdims=True)
    ia = jnp.min(jnp.where(m1 == best, i1, big), axis=0, keepdims=True)
    taken = i1 == ia
    cm = jnp.where(taken, m2, m1)
    ci = jnp.where(taken, i2, i1)
    second = jnp.max(cm, axis=0, keepdims=True)
    ib = jnp.min(jnp.where(cm == second, ci, big), axis=0, keepdims=True)
    idx_a = jnp.clip(ia.astype(I32)[0, 0], 0, S - 1)
    idx_b = jnp.clip(ib.astype(I32)[0, 0], 0, S - 1)

    sub = lax.broadcasted_iota(I32, (16, D), 0)
    xa = jnp.broadcast_to(x1_v[pl.ds(idx_a, 1), :], (16, D))
    xb = jnp.broadcast_to(x1_v[pl.ds(idx_b, 1), :], (16, D))
    xc, rs = _center(jnp.where(sub == 0, xa, xb))
    gate_r = jax.nn.sigmoid(router(xc, rs))
    hb = (xc * rs * rows_of(4, 16) + rows_of(3, 16)).astype(BF)
    wait("wu", "wd")
    g = _dot(hb, wg_v[...], NN)
    u = _dot(hb, wu_v[...], NN)
    act = (g * jax.nn.sigmoid(g) * u).astype(BF)
    y = _dot(act, wd_v[:, pl.ds(0, D)], NN) * gate_r * rows_of(5, 16)

    for t in range(NTILE):
        out_copy(t, 0).wait()
        out_copy(t, 1).wait()

    def fix(idx, slot):
        start = pl.multiple_of((idx // 16) * 16, 16)
        x1 = x1_v[pl.ds(start, 16), :]
        o = block_out(x1, *_center(x1))
        o = o + jnp.where(sub + start == idx_a, y[0:1], 0.0) + jnp.where(sub + start == idx_b, y[1:2], 0.0)
        slab_v[slot] = o.astype(BF)
        return pltpu.make_async_copy(slab_v.at[slot], out_hbm.at[pl.ds(start, 16)], osems.at[slot])

    fa = fix(idx_a, 0)
    fb = fix(idx_b, 1)
    fa.start()

    @pl.when(idx_a // 16 != idx_b // 16)
    def _():
        fb.start()
        fb.wait()

    fa.wait()
    mark(None)


def make(flags=None, **cfg):
    cfg = dict(dict(tie=False, vmod=32, chain3=1, w1=2, sa=3, w3=1), **cfg)
    if cfg.get("ev", True):
        flags = dict(flags or {}, XLA_TPU_EVENLY_DISTRIBUTE_CRITICAL_NODES=True)
    pad = cfg.get("pad", 128)

    def run(A_x, A_wqkv, A_w_phi, A_wo, B_x, B_w_r, B_w_gate, B_w_up, B_w_down, c, w_mod):
        del B_x
        any_spec = pl.BlockSpec(memory_space=pl.ANY)
        scratch = [
            pltpu.VMEM((S, D), BF), pltpu.VMEM((3 * NCH, D, 256), BF), pltpu.VMEM((H, DH, DH), BF),
            pltpu.VMEM((D, D), BF), pltpu.VMEM((8, 128), BF),
            pltpu.VMEM((D, F), BF), pltpu.VMEM((D, F), BF), pltpu.VMEM((F, D + pad), BF),
            pltpu.VMEM((1, D), BF), pltpu.VMEM((6, D, D + pad), BF),
            pltpu.VMEM((NCH, 7, 256, DHALF), BF), pltpu.VMEM((NCH, 7, 64, DHALF), I32),
            pltpu.VMEM((7, DHALF // 2, DHALF), I32),
            pltpu.VMEM((NTILE + 1, 4, TH, D), BF), pltpu.VMEM((NTILE, 7, TH, DHALF), BF), pltpu.VMEM((S, D), F32),
            pltpu.VMEM((H // 2, 64, 128), F32), pltpu.VMEM((H // 2, 128, 128), F32),
            pltpu.VMEM((H // 2, 80, 128), BF),
            pltpu.VMEM((10, 8, D), F32), pltpu.VMEM((D, 128), F32), pltpu.VMEM((512 * EARLY, 128), F32), pltpu.VMEM((2, 16, D), BF), pltpu.SemaphoreType.REGULAR,
            pltpu.SemaphoreType.DMA((40,)), pltpu.SemaphoreType.DMA((2 * NTILE,)),
        ]
        out = pl.pallas_call(
            functools.partial(_kernel, cfg=cfg),
            out_shape=jax.ShapeDtypeStruct((S, D), BF),
            in_specs=[any_spec] * 10,
            out_specs=any_spec,
            scratch_shapes=scratch,
            compiler_params=pltpu.CompilerParams(vmem_limit_bytes=120 * 2**20, flags=flags),
            name="fused_block",
        )(A_x.reshape(S, D), A_wqkv, A_w_phi, A_wo, B_w_r.reshape(8, 128), B_w_gate, B_w_up, B_w_down, c, w_mod)
        return out.reshape(1, S, D)
    return run


_run = make(**dict())


@jax.jit
def pallas_adaLN_cond__linear_kernel_hedgehog__moe_arch_mod__prompt_kernel(
    A_x: jax.Array,
    A_wqkv: jax.Array,
    A_w_phi: jax.Array,
    A_wo: jax.Array,
    B_x: jax.Array,
    B_w_r: jax.Array,
    B_w_gate: jax.Array,
    B_w_up: jax.Array,
    B_w_down: jax.Array,
    c: jax.Array,
    w_mod: jax.Array,
):
    return _run(A_x, A_wqkv, A_w_phi, A_wo, B_x, B_w_r, B_w_gate, B_w_up, B_w_down, c, w_mod)
```

```python
import functools

import jax
import jax.numpy as jnp
from jax import lax
from jax.experimental import pallas as pl
from jax.experimental.pallas import tpu as pltpu

S, D, H, DH, F = 2048, 1024, 32, 32, 3584
T = 512
TH = T // 2
DHALF = D // 2
NTILE = S // T
NCH = D // 256
EARLY = 2
LOG2E = 1.4426950408889634
NN = (((1,), (0,)), ((), ()))
NT = (((1,), (1,)), ((), ()))
TN = (((0,), (0,)), ((), ()))
BF = jnp.bfloat16
F32 = jnp.float32
I32 = jnp.int32


def _dot(a, b, dims):
    return lax.dot_general(a, b, dims, preferred_element_type=F32)


def _recip(x):
    return pltpu.reciprocal(x, approx=False, full_range=False)


def _center(x, order=None):
    s = jnp.sum(x, axis=-1, keepdims=True)
    if order is not None:
        s = order.after(s)
    xc = x - s * (1.0 / D)
    rs = lax.rsqrt(jnp.sum(xc * xc, axis=-1, keepdims=True) * (1.0 / D) + 1e-5)
    if order is not None:
        order.link = rs
    return xc, rs


def _pair_reduce(x, op):
    r = x[0:8]
    for i in range(1, 8):
        r = op(r, x[8 * i:8 * i + 8])
    r = op(r, pltpu.roll(r, 4, 0))
    return op(r, pltpu.roll(r, 2, 0))


def _tile8(r, n):
    return jnp.concatenate([r] * n, axis=0)


def _hedgehog(p):
    mx = _tile8(_pair_reduce(p, jnp.maximum), 8)
    mn = _tile8(_pair_reduce(p, jnp.minimum), 8)
    ep = jnp.exp2(p - mx)
    en = jnp.exp2(mn - p)
    rp = _tile8(_recip(_pair_reduce(ep, jnp.add)), 8)
    rn = _tile8(_recip(_pair_reduce(en, jnp.add)), 8)
    return jnp.concatenate([ep * rp, en * rn], axis=0)


def _hedgehog_scaled(p):
    mx = _tile8(_pair_reduce(p, jnp.maximum), 8)
    mn = _tile8(_pair_reduce(p, jnp.minimum), 8)
    ep = jnp.exp2(p - mx)
    en = jnp.exp2(mn - p)
    sp = _pair_reduce(ep, jnp.add)
    ratio = _tile8(sp * _recip(_pair_reduce(en, jnp.add)), 8)
    return jnp.concatenate([ep, en * ratio], axis=0), sp


def _lhs_terms(a11, a12, a21, a22):
    return (a11 + a22, a21 + a22, a11, a22, a11 + a12, a21 - a11, a12 - a22)


def _rhs_terms(b11, b12, b21, b22):
    return (b11 + b22, b11, b12 - b22, b21 - b11, b22, b11 + b12, b21 + b22)


def _block_product(product, fill, lower_done=None):
    m0 = product(0)
    fill(0, m0)
    m1 = product(1)
    fill(1, m1)
    c22 = m0 - m1
    m3 = product(3)
    fill(2, m3)
    c21 = m1 + m3
    c11 = m0 + m3
    m2 = product(2)
    fill(3, m2)
    c22 = c22 + m2
    m5 = product(5)
    fill(4, m5)
    lower = jnp.concatenate([c21, c22 + m5], axis=1)
    if lower_done is not None:
        lower_done(lower)
    m4 = product(4)
    fill(5, m4)
    c12 = m2 + m4
    c11 = c11 - m4
    m6 = product(6)
    fill(6, m6)
    return jnp.concatenate([c11 + m6, c12], axis=1), lower


def _pack(x):
    return pltpu.bitcast(x.astype(BF), I32)


def _unpack(x):
    return pltpu.bitcast(x, BF)


class _Order:
    def __init__(self, never):
        self.never = never
        self.link = None
        self.release = None

    def after(self, v):
        for dep in (self.link, self.release):
            if dep is not None:
                probe = self.never[:v.shape[0], :v.shape[1]]
                v = jnp.where(probe != probe, dep[:v.shape[0], :v.shape[1]], v)
        return v


def _kernel(x_hbm, wqkv_hbm, wphi_hbm, wo_hbm, wr_hbm, wg_hbm, wu_hbm, wd_hbm, c_hbm, wmod_hbm,
            out_hbm,
            x_v, wqkv_v, wphi_v, wo_v, wr_v, wg_v, wu_v, wd_v, c_v, wmod_v,
            wkv_c, wq_c, wo_c, hc_v, oc_v, x1_v, kv_acc, z_acc, kvT, mod_v, sb_v, bias_v, slab_v, idle_sem,
            sems, osems, *, cfg):
    R1, R2 = cfg.get("R1", 16), cfg.get("R2", 16)
    NCA = cfg.get("nca", 4)

    def col(ref, j, w=D):
        return ref.at[:, pl.ds(j * w, w)]

    def x_copy(t):
        return ("x%d" % t, x_hbm.at[pl.ds(t * T, T)], x_v.at[pl.ds(t * T, T)])

    def w_copy(name, j, c):
        return ("%s%d" % (name, c), col(wqkv_hbm, j * NCH + c, 256), wqkv_v.at[j * NCH + c])

    def mod_copy(name, j):
        return (name, col(wmod_hbm, j), wmod_v.at[j, :, pl.ds(0, D)])

    def scale_copy(k):
        rows = pl.ds(k * (D // NCA), D // NCA)
        return ("ca%d" % k, wmod_hbm.at[rows, pl.ds(D, D)], wmod_v.at[1, rows, pl.ds(0, D)])

    order = [("c", c_hbm, c_v), x_copy(0), ("wphi", wphi_hbm, wphi_v),
             w_copy("wk", 1, 0), w_copy("wv", 2, 0), *[scale_copy(k) for k in range(NCA)],
             w_copy("wk", 1, 1), w_copy("wv", 2, 1), mod_copy("sa", 0),
             w_copy("wk", 1, 2), w_copy("wv", 2, 2), x_copy(1), w_copy("wk", 1, 3), w_copy("wv", 2, 3),
             x_copy(2), x_copy(3)]
    order += [w_copy("wq", 0, c) for c in range(NCH)]
    order += [("wr", wr_hbm, wr_v), ("wo", wo_hbm, wo_v), mod_copy("ga", 2), mod_copy("sb", 3), mod_copy("cb", 4), mod_copy("gb", 5),
              ("wg", wg_hbm, wg_v), ("wu", wu_hbm, wu_v), ("wd", wd_hbm, wd_v.at[:, pl.ds(0, D)])]
    copies = {}
    for i, (name, src, dst) in enumerate(order):
        copies[name] = pltpu.make_async_copy(src, dst, sems.at[i])
        copies[name].start()

    waited, started = set(), []

    scope = []

    def mark(name):
        if cfg.get("marks"):
            if scope:
                scope.pop().__exit__(None, None, None)
            if name:
                scope.append(jax.named_scope(name))
                scope[0].__enter__()

    def wait(*names):
        mark("w_" + names[0])
        for name in names:
            copies[name].wait()
            waited.add(name)
        mark("r_" + names[0])


    wait("c", "x0")
    cf = c_v[...].astype(F32)
    never = jnp.broadcast_to(cf[:, 0:128], (32, 128))
    order1, order2, order3, order4 = [_Order(never) for _ in range(4)]
    sc = jnp.broadcast_to(cf * jax.nn.sigmoid(cf), (16, D)).astype(BF)

    def normalized(tok, n, order=None):
        xc, rs = _center(x_v[pl.ds(tok, n), :].astype(F32), order)
        return xc * rs

    for r0 in range(0, T, 32):
        x1_v[pl.ds(r0, 32), :] = normalized(r0, 32)

    wait("wphi")
    row = lax.broadcasted_iota(I32, (128, DH), 0)
    lane = lax.broadcasted_iota(I32, (128, DH), 1)
    expand = jnp.where(((row % 64) // 2) == lane, 1.0, 0.0).astype(BF)
    bdt = _dot(expand, wphi_v[...].reshape(H * DH, DH), NT)
    row = lax.broadcasted_iota(I32, (128, D), 0)
    lane = lax.broadcasted_iota(I32, (128, D), 1)
    bdt = jnp.where(2 * (row // 64) + (row % 2) == (lane % 128) // DH, bdt, 0.0).astype(BF)

    def mod_row(j):
        return _dot(sc, wmod_v[j, :, pl.ds(0, D)], NN)[0:8]

    def mod_part(j, n, half):
        part = _dot(sc[:, half * DHALF:(half + 1) * DHALF],
                    wmod_v[j, pl.ds(half * DHALF, DHALF), pl.ds(n * 128, 128)], NN)[0:8]
        if half == 0:
            mod_v[j, :, pl.ds(n * 128, 128)] = part
        else:
            mod_v[j, :, pl.ds(n * 128, 128)] += part

    for k0 in range(0, D, 128):
        sb_v[pl.ds(k0, 128), :] = jnp.broadcast_to(sc[0:1, k0:k0 + 128].astype(F32), (128, 128)).T

    partial_mod = {}

    def mod_piece(j, k0, nk):
        acc = partial_mod.pop(j, None)
        step = cfg.get("mstep", 16)
        for k in range(k0, k0 + nk, step):
            s_col = sb_v[pl.ds(k, step), :]
            if k == k0 and cfg.get("chain3"):
                s_col = order3.after(s_col)
            term = wmod_v[j, pl.ds(k, step), pl.ds(0, D)].astype(F32) * jnp.concatenate([s_col] * (D // 128), axis=1)
            if step == 16:
                term = term[0:8] + term[8:16]
            acc = term if acc is None else acc + term
        if cfg.get("chain3"):
            link = acc[:, 0:128]
            for _ in range(cfg["chain3"]):
                link = jnp.broadcast_to(jnp.max(link, axis=-1, keepdims=True), (8, 128))
            order3.link = jnp.concatenate([link, link], axis=0)
        if k0 + nk < D:
            partial_mod[j] = acc
        else:
            mod_v[j] = jnp.broadcast_to(jnp.sum(acc, axis=0, keepdims=True), (8, D))

    def finish_mod():
        wr = wr_v[...].astype(F32)
        wr_row = jnp.concatenate([jnp.broadcast_to(wr[j:j + 1, :], (8, 128)) for j in range(8)], axis=1)
        shift, scale, gate = mod_v[3], 1.0 + mod_v[4], mod_v[5]
        mod_v[4] = scale
        mod_v[6] = gate * scale
        mod_v[7] = gate * shift
        mod_v[8] = wr_row * scale
        mod_v[9] = jnp.broadcast_to(jnp.sum(wr_row * shift, axis=-1, keepdims=True), (8, D))

    def rows_of(j, n):
        return _tile8(mod_v[j], n // 8)

    def h_term(t, i, r0=0, n=TH):
        return (t, i // 2, pl.ds(r0, n), pl.ds((i % 2) * DHALF, DHALF))

    def store_h_terms(t, r0, n, a, b):
        h1 = a * rows_of(1, n) + rows_of(0, n)
        h2 = b * rows_of(1, n) + rows_of(0, n)
        terms = _rhs_terms(h1[:, :DHALF], h2[:, :DHALF], h1[:, DHALF:], h2[:, DHALF:])
        for i, term in enumerate(terms):
            hc_v[h_term(t, i, r0, n)] = term.astype(BF)

    def ln1_piece(t, r0):
        second = order4 if t == 1 else order1
        store_h_terms(t, r0, R1, normalized(t * T + r0, R1, order1), normalized(t * T + TH + r0, R1, second))

    def store_lhs_terms(top, bot, dst, c, r0):
        terms = _lhs_terms(top[:, :DHALF], top[:, DHALF:], bot[:, :DHALF], bot[:, DHALF:])
        for i, term in enumerate(terms):
            if dst.dtype == I32:
                dst[c, i] = _pack(term)
            else:
                dst[c, i, pl.ds(r0, 128), :] = term.astype(BF)

    def keep_weights(c, r0, halves):
        if c < EARLY:
            for g in range(2):
                x1_v[pl.ds(T + c * 512 + g * 256 + r0, 128), :] = halves[g]

    def early_bias(r0, n):
        b = jnp.sum(x1_v[pl.ds(T + r0, n), :] * rows_of(0, n), axis=-1, keepdims=True)
        bias_v[pl.ds(r0, n), :] = jnp.broadcast_to(b, (n, 128))

    def first_tile_terms(r0):
        store_h_terms(0, r0, 32, x1_v[pl.ds(r0, 32), :], x1_v[pl.ds(TH + r0, 32), :])

    def fold(j, c, dst):
        halves = []
        for g in range(2):
            w = wqkv_v[j * NCH + c, :, g * 128:(g + 1) * 128]
            gg = 2 * c + g
            halves.append(_dot(bdt[:, gg * 128:(gg + 1) * 128], w, NT) * LOG2E)
        store_lhs_terms(halves[0], halves[1], dst, c, 0)
        if j == 1:
            keep_weights(c, 0, halves)

    def prep_v(c):
        halves = [wqkv_v[2 * NCH + c, :, g * 128:(g + 1) * 128].T.astype(F32) for g in range(2)]
        store_lhs_terms(halves[0], halves[1], wkv_c, c, 128)
        keep_weights(c, 128, halves)

    def prep_wo(c, r0):
        def rows(r):
            w = wo_v[pl.ds(r, 16), :].astype(F32)
            return jnp.concatenate([order3.after(w[:, l:l + 128]) for l in range(0, D, 128)], axis=1)
        top, bot = rows(c * 256 + r0), wo_v[pl.ds(c * 256 + 128 + r0, 16), :].astype(F32)
        terms = _rhs_terms(top[:, :DHALF], top[:, DHALF:], bot[:, :DHALF], bot[:, DHALF:])
        for i, term in enumerate(terms):
            wo_c[i, pl.ds(c * 64 + r0 // 2, 8), :] = _pack(term)
        order3.link = jnp.broadcast_to(jnp.max(terms[0][:, 0:128], axis=-1, keepdims=True), (16, 128))

    stream = _Order(never)

    def behind_product(v):
        head = jnp.concatenate([stream.after(v[0:8, l:l + 128]) for l in range(0, T, 128)], axis=1)
        return jnp.concatenate([head, v[8:]], axis=0)

    def kv_pair(t, c, res, k):
        g, q = divmod(k, 2)
        pair = 4 * c + k

        def rows(r0):
            val = res[g][r0:r0 + 64]
            if t == 0 and c < EARLY:
                val = val + jnp.concatenate([bias_v[pl.ds(c * 512 + g * 256 + r0, 64), :]] * (T // 128), axis=1)
            return val

        phi = _hedgehog(rows(q * 64))
        vt = behind_product(rows(128 + q * 64)).astype(BF)
        zs = phi[:, 0:128]
        for l in range(1, T // 128):
            zs = zs + phi[:, l * 128:(l + 1) * 128]
        kv = _dot(vt, phi.astype(BF), NT)
        if t > 0:
            zs = zs + z_acc[pair]
            kv = kv + kv_acc[pair]
        if t < NTILE - 1:
            z_acc[pair] = zs
            kv_acc[pair] = kv
        else:
            z = jnp.broadcast_to(jnp.sum(zs.T, axis=0, keepdims=True), (16, 128))
            row = lax.broadcasted_iota(I32, (80, 128), 0)
            lane = lax.broadcasted_iota(I32, (80, 128), 1)
            head = jnp.where(row < 64, row // DH, (row - 64) // 8)
            kvT[pair] = jnp.where(head == lane % 2, jnp.concatenate([kv, z], axis=0), 0.0).astype(BF)

    def q_pair(c, res, k):
        g, q = divmod(k, 2)
        pair = 4 * c + k
        even = (lax.broadcasted_iota(I32, (8, T), 0) % 2) == 0
        phi, scale = _hedgehog_scaled(res[g][q * 64:(q + 1) * 64])
        if cfg.get("tq"):
            phi = behind_product(phi)
        nd = _dot(kvT[pair], phi.astype(BF), NN)
        swapped = pltpu.roll(scale, 1, 0)
        inv_a = _recip(nd[64:72] + 1e-6 * jnp.where(even, scale, swapped))
        inv_b = _recip(nd[72:80] + 1e-6 * jnp.where(even, swapped, scale))
        return nd[0:64] * jnp.concatenate([inv_a] * 4 + [inv_b] * 4, axis=0)

    held = {}

    def q_step(t, c, res, k):
        held[k] = q_pair(c, res, k)
        if k == 3:
            held["lower"] = jnp.concatenate([held.pop(2), held.pop(3)], axis=0).T
        if k == 1:
            o1, o2 = jnp.concatenate([held.pop(0), held.pop(1)], axis=0).T, held.pop("lower")
            for i, term in enumerate(_lhs_terms(o1[:TH], o2[:TH], o1[TH:], o2[TH:])):
                oc_v[t, i, :, pl.ds(c * 128, 128)] = term.astype(BF)

    def residual(tok, attn):
        rows = pl.ds(tok, 128)
        x1_v[rows, :] = x_v[rows, :].astype(F32) + rows_of(2, 128) * attn

    def block_out(x1, xc, rs):
        n = x1.shape[0]
        return xc * (rs * rows_of(6, n)) + (x1 + rows_of(7, n))

    def router(xc, rs):
        n = xc.shape[0]
        return jnp.sum(xc * rows_of(8, n), axis=-1, keepdims=True) * rs + rows_of(9, n)[:, 0:1]

    neg = jnp.full((8, 128), -jnp.inf, F32)
    top = [neg, neg, jnp.zeros((8, 128), F32), jnp.zeros((8, 128), F32)]

    def ln2_piece(tok, order):
        x1 = x1_v[pl.ds(tok, R2), :]
        xc, rs = _center(x1, order)
        t, r0 = divmod(tok, T)
        hc_v[t, r0 // TH, pl.ds(r0 % TH, R2), :] = block_out(x1, xc, rs).astype(BF)
        r = router(xc, rs)
        sub = lax.broadcasted_iota(I32, (8, 128), 0).astype(F32)
        m1, m2, i1, i2 = top
        for g in range(R2 // 8):
            rg = jnp.broadcast_to(r[g * 8:(g + 1) * 8], (8, 128))
            ig = sub + float(tok + g * 8)
            gt1 = (rg > m1) | ((rg == m1) & (ig < i1))
            gt2 = (rg > m2) | ((rg == m2) & (ig < i2))
            m2 = jnp.where(gt1, m1, jnp.where(gt2, rg, m2))
            i2 = jnp.where(gt1, i1, jnp.where(gt2, ig, i2))
            m1 = jnp.where(gt1, rg, m1)
            i1 = jnp.where(gt1, ig, i1)
        top[:] = m1, m2, i1, i2

    def out_copy(t, half):
        return pltpu.make_async_copy(hc_v.at[t, half], out_hbm.at[pl.ds(t * T + half * TH, TH)],
                                     osems.at[2 * t + half])

    def start_out(t):
        for half in range(2):
            out_copy(t, half).start()
        started.append(t)

    wait("wk0", "wv0")
    fold(1, 0, wkv_c)
    prep_v(0)
    scale = 1.0
    for k in range(NCA):
        wait("ca%d" % k)
        n = D // NCA
        scale = scale + _dot(sc[:, k * n:(k + 1) * n], wmod_v[1, pl.ds(k * n, n), pl.ds(0, D)], NN)[0:8]
    mod_v[1] = scale

    def scaled(half, d):
        cols = slice(d * DHALF, (d + 1) * DHALF)
        return lambda r0: x1_v[pl.ds(half * TH + r0, 64), cols] * _tile8(scale[:, cols], 8)

    b11, b12, b21, b22 = scaled(0, 0), scaled(1, 0), scaled(0, 1), scaled(1, 1)
    for group in cfg.get("tg", ((0,), (1, 2, 3, 4, 5, 6))):
        for r0 in range(0, TH, 64):
            terms = _rhs_terms(b11(r0), b12(r0), b21(r0), b22(r0))
            for i in group:
                hc_v[h_term(NTILE, i, r0, 64)] = terms[i].astype(BF)

    P = functools.partial

    def spread(slots, lo, hi, works):
        for n, work in enumerate(works):
            slots[lo + n * (hi - lo) // len(works)].append(work)

    steps = [("kv", t, c) for t in range(NTILE) for c in range(NCH)]
    steps += [("q", t, c) for t in range(NTILE) for c in range(NCH)]
    steps += [("o", t, s) for t in range(NTILE) for s in range(2)]
    if cfg.get("only"):
        steps = [steps[i] for i in cfg["only"]]
    mod_parts = [P(mod_part, j, n, half) for j in range(2, 6) for half in range(2) for n in range(8)]
    prev = None
    for step, (kind, t, c) in enumerate(steps):
        slots = [[] for _ in range(7)]
        lower_done = None
        if prev is not None:
            pkind, pt, pc, pres = prev
            if pkind == "kv":
                works = [P(kv_pair, pt, pc, pres, k) for k in (2, 3, 0, 1)]
                if (pt, pc) == (0, 0):
                    late, works = works[:2], works[2:]
                    delayed = works
                elif (pt, pc) == (0, 1):
                    for slot, work in enumerate(delayed + works):
                        slots[slot].append(work)
                else:
                    for slot, work in zip(cfg.get("ks", (0, 1, 2, 3)), works):
                        slots[slot].append(work)
            elif pkind == "q":
                qs = cfg.get("qs", (0, 1, 3, 5))
                for slot, k in zip(qs, (2, 3, 0, 1)):
                    slots[slot].append(P(q_step, pt, pc, pres, k))
            else:
                tok = pt * T + pc * 128
                slots[0].append(P(residual, tok, pres[0]))
                lo, hi = cfg.get("l2a", (0, 4))
                group = _Order(never)
                spread(slots, lo, hi, [P(ln2_piece, tok + r0, group) for r0 in range(0, 128, R2)])
                if pc == 1:
                    slots[hi].append(P(start_out, pt))
        if kind == "kv":
            if t == 0:
                if c == 0:
                    slots[cfg.get("w1", 2)] += [P(wait, "wk1", "wv1"), P(prep_v, 1), P(fold, 1, 1, wkv_c)]
                if c == 1:
                    sa = cfg.get("sa", 2)
                    slots[sa] += [P(wait, "sa", "wk2", "wv2"), lambda: mod_v.__setitem__(0, mod_row(0)),
                                  P(prep_v, 2), P(fold, 1, 2, wkv_c)]
                    slots[sa] += [P(first_tile_terms, r0) for r0 in range(0, TH, 32)]
                    slots[sa] += [P(early_bias, r0, 32) for r0 in range(0, 512 * EARLY, 32)]
                    slots[5].append(late[0])
                    slots[6].append(late[1])
                if c == 2:
                    w3 = cfg.get("w3", 3)
                    slots[w3] = [P(wait, "x1", "wk3", "wv3"), P(prep_v, 3), P(fold, 1, 3, wkv_c)] + slots[w3]
            if (t, c) == (1, 0):
                slots[0].insert(0, P(wait, "x2", "x3", "wq0", "wq1", "wq2", "wq3"))
            if t + 1 < NTILE:
                chunks = (cfg.get('l1', (3,)), (0, 1, 2, 3), (0, 1, 2, 3))[t]
                if c in chunks:
                    pieces = list(range(0, TH, R1))
                    k = chunks.index(c)
                    mine = pieces[k * len(pieces) // len(chunks):(k + 1) * len(pieces) // len(chunks)]
                    spread(slots, 3 if (t, c) == (0, 2) else 0, 6, [P(ln1_piece, t + 1, r0) for r0 in mine])
            if t == cfg.get("foldq", 2):
                slots[5].append(P(fold, 0, c, wq_c))
            if t == 3:
                if c == 0:
                    slots[0].insert(0, P(wait, "wr", "wo", "ga", "sb", "cb", "gb"))
                works = []
                for n in range(8):
                    k0 = n * 128
                    for nk in cfg.get("nks", (64, 64)):
                        works.append(P(mod_piece, 2 + c, k0, nk))
                        k0 += nk
                    works.append(P(prep_wo, c, n * 16))
                spread(slots, 1, 7, works)
        if (kind, t, c) == ("q", 0, 0):
            slots[0].insert(0, P(wait, "wg"))
            slots[6].append(finish_mod)
        if kind == "o":
            last = step == len(steps) - 1
            tok2 = t * T + TH + c * 128
            lower_done = P(residual, tok2)
            lo, hi = (5, 6) if last else cfg.get("l2b", (5, 7))
            group = _Order(never)
            spread(slots, lo, hi, [P(ln2_piece, tok2 + r0, None if last else group) for r0 in range(0, 128, R2)])

        def fill(k, m, slots=slots):
            stream.release = m
            for work in slots[k]:
                work()

        if kind == "kv":
            slot = NTILE if t == 0 and c < EARLY else t
            res = _block_product(lambda i: _dot(wkv_c[c, i], hc_v[h_term(slot, i)], NT), fill)
        elif kind == "q":
            res = _block_product(lambda i: _dot(_unpack(wq_c[c, i]), hc_v[h_term(t, i)], NT), fill)
        else:
            res = _block_product(
                lambda i: _dot(oc_v[t, i, pl.ds(c * 128, 128), :], _unpack(wo_c[i]), NN), fill, lower_done)
        if kind == "kv" and c == NCH - 1:
            order1.link = None
        prev = (kind, t, c, res)

    if cfg.get("only"):
        for name in copies:
            if name not in waited:
                wait(name)
        a, b = prev[3]
        x1_v[0:128, 0:256] = a[0:128, 0:256] + b[0:128, 0:256] + a[0:128, 256:512] + b[0:128, 256:512]
        x1_v[128:136, 0:128] = top[0] + top[1] + top[2] + top[3]
        z = pl.semaphore_read(idle_sem)
        x1_v[136:144, :] = mod_v[z]
        x1_v[144:160, 0:512] = oc_v[z, z, 0:16, :].astype(F32) + hc_v[z, z, 0:16, 0:512].astype(F32) + (
            wo_c[z, 0:16, :] + wq_c[z, z, 0:16, :] + wkv_c[z, z, 0:16, :]).astype(F32)
        x1_v[160:176, 0:128] = kvT[z, 0:16, :].astype(F32) + kv_acc[z, 0:16, :] + z_acc[z, 0:16, :]
        slab_v[0] = x1_v[pl.ds(pl.multiple_of(z * 16, 16), 16), :].astype(BF)
        cpy = pltpu.make_async_copy(slab_v.at[0], out_hbm.at[pl.ds(0, 16)], osems.at[0])
        cpy.start()
        cpy.wait()
        for t in started:
            out_copy(t, 0).wait()
            out_copy(t, 1).wait()
        return

    _, pt, pc, pres = prev
    tok = pt * T + pc * 128
    residual(tok, pres[0])
    for r0 in range(0, 128, R2):
        ln2_piece(tok + r0, None)
    start_out(pt)

    m1, m2, i1, i2 = top
    big = float(2 * S)
    best = jnp.max(m1, axis=0, keepdims=True)
    ia = jnp.min(jnp.where(m1 == best, i1, big), axis=0, keepdims=True)
    taken = i1 == ia
    cm = jnp.where(taken, m2, m1)
    ci = jnp.where(taken, i2, i1)
    second = jnp.max(cm, axis=0, keepdims=True)
    ib = jnp.min(jnp.where(cm == second, ci, big), axis=0, keepdims=True)
    idx_a = jnp.clip(ia.astype(I32)[0, 0], 0, S - 1)
    idx_b = jnp.clip(ib.astype(I32)[0, 0], 0, S - 1)

    sub = lax.broadcasted_iota(I32, (16, D), 0)
    xa = jnp.broadcast_to(x1_v[pl.ds(idx_a, 1), :], (16, D))
    xb = jnp.broadcast_to(x1_v[pl.ds(idx_b, 1), :], (16, D))
    xc, rs = _center(jnp.where(sub == 0, xa, xb))
    gate_r = jax.nn.sigmoid(router(xc, rs))
    hb = (xc * rs * rows_of(4, 16) + rows_of(3, 16)).astype(BF)
    wait("wu", "wd")
    g = _dot(hb, wg_v[...], NN)
    u = _dot(hb, wu_v[...], NN)
    act = (g * jax.nn.sigmoid(g) * u).astype(BF)
    y = _dot(act, wd_v[:, pl.ds(0, D)], NN) * gate_r * rows_of(5, 16)

    for t in range(NTILE):
        out_copy(t, 0).wait()
        out_copy(t, 1).wait()

    def fix(idx, slot):
        start = pl.multiple_of((idx // 16) * 16, 16)
        x1 = x1_v[pl.ds(start, 16), :]
        o = block_out(x1, *_center(x1))
        o = o + jnp.where(sub + start == idx_a, y[0:1], 0.0) + jnp.where(sub + start == idx_b, y[1:2], 0.0)
        slab_v[slot] = o.astype(BF)
        return pltpu.make_async_copy(slab_v.at[slot], out_hbm.at[pl.ds(start, 16)], osems.at[slot])

    fa = fix(idx_a, 0)
    fb = fix(idx_b, 1)
    fa.start()

    @pl.when(idx_a // 16 != idx_b // 16)
    def _():
        fb.start()
        fb.wait()

    fa.wait()
    mark(None)


def make(flags=None, **cfg):
    cfg = dict(dict(tie=False, vmod=32, chain3=1, w1=2, sa=3, w3=1, nks=(40, 48, 40), mstep=8, ks=(1, 2, 3, 4)), **cfg)
    if cfg.get("ev", True):
        flags = dict(flags or {}, XLA_TPU_EVENLY_DISTRIBUTE_CRITICAL_NODES=True)
    pad = cfg.get("pad", 128)

    def run(A_x, A_wqkv, A_w_phi, A_wo, B_x, B_w_r, B_w_gate, B_w_up, B_w_down, c, w_mod):
        del B_x
        any_spec = pl.BlockSpec(memory_space=pl.ANY)
        scratch = [
            pltpu.VMEM((S, D), BF), pltpu.VMEM((3 * NCH, D, 256), BF), pltpu.VMEM((H, DH, DH), BF),
            pltpu.VMEM((D, D), BF), pltpu.VMEM((8, 128), BF),
            pltpu.VMEM((D, F), BF), pltpu.VMEM((D, F), BF), pltpu.VMEM((F, D + pad), BF),
            pltpu.VMEM((1, D), BF), pltpu.VMEM((6, D, D + pad), BF),
            pltpu.VMEM((NCH, 7, 256, DHALF), BF), pltpu.VMEM((NCH, 7, 64, DHALF), I32),
            pltpu.VMEM((7, DHALF // 2, DHALF), I32),
            pltpu.VMEM((NTILE + 1, 4, TH, D), BF), pltpu.VMEM((NTILE, 7, TH, DHALF), BF), pltpu.VMEM((S, D), F32),
            pltpu.VMEM((H // 2, 64, 128), F32), pltpu.VMEM((H // 2, 128, 128), F32),
            pltpu.VMEM((H // 2, 80, 128), BF),
            pltpu.VMEM((10, 8, D), F32), pltpu.VMEM((D, 128), F32), pltpu.VMEM((512 * EARLY, 128), F32), pltpu.VMEM((2, 16, D), BF), pltpu.SemaphoreType.REGULAR,
            pltpu.SemaphoreType.DMA((40,)), pltpu.SemaphoreType.DMA((2 * NTILE,)),
        ]
        out = pl.pallas_call(
            functools.partial(_kernel, cfg=cfg),
            out_shape=jax.ShapeDtypeStruct((S, D), BF),
            in_specs=[any_spec] * 10,
            out_specs=any_spec,
            scratch_shapes=scratch,
            compiler_params=pltpu.CompilerParams(vmem_limit_bytes=120 * 2**20, flags=flags),
            name="fused_block",
        )(A_x.reshape(S, D), A_wqkv, A_w_phi, A_wo, B_w_r.reshape(8, 128), B_w_gate, B_w_up, B_w_down, c, w_mod)
        return out.reshape(1, S, D)
    return run


_run = make(**dict())


@jax.jit
def pallas_adaLN_cond__linear_kernel_hedgehog__moe_arch_mod__prompt_kernel(
    A_x: jax.Array,
    A_wqkv: jax.Array,
    A_w_phi: jax.Array,
    A_wo: jax.Array,
    B_x: jax.Array,
    B_w_r: jax.Array,
    B_w_gate: jax.Array,
    B_w_up: jax.Array,
    B_w_down: jax.Array,
    c: jax.Array,
    w_mod: jax.Array,
):
    return _run(A_x, A_wqkv, A_w_phi, A_wo, B_x, B_w_r, B_w_gate, B_w_up, B_w_down, c, w_mod)
```

```python
import functools

import jax
import jax.numpy as jnp
from jax import lax
from jax.experimental import pallas as pl
from jax.experimental.pallas import tpu as pltpu

S, D, H, DH, F = 2048, 1024, 32, 32, 3584
T = 512
TH = T // 2
DHALF = D // 2
NTILE = S // T
NCH = D // 256
LOG2E = 1.4426950408889634
NN = (((1,), (0,)), ((), ()))
NT = (((1,), (1,)), ((), ()))
TN = (((0,), (0,)), ((), ()))
BF = jnp.bfloat16
F32 = jnp.float32
I32 = jnp.int32


def _dot(a, b, dims):
    return lax.dot_general(a, b, dims, preferred_element_type=F32)


def _recip(x):
    return pltpu.reciprocal(x, approx=False, full_range=False)


def _center(x, order=None):
    s = jnp.sum(x, axis=-1, keepdims=True)
    if order is not None:
        s = order.after(s)
    xc = x - s * (1.0 / D)
    rs = lax.rsqrt(jnp.sum(xc * xc, axis=-1, keepdims=True) * (1.0 / D) + 1e-5)
    if order is not None:
        order.link = rs
    return xc, rs


def _pair_reduce(x, op):
    r = x[0:8]
    for i in range(1, 8):
        r = op(r, x[8 * i:8 * i + 8])
    r = op(r, pltpu.roll(r, 4, 0))
    return op(r, pltpu.roll(r, 2, 0))


def _tile8(r, n):
    return jnp.concatenate([r] * n, axis=0)


def _hedgehog(p):
    mx = _tile8(_pair_reduce(p, jnp.maximum), 8)
    mn = _tile8(_pair_reduce(p, jnp.minimum), 8)
    ep = jnp.exp2(p - mx)
    en = jnp.exp2(mn - p)
    rp = _tile8(_recip(_pair_reduce(ep, jnp.add)), 8)
    rn = _tile8(_recip(_pair_reduce(en, jnp.add)), 8)
    return jnp.concatenate([ep * rp, en * rn], axis=0)


def _hedgehog_scaled(p):
    mx = _tile8(_pair_reduce(p, jnp.maximum), 8)
    mn = _tile8(_pair_reduce(p, jnp.minimum), 8)
    ep = jnp.exp2(p - mx)
    en = jnp.exp2(mn - p)
    sp = _pair_reduce(ep, jnp.add)
    ratio = _tile8(sp * _recip(_pair_reduce(en, jnp.add)), 8)
    return jnp.concatenate([ep, en * ratio], axis=0), sp


def _lhs_terms(a11, a12, a21, a22):
    return (a11 + a22, a21 + a22, a11, a22, a11 + a12, a21 - a11, a12 - a22)


def _rhs_terms(b11, b12, b21, b22):
    return (b11 + b22, b11, b12 - b22, b21 - b11, b22, b11 + b12, b21 + b22)


def _block_product(product, fill, lower_done=None):
    m0 = product(0)
    fill(0, m0)
    m1 = product(1)
    fill(1, m1)
    c22 = m0 - m1
    m3 = product(3)
    fill(2, m3)
    c21 = m1 + m3
    c11 = m0 + m3
    m2 = product(2)
    fill(3, m2)
    c22 = c22 + m2
    m5 = product(5)
    fill(4, m5)
    lower = jnp.concatenate([c21, c22 + m5], axis=1)
    if lower_done is not None:
        lower_done(lower)
    m4 = product(4)
    fill(5, m4)
    c12 = m2 + m4
    c11 = c11 - m4
    m6 = product(6)
    fill(6, m6)
    return jnp.concatenate([c11 + m6, c12], axis=1), lower


def _merge_top2(a, b):
    def ahead(v, i, w, j):
        return (v > w) | ((v == w) & (i < j))

    first = ahead(a[0], a[2], b[0], b[2])
    lose_v, lose_i = jnp.where(first, b[0], a[0]), jnp.where(first, b[2], a[2])
    next_v, next_i = jnp.where(first, a[1], b[1]), jnp.where(first, a[3], b[3])
    second = ahead(lose_v, lose_i, next_v, next_i)
    return (jnp.where(first, a[0], b[0]), jnp.where(second, lose_v, next_v),
            jnp.where(first, a[2], b[2]), jnp.where(second, lose_i, next_i))


def _pack(x):
    return pltpu.bitcast(x.astype(BF), I32)


def _unpack(x):
    return pltpu.bitcast(x, BF)


class _Order:
    def __init__(self, never):
        self.never = never
        self.link = None
        self.release = None

    def after(self, v):
        for dep in (self.link, self.release):
            if dep is not None:
                probe = self.never[:v.shape[0], :v.shape[1]]
                v = jnp.where(probe != probe, dep[:v.shape[0], :v.shape[1]], v)
        return v


def _kernel(x_hbm, wqkv_hbm, wphi_hbm, wo_hbm, wr_hbm, wg_hbm, wu_hbm, wd_hbm, c_hbm, wmod_hbm,
            out_hbm,
            x_v, wqkv_v, wphi_v, wo_v, wr_v, wg_v, wu_v, wd_v, c_v, wmod_v,
            wkv_c, wq_c, wo_c, hc_v, oc_v, x1_v, xn_v, kv_acc, z_acc, kvT, mod_v, sb_v, bias_v, slab_v, idle_sem,
            sems, osems, *, cfg):
    R1, R2, RB = cfg.get("R1", 16), cfg.get("R2", 16), cfg.get("RB", 32)

    def col(ref, j, w=D):
        return ref.at[:, pl.ds(j * w, w)]

    def x_copy(t):
        return ("x%d" % t, x_hbm.at[pl.ds(t * T, T)], x_v.at[pl.ds(t * T, T)])

    def w_copy(name, j, c):
        return ("%s%d" % (name, c), col(wqkv_hbm, j * NCH + c, 256), wqkv_v.at[j * NCH + c])

    def mod_copy(name, j):
        return (name, col(wmod_hbm, j), wmod_v.at[j, :, pl.ds(0, D)])

    def scale_copy(d, k):
        rows = pl.ds(k * DHALF, DHALF)
        return ("ca%d%d" % (d, k), wmod_hbm.at[rows, pl.ds(D + d * DHALF, DHALF)],
                wmod_v.at[1, rows, pl.ds(d * DHALF, DHALF)])

    order = [("c", c_hbm, c_v), x_copy(0), ("wphi", wphi_hbm, wphi_v),
             w_copy("wk", 1, 0), w_copy("wv", 2, 0), *[scale_copy(d, k) for d in range(2) for k in range(2)],
             w_copy("wk", 1, 1), w_copy("wv", 2, 1), w_copy("wk", 1, 2), w_copy("wv", 2, 2),
             w_copy("wk", 1, 3), w_copy("wv", 2, 3), x_copy(1), mod_copy("sa", 0), x_copy(2), x_copy(3)]
    order += [w_copy("wq", 0, c) for c in range(NCH)]
    order += [("wr", wr_hbm, wr_v), ("wo", wo_hbm, wo_v), mod_copy("ga", 2), mod_copy("sb", 3), mod_copy("cb", 4), mod_copy("gb", 5),
              ("wg", wg_hbm, wg_v), ("wu", wu_hbm, wu_v), ("wd", wd_hbm, wd_v.at[:, pl.ds(0, D)])]
    copies = {}
    for i, (name, src, dst) in enumerate(order):
        copies[name] = pltpu.make_async_copy(src, dst, sems.at[i])
        copies[name].start()

    waited, started = set(), []

    scope = []

    def mark(name):
        if cfg.get("marks"):
            if scope:
                scope.pop().__exit__(None, None, None)
            if name:
                scope.append(jax.named_scope(name))
                scope[0].__enter__()

    def wait(*names):
        mark("w_" + names[0])
        for name in names:
            copies[name].wait()
            waited.add(name)
        mark("r_" + names[0])


    wait("c", "x0")
    cf = c_v[...].astype(F32)
    never = jnp.broadcast_to(cf[:, 0:128], (32, 128))
    order1, order2, order3, order4 = [_Order(never) for _ in range(4)]
    sc = jnp.broadcast_to(cf * jax.nn.sigmoid(cf), (16, D)).astype(BF)

    def normalized(tok, n, order=None):
        xc, rs = _center(x_v[pl.ds(tok, n), :].astype(F32), order)
        return xc * rs

    for r0 in range(0, T, 32):
        xn_v[pl.ds(r0, 32), :] = normalized(r0, 32)

    wait("wphi")
    row = lax.broadcasted_iota(I32, (128, DH), 0)
    lane = lax.broadcasted_iota(I32, (128, DH), 1)
    expand = jnp.where(((row % 64) // 2) == lane, 1.0, 0.0).astype(BF)
    bdt = _dot(expand, wphi_v[...].reshape(H * DH, DH), NT)
    row = lax.broadcasted_iota(I32, (128, D), 0)
    lane = lax.broadcasted_iota(I32, (128, D), 1)
    bdt = jnp.where(2 * (row // 64) + (row % 2) == (lane % 128) // DH, bdt, 0.0).astype(BF)

    def mod_row(j):
        return _dot(sc, wmod_v[j, :, pl.ds(0, D)], NN)[0:8]

    def mod_part(j, n, half):
        part = _dot(sc[:, half * DHALF:(half + 1) * DHALF],
                    wmod_v[j, pl.ds(half * DHALF, DHALF), pl.ds(n * 128, 128)], NN)[0:8]
        if half == 0:
            mod_v[j, :, pl.ds(n * 128, 128)] = part
        else:
            mod_v[j, :, pl.ds(n * 128, 128)] += part

    for k0 in range(0, D, 128):
        sb_v[pl.ds(k0, 128), :] = jnp.broadcast_to(sc[0:1, k0:k0 + 128].astype(F32), (128, 128)).T

    partial_mod = {}

    def mod_piece(j, k0, nk):
        acc = partial_mod.pop(j, None)
        step = cfg.get("mstep", 16)
        for k in range(k0, k0 + nk, step):
            s_col = sb_v[pl.ds(k, step), :]
            if k == k0 and cfg.get("chain3"):
                s_col = order3.after(s_col)
            term = wmod_v[j, pl.ds(k, step), pl.ds(0, D)].astype(F32) * jnp.concatenate([s_col] * (D // 128), axis=1)
            if step == 16:
                term = term[0:8] + term[8:16]
            acc = term if acc is None else acc + term
        if cfg.get("chain3"):
            link = acc[:, 0:128]
            for _ in range(cfg["chain3"]):
                link = jnp.broadcast_to(jnp.max(link, axis=-1, keepdims=True), (8, 128))
            order3.link = jnp.concatenate([link, link], axis=0)
        if k0 + nk < D:
            partial_mod[j] = acc
        else:
            mod_v[j] = jnp.broadcast_to(jnp.sum(acc, axis=0, keepdims=True), (8, D))

    def finish_mod():
        wr = wr_v[...].astype(F32)
        wr_row = jnp.concatenate([jnp.broadcast_to(wr[j:j + 1, :], (8, 128)) for j in range(8)], axis=1)
        shift, scale, gate = mod_v[3], 1.0 + mod_v[4], mod_v[5]
        mod_v[4] = scale
        mod_v[6] = gate * scale
        mod_v[7] = gate * shift
        mod_v[8] = wr_row * scale
        mod_v[9] = jnp.broadcast_to(jnp.sum(wr_row * shift, axis=-1, keepdims=True), (8, D))

    def rows_of(j, n):
        return _tile8(mod_v[j], n // 8)

    def h_term(t, i, r0=0, n=TH):
        return (t, i // 2, pl.ds(r0, n), pl.ds((i % 2) * DHALF, DHALF))

    def store_h_terms(t, r0, n, a, b):
        h1, h2 = a * rows_of(1, n), b * rows_of(1, n)
        terms = _rhs_terms(h1[:, :DHALF], h2[:, :DHALF], h1[:, DHALF:], h2[:, DHALF:])
        for i, term in enumerate(terms):
            hc_v[h_term(t, i, r0, n)] = term.astype(BF)

    def ln1_piece(t, r0):
        second = order4 if t == 1 else order1
        store_h_terms(t, r0, R1, normalized(t * T + r0, R1, order1), normalized(t * T + TH + r0, R1, second))

    def store_lhs_terms(top, bot, dst, c, r0):
        terms = _lhs_terms(top[:, :DHALF], top[:, DHALF:], bot[:, :DHALF], bot[:, DHALF:])
        for i, term in enumerate(terms):
            if dst.dtype == I32:
                dst[c, i] = _pack(term)
            else:
                dst[c, i, pl.ds(r0, 128), :] = term.astype(BF)

    def shift_bias(dst, w, order):
        shift = jnp.concatenate([order.after(mod_v[0, :, l:l + 128]) for l in range(0, D, 128)], axis=1)
        b = jnp.sum(w * _tile8(shift, w.shape[0] // 8), axis=-1, keepdims=True)
        order.link = jnp.broadcast_to(b, (w.shape[0], 128))
        bias_v[pl.ds(dst, w.shape[0]), :] = order.link

    def kv_bias(r0):
        shift_bias(r0, x1_v[pl.ds(r0, RB), :], order2)

    def keep_weights(c, r0, halves):
        for g in range(2):
            x1_v[pl.ds(c * 512 + g * 256 + r0, 128), :] = halves[g]

    def folded(j, c):
        halves = []
        for g in range(2):
            w = wqkv_v[j * NCH + c, :, g * 128:(g + 1) * 128]
            gg = 2 * c + g
            halves.append(_dot(bdt[:, gg * 128:(gg + 1) * 128], w, NT) * LOG2E)
        return halves

    def prep_k(c):
        halves = folded(1, c)
        store_lhs_terms(halves[0], halves[1], wkv_c, c, 0)
        keep_weights(c, 0, halves)

    def prep_q(c):
        halves = folded(0, c)
        for r0 in range(0, 128, 16):
            top, bot = [jnp.concatenate([order2.after(half[r0:r0 + 16, l:l + 128]) for l in range(0, D, 128)], axis=1)
                        if g == 0 and cfg.get("pq", 1) else half[r0:r0 + 16] for g, half in enumerate(halves)]
            terms = _lhs_terms(top[:, :DHALF], top[:, DHALF:], bot[:, :DHALF], bot[:, DHALF:])
            for i, term in enumerate(terms):
                wq_c[c, i, pl.ds(r0 // 2, 8), :] = _pack(term)
            shift_bias(S + c * 256 + r0, top, _Order(never))
            shift_bias(S + c * 256 + 128 + r0, bot, order2 if cfg.get("pq", 1) else _Order(never))

    def prep_v(c):
        halves = [wqkv_v[2 * NCH + c, :, g * 128:(g + 1) * 128].T.astype(F32) for g in range(2)]
        store_lhs_terms(halves[0], halves[1], wkv_c, c, 128)
        keep_weights(c, 128, halves)

    def prep_wo(c, r0):
        def rows(r):
            w = wo_v[pl.ds(r, 16), :].astype(F32)
            return jnp.concatenate([order3.after(w[:, l:l + 128]) for l in range(0, D, 128)], axis=1)
        top, bot = rows(c * 256 + r0), wo_v[pl.ds(c * 256 + 128 + r0, 16), :].astype(F32)
        terms = _rhs_terms(top[:, :DHALF], top[:, DHALF:], bot[:, :DHALF], bot[:, DHALF:])
        for i, term in enumerate(terms):
            wo_c[i, pl.ds(c * 64 + r0 // 2, 8), :] = _pack(term)
        order3.link = jnp.broadcast_to(jnp.max(terms[0][:, 0:128], axis=-1, keepdims=True), (16, 128))

    stream = _Order(never)

    def behind_product(v):
        head = jnp.concatenate([stream.after(v[0:8, l:l + 128]) for l in range(0, T, 128)], axis=1)
        return jnp.concatenate([head, v[8:]], axis=0)

    def bias_rows(r0):
        return jnp.concatenate([bias_v[pl.ds(r0, 64), :]] * (T // 128), axis=1)

    def kv_pair(t, c, res, k):
        g, q = divmod(k, 2)
        pair = 4 * c + k
        r0 = c * 512 + g * 256 + q * 64
        phi = _hedgehog(res[g][q * 64:(q + 1) * 64] + bias_rows(r0))
        vt = behind_product(res[g][128 + q * 64:128 + (q + 1) * 64]).astype(BF)
        zs = phi[:, 0:128]
        for l in range(1, T // 128):
            zs = zs + phi[:, l * 128:(l + 1) * 128]
        kv = _dot(vt, phi.astype(BF), NT)
        if t > 0:
            zs = zs + z_acc[pair]
            kv = kv + kv_acc[pair]
        if t < NTILE - 1:
            z_acc[pair] = zs
            kv_acc[pair] = kv
        else:
            z = jnp.broadcast_to(jnp.sum(zs.T, axis=0, keepdims=True), (16, 128))
            kv = kv + bias_v[pl.ds(r0 + 128, 64), :] * _tile8(z[0:8], 8)
            row = lax.broadcasted_iota(I32, (80, 128), 0)
            lane = lax.broadcasted_iota(I32, (80, 128), 1)
            head = jnp.where(row < 64, row // DH, (row - 64) // 8)
            kvT[pair] = jnp.where(head == lane % 2, jnp.concatenate([kv, z], axis=0), 0.0).astype(BF)

    def q_pair(c, res, k):
        g, q = divmod(k, 2)
        pair = 4 * c + k
        even = (lax.broadcasted_iota(I32, (8, T), 0) % 2) == 0
        phi, scale = _hedgehog_scaled(res[g][q * 64:(q + 1) * 64] + bias_rows(S + pair * 64))
        if cfg.get("tq"):
            phi = behind_product(phi)
        nd = _dot(kvT[pair], phi.astype(BF), NN)
        swapped = pltpu.roll(scale, 1, 0)
        inv_a = _recip(nd[64:72] + 1e-6 * jnp.where(even, scale, swapped))
        inv_b = _recip(nd[72:80] + 1e-6 * jnp.where(even, swapped, scale))
        return nd[0:64] * jnp.concatenate([inv_a] * 4 + [inv_b] * 4, axis=0)

    held = {}

    def q_step(t, c, res, k):
        held[k] = q_pair(c, res, k)
        if k == 3:
            held["lower"] = jnp.concatenate([held.pop(2), held.pop(3)], axis=0).T
        if k == 1:
            o1, o2 = jnp.concatenate([held.pop(0), held.pop(1)], axis=0).T, held.pop("lower")
            for i, term in enumerate(_lhs_terms(o1[:TH], o2[:TH], o1[TH:], o2[TH:])):
                oc_v[t, i, :, pl.ds(c * 128, 128)] = term.astype(BF)

    def residual(tok, attn):
        rows = pl.ds(tok, 128)
        x1_v[rows, :] = x_v[rows, :].astype(F32) + rows_of(2, 128) * attn

    def block_out(x1, xc, rs):
        n = x1.shape[0]
        return xc * (rs * rows_of(6, n)) + (x1 + rows_of(7, n))

    def router(xc, rs):
        n = xc.shape[0]
        return jnp.sum(xc * rows_of(8, n), axis=-1, keepdims=True) * rs + rows_of(9, n)[:, 0:1]

    found = []

    def ln2_piece(tok, order):
        x1 = x1_v[pl.ds(tok, R2), :]
        xc, rs = _center(x1, order)
        t, r0 = divmod(tok, T)
        hc_v[t, r0 // TH, pl.ds(r0 % TH, R2), :] = block_out(x1, xc, rs).astype(BF)
        r = router(xc, rs)
        sub = lax.broadcasted_iota(I32, (8, 128), 0).astype(F32)
        ra, rb = jnp.broadcast_to(r[0:8], (8, 128)), jnp.broadcast_to(r[8:16], (8, 128))
        ia, ib = sub + float(tok), sub + float(tok + 8)
        first = ra >= rb
        found.append((jnp.where(first, ra, rb), jnp.where(first, rb, ra),
                      jnp.where(first, ia, ib), jnp.where(first, ib, ia)))
        if order is not None:
            found[:] = [_merge_top2(found[0], found[1])] if len(found) == 2 else found

    def out_copy(t, half):
        return pltpu.make_async_copy(hc_v.at[t, half], out_hbm.at[pl.ds(t * T + half * TH, TH)],
                                     osems.at[2 * t + half])

    def start_out(t):
        for half in range(2):
            out_copy(t, half).start()
        started.append(t)

    wait("wk0", "wv0")
    prep_k(0)
    prep_v(0)

    def first_terms(d, wanted):
        cols = pl.ds(d * DHALF, DHALF)
        scale = 1.0
        for k in range(2):
            wait("ca%d%d" % (d, k))
            scale = scale + _dot(sc[:, k * DHALF:(k + 1) * DHALF], wmod_v[1, pl.ds(k * DHALF, DHALF), cols], NN)[0:8]
        mod_v[1, :, cols] = scale

        def block(half, dd, r0):
            if dd > d:
                return None
            cc = pl.ds(dd * DHALF, DHALF)
            return xn_v[pl.ds(half * TH + r0, 64), cc] * _tile8(mod_v[1, :, cc], 8)

        for group in wanted:
            for r0 in range(0, TH, 64):
                b11, b12, b21, b22 = block(0, 0, r0), block(1, 0, r0), block(0, 1, r0), block(1, 1, r0)
                terms = _rhs_terms(b11, b12, b21, b22) if d else {1: b11, 5: b11 + b12}
                for i in group:
                    hc_v[h_term(0, i, r0, 64)] = terms[i].astype(BF)

    def kv_product(t, c, i):
        return _dot(wkv_c[c, i], hc_v[h_term(t, i)], NT)

    first_terms(0, ((1,), (5,)))
    head_start = {i: kv_product(0, 0, i) for i in (1, 5)}
    first_terms(1, cfg.get("tg", ((0,), (3, 2, 4, 6))))

    P = functools.partial

    def spread(slots, lo, hi, works):
        for n, work in enumerate(works):
            slots[lo + n * (hi - lo) // len(works)].append(work)

    steps = [("kv", t, c) for t in range(NTILE) for c in range(NCH)]
    steps += [("q", t, c) for t in range(NTILE) for c in range(NCH)]
    steps += [("o", t, s) for t in range(NTILE) for s in range(2)]
    if cfg.get("only"):
        steps = [steps[i] for i in cfg["only"]]
    mod_parts = [P(mod_part, j, n, half) for j in range(2, 6) for half in range(2) for n in range(8)]
    prev = None
    pending = []
    for step, (kind, t, c) in enumerate(steps):
        slots = [[] for _ in range(7)]
        lower_done = None
        if prev is not None:
            pkind, pt, pc, pres = prev
            if pkind == "kv":
                pending += [P(kv_pair, pt, pc, pres, k) for k in (2, 3, 0, 1)]
                n = len(pending) if cfg.get("only") or kind != "kv" else cfg["quota"][t * NCH + c]
                for slot in cfg["kslots"][n]:
                    slots[slot].append(pending.pop(0))
            elif pkind == "q":
                qs = cfg.get("qs", (0, 1, 3, 5))
                for slot, k in zip(qs, (2, 3, 0, 1)):
                    slots[slot].append(P(q_step, pt, pc, pres, k))
            else:
                tok = pt * T + pc * 128
                slots[0].append(P(residual, tok, pres[0]))
                lo, hi = cfg.get("l2a", (0, 4))
                group = _Order(never)
                spread(slots, lo, hi, [P(ln2_piece, tok + r0, group) for r0 in range(0, 128, R2)])
                if pc == 1:
                    slots[hi].append(P(start_out, pt))
        if kind == "kv":
            if t == 0 and c + 1 < NCH:
                names = (("wk1", "wv1"), ("wk2", "wv2", "wk3", "wv3"), ("x1",))[c]
                k = cfg["ws"][c]
                slots[k] += [P(wait, *names), P(prep_v, c + 1), P(prep_k, c + 1)]
            if (t, c) == (1, 0):
                slots[0] = [P(wait, "sa", "x2"), lambda: mod_v.__setitem__(0, mod_row(0))] + slots[0]
            if t == 1 and c < 2:
                for k in range(2):
                    first = (2 * c + k) * 512
                    at = cfg["bs"][c][k]
                    slots[at] += [P(kv_bias, r0) for r0 in range(first, first + 512, RB)]
            if (t, c) == (2, 0):
                slots[0].insert(0, P(wait, "x3", "wq0", "wq1", "wq2", "wq3", "wr", "wo"))
            if t + 1 < NTILE:
                chunks = ((2, 3), (0, 1, 2, 3), (0, 1, 2, 3))[t]
                if c in chunks:
                    pieces = list(range(0, TH, R1))
                    k = chunks.index(c)
                    mine = pieces[k * len(pieces) // len(chunks):(k + 1) * len(pieces) // len(chunks)]
                    spread(slots, cfg["ws"][2] + 1 if (t, c) == (0, 2) else 0, 6, [P(ln1_piece, t + 1, r0) for r0 in mine])
            if t == cfg.get("foldq", 2):
                slots[5].append(P(prep_q, c))
            if t == 3:
                if c == 0:
                    slots[0].insert(0, P(wait, "ga", "sb", "cb", "gb"))
                works = []
                for n in range(8):
                    k0 = n * 128
                    for nk in cfg.get("nks", (64, 64)):
                        works.append(P(mod_piece, 2 + c, k0, nk))
                        k0 += nk
                    works.append(P(prep_wo, c, n * 16))
                spread(slots, 1, 7, works)
        if (kind, t, c) == ("q", 0, 0):
            slots[0].insert(0, P(wait, "wg"))
            slots[6].append(finish_mod)
        if kind == "o":
            last = step == len(steps) - 1
            tok2 = t * T + TH + c * 128
            lower_done = P(residual, tok2)
            lo, hi = (5, 6) if last else cfg.get("l2b", (5, 7))
            group = _Order(never)
            spread(slots, lo, hi, [P(ln2_piece, tok2 + r0, None if last else group) for r0 in range(0, 128, R2)])

        def fill(k, m, slots=slots):
            stream.release = m
            for work in slots[k]:
                work()

        if kind == "kv":
            res = _block_product(lambda i: head_start.pop(i) if i in head_start else kv_product(t, c, i), fill)
        elif kind == "q":
            res = _block_product(lambda i: _dot(_unpack(wq_c[c, i]), hc_v[h_term(t, i)], NT), fill)
        else:
            res = _block_product(
                lambda i: _dot(oc_v[t, i, pl.ds(c * 128, 128), :], _unpack(wo_c[i]), NN), fill, lower_done)
        if kind == "kv" and c == NCH - 1:
            order1.link = None
        prev = (kind, t, c, res)

    if cfg.get("only"):
        for name in copies:
            if name not in waited:
                wait(name)
        a, b = prev[3]
        x1_v[0:128, 0:256] = a[0:128, 0:256] + b[0:128, 0:256] + a[0:128, 256:512] + b[0:128, 256:512]
        x1_v[128:136, 0:128] = sum(sum(f) for f in found) if found else jnp.zeros((8, 128), F32)
        z = pl.semaphore_read(idle_sem)
        x1_v[136:144, :] = mod_v[z]
        x1_v[144:160, 0:512] = oc_v[z, z, 0:16, :].astype(F32) + hc_v[z, z, 0:16, 0:512].astype(F32) + (
            wo_c[z, 0:16, :] + wq_c[z, z, 0:16, :] + wkv_c[z, z, 0:16, :]).astype(F32)
        x1_v[160:176, 0:128] = kvT[z, 0:16, :].astype(F32) + kv_acc[z, 0:16, :] + z_acc[z, 0:16, :]
        slab_v[0] = x1_v[pl.ds(pl.multiple_of(z * 16, 16), 16), :].astype(BF)
        cpy = pltpu.make_async_copy(slab_v.at[0], out_hbm.at[pl.ds(0, 16)], osems.at[0])
        cpy.start()
        cpy.wait()
        for t in started:
            out_copy(t, 0).wait()
            out_copy(t, 1).wait()
        return

    _, pt, pc, pres = prev
    tok = pt * T + pc * 128
    residual(tok, pres[0])
    for r0 in range(0, 128, R2):
        ln2_piece(tok + r0, None)
    start_out(pt)

    while len(found) > 1:
        found[:] = [_merge_top2(*found[k:k + 2]) if k + 1 < len(found) else found[k]
                    for k in range(0, len(found), 2)]
    m1, m2, i1, i2 = found[0]
    big = float(2 * S)
    best = jnp.max(m1, axis=0, keepdims=True)
    ia = jnp.min(jnp.where(m1 == best, i1, big), axis=0, keepdims=True)
    taken = i1 == ia
    cm = jnp.where(taken, m2, m1)
    ci = jnp.where(taken, i2, i1)
    second = jnp.max(cm, axis=0, keepdims=True)
    ib = jnp.min(jnp.where(cm == second, ci, big), axis=0, keepdims=True)
    idx_a = jnp.clip(ia.astype(I32)[0, 0], 0, S - 1)
    idx_b = jnp.clip(ib.astype(I32)[0, 0], 0, S - 1)

    sub = lax.broadcasted_iota(I32, (16, D), 0)
    xa = jnp.broadcast_to(x1_v[pl.ds(idx_a, 1), :], (16, D))
    xb = jnp.broadcast_to(x1_v[pl.ds(idx_b, 1), :], (16, D))
    xc, rs = _center(jnp.where(sub == 0, xa, xb))
    gate_r = jax.nn.sigmoid(router(xc, rs))
    hb = (xc * rs * rows_of(4, 16) + rows_of(3, 16)).astype(BF)
    wait("wu", "wd")
    for t in range(NTILE - 1):
        out_copy(t, 0).wait()
        out_copy(t, 1).wait()

    def slab(idx):
        start = pl.multiple_of((idx // 16) * 16, 16)
        x1 = x1_v[pl.ds(start, 16), :]
        return start, block_out(x1, *_center(x1))

    slabs = [slab(idx_a), slab(idx_b)]
    g = _dot(hb, wg_v[...], NN)
    u = _dot(hb, wu_v[...], NN)
    act = (g * jax.nn.sigmoid(g) * u).astype(BF)
    y = _dot(act, wd_v[:, pl.ds(0, D)], NN) * (gate_r * rows_of(5, 16))

    fixes = []
    for slot, (start, o) in enumerate(slabs):
        o = o + jnp.where(sub + start == idx_a, y[0:1], 0.0) + jnp.where(sub + start == idx_b, y[1:2], 0.0)
        slab_v[slot] = o.astype(BF)
        fixes.append(pltpu.make_async_copy(slab_v.at[slot], out_hbm.at[pl.ds(start, 16)], osems.at[slot]))
    out_copy(NTILE - 1, 0).wait()
    out_copy(NTILE - 1, 1).wait()
    fixes[0].start()

    @pl.when(idx_a // 16 != idx_b // 16)
    def _():
        fixes[1].start()
        fixes[1].wait()

    fixes[0].wait()
    mark(None)


def make(flags=None, **cfg):
    cfg = dict(dict(tie=False, vmod=32, chain3=1, ws=(3, 3, 2), bs=((0, 2), (0, 2)),
                    quota=(0, 0, 0, 0, 2, 4, 5, 5, 6, 6, 6, 6, 5, 5, 5, 5),
                    kslots={0: (), 2: (4, 5), 3: (3, 4, 5), 4: (1, 2, 3, 4), 5: (1, 2, 3, 4, 5), 6: (0, 1, 2, 3, 4, 5)},
                    nks=(40, 48, 40), mstep=8, ks=(1, 2, 3, 4)), **cfg)
    if cfg.get("ev", True):
        flags = dict(flags or {}, XLA_TPU_EVENLY_DISTRIBUTE_CRITICAL_NODES=True)
    pad = cfg.get("pad", 128)

    def run(A_x, A_wqkv, A_w_phi, A_wo, B_x, B_w_r, B_w_gate, B_w_up, B_w_down, c, w_mod):
        del B_x
        any_spec = pl.BlockSpec(memory_space=pl.ANY)
        scratch = [
            pltpu.VMEM((S, D), BF), pltpu.VMEM((3 * NCH, D, 256), BF), pltpu.VMEM((H, DH, DH), BF),
            pltpu.VMEM((D, D), BF), pltpu.VMEM((8, 128), BF),
            pltpu.VMEM((D, F), BF), pltpu.VMEM((D, F), BF), pltpu.VMEM((F, D + pad), BF),
            pltpu.VMEM((1, D), BF), pltpu.VMEM((6, D, D + pad), BF),
            pltpu.VMEM((NCH, 7, 256, DHALF), BF), pltpu.VMEM((NCH, 7, 64, DHALF), I32),
            pltpu.VMEM((7, DHALF // 2, DHALF), I32),
            pltpu.VMEM((NTILE, 4, TH, D), BF), pltpu.VMEM((NTILE, 7, TH, DHALF), BF), pltpu.VMEM((S, D), F32), pltpu.VMEM((T, D), F32),
            pltpu.VMEM((H // 2, 64, 128), F32), pltpu.VMEM((H // 2, 128, 128), F32),
            pltpu.VMEM((H // 2, 80, 128), BF),
            pltpu.VMEM((10, 8, D), F32), pltpu.VMEM((D, 128), F32), pltpu.VMEM((S + D, 128), F32), pltpu.VMEM((2, 16, D), BF), pltpu.SemaphoreType.REGULAR,
            pltpu.SemaphoreType.DMA((40,)), pltpu.SemaphoreType.DMA((2 * NTILE,)),
        ]
        out = pl.pallas_call(
            functools.partial(_kernel, cfg=cfg),
            out_shape=jax.ShapeDtypeStruct((S, D), BF),
            in_specs=[any_spec] * 10,
            out_specs=any_spec,
            scratch_shapes=scratch,
            compiler_params=pltpu.CompilerParams(vmem_limit_bytes=120 * 2**20, flags=flags),
            name="fused_block",
        )(A_x.reshape(S, D), A_wqkv, A_w_phi, A_wo, B_w_r.reshape(8, 128), B_w_gate, B_w_up, B_w_down, c, w_mod)
        return out.reshape(1, S, D)
    return run


_run = make(**dict())


@jax.jit
def pallas_adaLN_cond__linear_kernel_hedgehog__moe_arch_mod__prompt_kernel(
    A_x: jax.Array,
    A_wqkv: jax.Array,
    A_w_phi: jax.Array,
    A_wo: jax.Array,
    B_x: jax.Array,
    B_w_r: jax.Array,
    B_w_gate: jax.Array,
    B_w_up: jax.Array,
    B_w_down: jax.Array,
    c: jax.Array,
    w_mod: jax.Array,
):
    return _run(A_x, A_wqkv, A_w_phi, A_wo, B_x, B_w_r, B_w_gate, B_w_up, B_w_down, c, w_mod)
```

```python
import functools

import jax
import jax.numpy as jnp
from jax import lax
from jax.experimental import pallas as pl
from jax.experimental.pallas import tpu as pltpu

S, D, H, DH, F = 2048, 1024, 32, 32, 3584
T = 512
TH = T // 2
DHALF = D // 2
NTILE = S // T
NCH = D // 256
LOG2E = 1.4426950408889634
NN = (((1,), (0,)), ((), ()))
NT = (((1,), (1,)), ((), ()))
TN = (((0,), (0,)), ((), ()))
BF = jnp.bfloat16
F32 = jnp.float32
I32 = jnp.int32


def _dot(a, b, dims):
    return lax.dot_general(a, b, dims, preferred_element_type=F32)


def _recip(x):
    return pltpu.reciprocal(x, approx=False, full_range=False)


def _center(x, order=None):
    s = jnp.sum(x, axis=-1, keepdims=True)
    if order is not None:
        s = order.after(s)
    xc = x - s * (1.0 / D)
    rs = lax.rsqrt(jnp.sum(xc * xc, axis=-1, keepdims=True) * (1.0 / D) + 1e-5)
    if order is not None:
        order.link = rs
    return xc, rs


def _pair_reduce(x, op):
    r = x[0:8]
    for i in range(1, 8):
        r = op(r, x[8 * i:8 * i + 8])
    r = op(r, pltpu.roll(r, 4, 0))
    return op(r, pltpu.roll(r, 2, 0))


def _tile8(r, n):
    return jnp.concatenate([r] * n, axis=0)


def _hedgehog(p):
    mx = _tile8(_pair_reduce(p, jnp.maximum), 8)
    mn = _tile8(_pair_reduce(p, jnp.minimum), 8)
    ep = jnp.exp2(p - mx)
    en = jnp.exp2(mn - p)
    rp = _tile8(_recip(_pair_reduce(ep, jnp.add)), 8)
    rn = _tile8(_recip(_pair_reduce(en, jnp.add)), 8)
    return jnp.concatenate([ep * rp, en * rn], axis=0)


def _hedgehog_scaled(p):
    mx = _tile8(_pair_reduce(p, jnp.maximum), 8)
    mn = _tile8(_pair_reduce(p, jnp.minimum), 8)
    ep = jnp.exp2(p - mx)
    en = jnp.exp2(mn - p)
    sp = _pair_reduce(ep, jnp.add)
    ratio = _tile8(sp * _recip(_pair_reduce(en, jnp.add)), 8)
    return jnp.concatenate([ep, en * ratio], axis=0), sp


def _lhs_terms(a11, a12, a21, a22):
    return (a11 + a22, a21 + a22, a11, a22, a11 + a12, a21 - a11, a12 - a22)


def _rhs_terms(b11, b12, b21, b22):
    return (b11 + b22, b11, b12 - b22, b21 - b11, b22, b11 + b12, b21 + b22)


def _block_product(product, fill, lower_done=None):
    m0 = product(0)
    fill(0, m0)
    m1 = product(1)
    fill(1, m1)
    c22 = m0 - m1
    m3 = product(3)
    fill(2, m3)
    c21 = m1 + m3
    c11 = m0 + m3
    m2 = product(2)
    fill(3, m2)
    c22 = c22 + m2
    m5 = product(5)
    fill(4, m5)
    lower = jnp.concatenate([c21, c22 + m5], axis=1)
    if lower_done is not None:
        lower_done(lower)
    m4 = product(4)
    fill(5, m4)
    c12 = m2 + m4
    c11 = c11 - m4
    m6 = product(6)
    fill(6, m6)
    return jnp.concatenate([c11 + m6, c12], axis=1), lower


def _merge_top2(a, b):
    def ahead(v, i, w, j):
        return (v > w) | ((v == w) & (i < j))

    first = ahead(a[0], a[2], b[0], b[2])
    lose_v, lose_i = jnp.where(first, b[0], a[0]), jnp.where(first, b[2], a[2])
    next_v, next_i = jnp.where(first, a[1], b[1]), jnp.where(first, a[3], b[3])
    second = ahead(lose_v, lose_i, next_v, next_i)
    return (jnp.where(first, a[0], b[0]), jnp.where(second, lose_v, next_v),
            jnp.where(first, a[2], b[2]), jnp.where(second, lose_i, next_i))


def _pack(x):
    return pltpu.bitcast(x.astype(BF), I32)


def _unpack(x):
    return pltpu.bitcast(x, BF)


class _Order:
    def __init__(self, never):
        self.never = never
        self.link = None
        self.release = None

    def after(self, v):
        for dep in (self.link, self.release):
            if dep is not None:
                probe = self.never[:v.shape[0], :v.shape[1]]
                v = jnp.where(probe != probe, dep[:v.shape[0], :v.shape[1]], v)
        return v


def _kernel(x_hbm, wqkv_hbm, wphi_hbm, wo_hbm, wr_hbm, wg_hbm, wu_hbm, wd_hbm, c_hbm, wmod_hbm,
            out_hbm,
            x_v, wqkv_v, wphi_v, wo_v, wr_v, wg_v, wu_v, wd_v, c_v, wmod_v,
            wkv_c, wq_c, wo_c, hc_v, oc_v, x1_v, xn_v, kv_acc, z_acc, kvT, mod_v, sb_v, bias_v, slab_v, idle_sem,
            sems, osems, *, cfg):
    R1, R2, RB = cfg.get("R1", 16), cfg.get("R2", 16), cfg.get("RB", 32)

    def col(ref, j, w=D):
        return ref.at[:, pl.ds(j * w, w)]

    def x_copy(t):
        return ("x%d" % t, x_hbm.at[pl.ds(t * T, T)], x_v.at[pl.ds(t * T, T)])

    def w_copy(name, j, c):
        return ("%s%d" % (name, c), col(wqkv_hbm, j * NCH + c, 256), wqkv_v.at[j * NCH + c])

    def mod_copy(name, j):
        return (name, col(wmod_hbm, j), wmod_v.at[j, :, pl.ds(0, D)])

    def scale_copy(d, k):
        rows = pl.ds(k * DHALF, DHALF)
        return ("ca%d%d" % (d, k), wmod_hbm.at[rows, pl.ds(D + d * DHALF, DHALF)],
                wmod_v.at[1, rows, pl.ds(d * DHALF, DHALF)])

    order = [("c", c_hbm, c_v), x_copy(0), ("wphi", wphi_hbm, wphi_v),
             w_copy("wk", 1, 0), w_copy("wv", 2, 0), *[scale_copy(d, k) for d in range(2) for k in range(2)],
             w_copy("wk", 1, 1), w_copy("wv", 2, 1), w_copy("wk", 1, 2), w_copy("wv", 2, 2),
             w_copy("wk", 1, 3), w_copy("wv", 2, 3), x_copy(1), mod_copy("sa", 0), x_copy(2), x_copy(3)]
    order += [w_copy("wq", 0, c) for c in range(NCH)]
    order += [("wr", wr_hbm, wr_v), ("wo", wo_hbm, wo_v), mod_copy("ga", 2), mod_copy("sb", 3), mod_copy("cb", 4), mod_copy("gb", 5),
              ("wg", wg_hbm, wg_v), ("wu", wu_hbm, wu_v), ("wd", wd_hbm, wd_v.at[:, pl.ds(0, D)])]
    copies = {}
    for i, (name, src, dst) in enumerate(order):
        copies[name] = pltpu.make_async_copy(src, dst, sems.at[i])
        copies[name].start()

    waited, started = set(), []

    scope = []

    def mark(name):
        if cfg.get("marks"):
            if scope:
                scope.pop().__exit__(None, None, None)
            if name:
                scope.append(jax.named_scope(name))
                scope[0].__enter__()

    def wait(*names):
        mark("w_" + names[0])
        for name in names:
            copies[name].wait()
            waited.add(name)
        mark("r_" + names[0])


    wait("c", "x0")
    cf = c_v[...].astype(F32)
    never = jnp.broadcast_to(cf[:, 0:128], (32, 128))
    order1, order2, order3, order4 = [_Order(never) for _ in range(4)]
    sc = jnp.broadcast_to(cf * jax.nn.sigmoid(cf), (16, D)).astype(BF)

    def normalized(tok, n, order=None):
        xc, rs = _center(x_v[pl.ds(tok, n), :].astype(F32), order)
        return xc * rs

    for r0 in range(0, T, 32):
        xn_v[pl.ds(r0, 32), :] = normalized(r0, 32)

    wait("wphi")
    row = lax.broadcasted_iota(I32, (128, DH), 0)
    lane = lax.broadcasted_iota(I32, (128, DH), 1)
    expand = jnp.where(((row % 64) // 2) == lane, 1.0, 0.0).astype(BF)
    bdt = _dot(expand, wphi_v[...].reshape(H * DH, DH), NT)
    row = lax.broadcasted_iota(I32, (128, D), 0)
    lane = lax.broadcasted_iota(I32, (128, D), 1)
    bdt = jnp.where(2 * (row // 64) + (row % 2) == (lane % 128) // DH, bdt, 0.0).astype(BF)

    def mod_row(j):
        return _dot(sc, wmod_v[j, :, pl.ds(0, D)], NN)[0:8]

    def mod_part(j, n, half):
        part = _dot(sc[:, half * DHALF:(half + 1) * DHALF],
                    wmod_v[j, pl.ds(half * DHALF, DHALF), pl.ds(n * 128, 128)], NN)[0:8]
        if half == 0:
            mod_v[j, :, pl.ds(n * 128, 128)] = part
        else:
            mod_v[j, :, pl.ds(n * 128, 128)] += part

    for k0 in range(0, D, 128):
        sb_v[pl.ds(k0, 128), :] = jnp.broadcast_to(sc[0:1, k0:k0 + 128].astype(F32), (128, 128)).T

    partial_mod = {}

    def mod_piece(j, k0, nk):
        acc = partial_mod.pop(j, None)
        step = cfg.get("mstep", 16)
        for k in range(k0, k0 + nk, step):
            s_col = sb_v[pl.ds(k, step), :]
            if k == k0 and cfg.get("chain3"):
                s_col = order3.after(s_col)
            term = wmod_v[j, pl.ds(k, step), pl.ds(0, D)].astype(F32) * jnp.concatenate([s_col] * (D // 128), axis=1)
            if step == 16:
                term = term[0:8] + term[8:16]
            acc = term if acc is None else acc + term
        if cfg.get("chain3"):
            link = acc[:, 0:128]
            for _ in range(cfg["chain3"]):
                link = jnp.broadcast_to(jnp.max(link, axis=-1, keepdims=True), (8, 128))
            order3.link = jnp.concatenate([link, link], axis=0)
        if k0 + nk < D:
            partial_mod[j] = acc
        else:
            mod_v[j] = jnp.broadcast_to(jnp.sum(acc, axis=0, keepdims=True), (8, D))

    def finish_mod():
        wr = wr_v[...].astype(F32)
        wr_row = jnp.concatenate([jnp.broadcast_to(wr[j:j + 1, :], (8, 128)) for j in range(8)], axis=1)
        shift, scale, gate = mod_v[3], 1.0 + mod_v[4], mod_v[5]
        mod_v[4] = scale
        mod_v[6] = gate * scale
        mod_v[7] = gate * shift
        mod_v[8] = wr_row * scale
        mod_v[9] = jnp.broadcast_to(jnp.sum(wr_row * shift, axis=-1, keepdims=True), (8, D))

    def rows_of(j, n):
        return _tile8(mod_v[j], n // 8)

    def h_term(t, i, r0=0, n=TH):
        return (t, i // 2, pl.ds(r0, n), pl.ds((i % 2) * DHALF, DHALF))

    def store_h_terms(t, r0, n, a, b):
        h1, h2 = a * rows_of(1, n), b * rows_of(1, n)
        terms = _rhs_terms(h1[:, :DHALF], h2[:, :DHALF], h1[:, DHALF:], h2[:, DHALF:])
        for i, term in enumerate(terms):
            hc_v[h_term(t, i, r0, n)] = term.astype(BF)

    def ln1_piece(t, r0):
        second = order4 if t == 1 else order1
        store_h_terms(t, r0, R1, normalized(t * T + r0, R1, order1), normalized(t * T + TH + r0, R1, second))

    def store_lhs_terms(top, bot, dst, c, r0):
        terms = _lhs_terms(top[:, :DHALF], top[:, DHALF:], bot[:, :DHALF], bot[:, DHALF:])
        for i, term in enumerate(terms):
            if dst.dtype == I32:
                dst[c, i] = _pack(term)
            else:
                dst[c, i, pl.ds(r0, 128), :] = term.astype(BF)

    def shift_bias(dst, w, order):
        shift = jnp.concatenate([order.after(mod_v[0, :, l:l + 128]) for l in range(0, D, 128)], axis=1)
        b = jnp.sum(w * _tile8(shift, w.shape[0] // 8), axis=-1, keepdims=True)
        order.link = jnp.broadcast_to(b, (w.shape[0], 128))
        bias_v[pl.ds(dst, w.shape[0]), :] = order.link

    def kv_bias(r0):
        shift_bias(r0, x1_v[pl.ds(r0, RB), :], order2)

    def keep_weights(c, r0, halves):
        for g in range(2):
            x1_v[pl.ds(c * 512 + g * 256 + r0, 128), :] = halves[g]

    def folded(j, c):
        halves = []
        for g in range(2):
            w = wqkv_v[j * NCH + c, :, g * 128:(g + 1) * 128]
            gg = 2 * c + g
            halves.append(_dot(bdt[:, gg * 128:(gg + 1) * 128], w, NT) * LOG2E)
        return halves

    def prep_k(c):
        halves = folded(1, c)
        store_lhs_terms(halves[0], halves[1], wkv_c, c, 0)
        keep_weights(c, 0, halves)

    def prep_q(c):
        halves = folded(0, c)
        for r0 in range(0, 128, 16):
            top, bot = [jnp.concatenate([order2.after(half[r0:r0 + 16, l:l + 128]) for l in range(0, D, 128)], axis=1)
                        if g == 0 and cfg.get("pq", 1) else half[r0:r0 + 16] for g, half in enumerate(halves)]
            terms = _lhs_terms(top[:, :DHALF], top[:, DHALF:], bot[:, :DHALF], bot[:, DHALF:])
            for i, term in enumerate(terms):
                wq_c[c, i, pl.ds(r0 // 2, 8), :] = _pack(term)
            shift_bias(S + c * 256 + r0, top, _Order(never))
            shift_bias(S + c * 256 + 128 + r0, bot, order2 if cfg.get("pq", 1) else _Order(never))

    def prep_v(c):
        halves = [wqkv_v[2 * NCH + c, :, g * 128:(g + 1) * 128].T.astype(F32) for g in range(2)]
        store_lhs_terms(halves[0], halves[1], wkv_c, c, 128)
        keep_weights(c, 128, halves)

    def prep_wo(c, r0):
        def rows(r):
            w = wo_v[pl.ds(r, 16), :].astype(F32)
            return jnp.concatenate([order3.after(w[:, l:l + 128]) for l in range(0, D, 128)], axis=1)
        top, bot = rows(c * 256 + r0), wo_v[pl.ds(c * 256 + 128 + r0, 16), :].astype(F32)
        terms = _rhs_terms(top[:, :DHALF], top[:, DHALF:], bot[:, :DHALF], bot[:, DHALF:])
        for i, term in enumerate(terms):
            wo_c[i, pl.ds(c * 64 + r0 // 2, 8), :] = _pack(term)
        order3.link = jnp.broadcast_to(jnp.max(terms[0][:, 0:128], axis=-1, keepdims=True), (16, 128))

    stream = _Order(never)

    def behind_product(v):
        head = jnp.concatenate([stream.after(v[0:8, l:l + 128]) for l in range(0, T, 128)], axis=1)
        return jnp.concatenate([head, v[8:]], axis=0)

    def bias_rows(r0):
        return jnp.concatenate([bias_v[pl.ds(r0, 64), :]] * (T // 128), axis=1)

    def kv_pair(t, c, res, k):
        g, q = divmod(k, 2)
        pair = 4 * c + k
        r0 = c * 512 + g * 256 + q * 64
        phi = _hedgehog(res[g][q * 64:(q + 1) * 64] + bias_rows(r0))
        vt = behind_product(res[g][128 + q * 64:128 + (q + 1) * 64]).astype(BF)
        zs = phi[:, 0:128]
        for l in range(1, T // 128):
            zs = zs + phi[:, l * 128:(l + 1) * 128]
        kv = _dot(vt, phi.astype(BF), NT)
        if t > 0:
            zs = zs + z_acc[pair]
            kv = kv + kv_acc[pair]
        if t < NTILE - 1:
            z_acc[pair] = zs
            kv_acc[pair] = kv
        else:
            z = jnp.broadcast_to(jnp.sum(zs.T, axis=0, keepdims=True), (16, 128))
            kv = kv + bias_v[pl.ds(r0 + 128, 64), :] * _tile8(z[0:8], 8)
            row = lax.broadcasted_iota(I32, (80, 128), 0)
            lane = lax.broadcasted_iota(I32, (80, 128), 1)
            head = jnp.where(row < 64, row // DH, (row - 64) // 8)
            kvT[pair] = jnp.where(head == lane % 2, jnp.concatenate([kv, z], axis=0), 0.0).astype(BF)

    def q_pair(c, res, k):
        g, q = divmod(k, 2)
        pair = 4 * c + k
        even = (lax.broadcasted_iota(I32, (8, T), 0) % 2) == 0
        phi, scale = _hedgehog_scaled(res[g][q * 64:(q + 1) * 64] + bias_rows(S + pair * 64))
        if cfg.get("tq"):
            phi = behind_product(phi)
        nd = _dot(kvT[pair], phi.astype(BF), NN)
        swapped = pltpu.roll(scale, 1, 0)
        inv_a = _recip(nd[64:72] + 1e-6 * jnp.where(even, scale, swapped))
        inv_b = _recip(nd[72:80] + 1e-6 * jnp.where(even, swapped, scale))
        return nd[0:64] * jnp.concatenate([inv_a] * 4 + [inv_b] * 4, axis=0)

    held = {}

    def q_step(t, c, res, k):
        held[k] = q_pair(c, res, k)
        if k == 3:
            held["lower"] = jnp.concatenate([held.pop(2), held.pop(3)], axis=0).T
        if k == 1:
            o1, o2 = jnp.concatenate([held.pop(0), held.pop(1)], axis=0).T, held.pop("lower")
            for i, term in enumerate(_lhs_terms(o1[:TH], o2[:TH], o1[TH:], o2[TH:])):
                oc_v[t, i, :, pl.ds(c * 128, 128)] = term.astype(BF)

    def residual(tok, attn):
        rows = pl.ds(tok, 128)
        x1_v[rows, :] = x_v[rows, :].astype(F32) + rows_of(2, 128) * attn

    def block_out(x1, xc, rs):
        n = x1.shape[0]
        return xc * (rs * rows_of(6, n)) + (x1 + rows_of(7, n))

    def router(xc, rs):
        n = xc.shape[0]
        return jnp.sum(xc * rows_of(8, n), axis=-1, keepdims=True) * rs + rows_of(9, n)[:, 0:1]

    found = []

    def ln2_piece(tok, order):
        x1 = x1_v[pl.ds(tok, R2), :]
        xc, rs = _center(x1, order)
        t, r0 = divmod(tok, T)
        hc_v[t, r0 // TH, pl.ds(r0 % TH, R2), :] = block_out(x1, xc, rs).astype(BF)
        r = router(xc, rs)
        sub = lax.broadcasted_iota(I32, (8, 128), 0).astype(F32)
        ra, rb = jnp.broadcast_to(r[0:8], (8, 128)), jnp.broadcast_to(r[8:16], (8, 128))
        ia, ib = sub + float(tok), sub + float(tok + 8)
        first = ra >= rb
        found.append((jnp.where(first, ra, rb), jnp.where(first, rb, ra),
                      jnp.where(first, ia, ib), jnp.where(first, ib, ia)))
        if order is not None:
            found[:] = [_merge_top2(found[0], found[1])] if len(found) == 2 else found

    def out_copy(t, half):
        return pltpu.make_async_copy(hc_v.at[t, half], out_hbm.at[pl.ds(t * T + half * TH, TH)],
                                     osems.at[2 * t + half])

    def start_out(t):
        for half in range(2):
            out_copy(t, half).start()
        started.append(t)

    wait("wk0", "wv0")
    prep_k(0)
    prep_v(0)

    def first_terms(d, wanted):
        cols = pl.ds(d * DHALF, DHALF)
        scale = 1.0
        for k in range(2):
            wait("ca%d%d" % (d, k))
            scale = scale + _dot(sc[:, k * DHALF:(k + 1) * DHALF], wmod_v[1, pl.ds(k * DHALF, DHALF), cols], NN)[0:8]
        mod_v[1, :, cols] = scale

        def block(half, dd, r0):
            if dd > d:
                return None
            cc = pl.ds(dd * DHALF, DHALF)
            return xn_v[pl.ds(half * TH + r0, 64), cc] * _tile8(mod_v[1, :, cc], 8)

        for group in wanted:
            for r0 in range(0, TH, 64):
                b11, b12, b21, b22 = block(0, 0, r0), block(1, 0, r0), block(0, 1, r0), block(1, 1, r0)
                terms = _rhs_terms(b11, b12, b21, b22) if d else {1: b11, 5: b11 + b12}
                for i in group:
                    hc_v[h_term(0, i, r0, 64)] = terms[i].astype(BF)

    def kv_product(t, c, i):
        return _dot(wkv_c[c, i], hc_v[h_term(t, i)], NT)

    first_terms(0, ((1,), (5,)))
    head_start = {i: kv_product(0, 0, i) for i in (1, 5)}
    first_terms(1, cfg.get("tg", ((0,), (3, 2, 4, 6))))

    P = functools.partial

    def spread(slots, lo, hi, works):
        for n, work in enumerate(works):
            slots[lo + n * (hi - lo) // len(works)].append(work)

    steps = [("kv", t, c) for t in range(NTILE) for c in range(NCH)]
    steps += [("q", t, c) for t in range(NTILE) for c in range(NCH)]
    steps += [("o", t, s) for t in range(NTILE) for s in range(2)]
    if cfg.get("only"):
        steps = [steps[i] for i in cfg["only"]]
    mod_parts = [P(mod_part, j, n, half) for j in range(2, 6) for half in range(2) for n in range(8)]
    prev = None
    pending = []
    for step, (kind, t, c) in enumerate(steps):
        slots = [[] for _ in range(7)]
        lower_done = None
        if prev is not None:
            pkind, pt, pc, pres = prev
            if pkind == "kv":
                pending += [P(kv_pair, pt, pc, pres, k) for k in (2, 3, 0, 1)]
                n = len(pending) if cfg.get("only") or kind != "kv" else cfg["quota"][t * NCH + c]
                for slot in cfg["kslots"][n]:
                    slots[slot].append(pending.pop(0))
            elif pkind == "q":
                qs = cfg.get("qs", (0, 1, 3, 5))
                for slot, k in zip(qs, (2, 3, 0, 1)):
                    slots[slot].append(P(q_step, pt, pc, pres, k))
            else:
                tok = pt * T + pc * 128
                slots[0].append(P(residual, tok, pres[0]))
                lo, hi = cfg.get("l2a", (0, 4))
                group = _Order(never)
                spread(slots, lo, hi, [P(ln2_piece, tok + r0, group) for r0 in range(0, 128, R2)])
                if pc == 1:
                    slots[hi].append(P(start_out, pt))
        if kind == "kv":
            if t == 0 and c + 1 < NCH:
                names = (("wk1", "wv1"), ("wk2", "wv2", "wk3", "wv3"), ("x1",))[c]
                k = cfg["ws"][c]
                slots[k] += [P(wait, *names), P(prep_v, c + 1), P(prep_k, c + 1)]
            if (t, c) == (1, 0):
                slots[0] = [P(wait, "sa", "x2", "x3"), lambda: mod_v.__setitem__(0, mod_row(0))] + slots[0]
            if t == 1 and c < 2:
                for k in range(2):
                    first = (2 * c + k) * 512
                    at = cfg["bs"][c][k]
                    slots[at] += [P(kv_bias, r0) for r0 in range(first, first + 512, RB)]
            n = t * NCH + c - cfg["n0"]
            if n == 0:
                slots[0].insert(0, P(wait, "wq0", "wq1", "wq2", "wq3", "wr", "wo", "ga", "sb", "cb", "gb"))
                late = []
                for j in range(4):
                    for m in range(8):
                        k0 = m * 128
                        for nk in cfg["nks"]:
                            late.append(P(mod_piece, 2 + j, k0, nk))
                            k0 += nk
                        late.append(P(prep_wo, j, m * 16))
            if 0 <= n < NCH:
                slots[5].append(P(prep_q, n))
            if n >= 0:
                left = NTILE * NCH - cfg["n0"]
                spread(slots, 1, 7, late[n * len(late) // left:(n + 1) * len(late) // left])
        if (kind, t, c) == ("q", 0, 0):
            slots[0].insert(0, P(wait, "wg"))
            slots[6].append(finish_mod)
        if kind == "o":
            last = step == len(steps) - 1
            tok2 = t * T + TH + c * 128
            lower_done = P(residual, tok2)
            lo, hi = (5, 6) if last else cfg.get("l2b", (5, 7))
            group = _Order(never)
            spread(slots, lo, hi, [P(ln2_piece, tok2 + r0, None if last else group) for r0 in range(0, 128, R2)])

        def fill(k, m, slots=slots):
            stream.release = m
            for work in slots[k]:
                work()

        if kind == "kv":
            res = _block_product(lambda i: head_start.pop(i) if i in head_start else kv_product(t, c, i), fill)
        elif kind == "q":
            res = _block_product(lambda i: _dot(_unpack(wq_c[c, i]), hc_v[h_term(t, i)], NT), fill)
        else:
            res = _block_product(
                lambda i: _dot(oc_v[t, i, pl.ds(c * 128, 128), :], _unpack(wo_c[i]), NN), fill, lower_done)
        if kind == "kv" and c == NCH - 1:
            order1.link = None
        prev = (kind, t, c, res)

    if cfg.get("only"):
        for name in copies:
            if name not in waited:
                wait(name)
        a, b = prev[3]
        x1_v[0:128, 0:256] = a[0:128, 0:256] + b[0:128, 0:256] + a[0:128, 256:512] + b[0:128, 256:512]
        x1_v[128:136, 0:128] = sum(sum(f) for f in found) if found else jnp.zeros((8, 128), F32)
        z = pl.semaphore_read(idle_sem)
        x1_v[136:144, :] = mod_v[z]
        x1_v[144:160, 0:512] = oc_v[z, z, 0:16, :].astype(F32) + hc_v[z, z, 0:16, 0:512].astype(F32) + (
            wo_c[z, 0:16, :] + wq_c[z, z, 0:16, :] + wkv_c[z, z, 0:16, :]).astype(F32)
        x1_v[160:176, 0:128] = kvT[z, 0:16, :].astype(F32) + kv_acc[z, 0:16, :] + z_acc[z, 0:16, :]
        slab_v[0] = x1_v[pl.ds(pl.multiple_of(z * 16, 16), 16), :].astype(BF)
        cpy = pltpu.make_async_copy(slab_v.at[0], out_hbm.at[pl.ds(0, 16)], osems.at[0])
        cpy.start()
        cpy.wait()
        for t in started:
            out_copy(t, 0).wait()
            out_copy(t, 1).wait()
        return

    _, pt, pc, pres = prev
    tok = pt * T + pc * 128
    residual(tok, pres[0])
    for r0 in range(0, 128, R2):
        ln2_piece(tok + r0, None)
    start_out(pt)

    while len(found) > 1:
        found[:] = [_merge_top2(*found[k:k + 2]) if k + 1 < len(found) else found[k]
                    for k in range(0, len(found), 2)]
    m1, m2, i1, i2 = found[0]
    big = float(2 * S)
    best = jnp.max(m1, axis=0, keepdims=True)
    ia = jnp.min(jnp.where(m1 == best, i1, big), axis=0, keepdims=True)
    taken = i1 == ia
    cm = jnp.where(taken, m2, m1)
    ci = jnp.where(taken, i2, i1)
    second = jnp.max(cm, axis=0, keepdims=True)
    ib = jnp.min(jnp.where(cm == second, ci, big), axis=0, keepdims=True)
    idx_a = jnp.clip(ia.astype(I32)[0, 0], 0, S - 1)
    idx_b = jnp.clip(ib.astype(I32)[0, 0], 0, S - 1)

    sub = lax.broadcasted_iota(I32, (16, D), 0)
    xa = jnp.broadcast_to(x1_v[pl.ds(idx_a, 1), :], (16, D))
    xb = jnp.broadcast_to(x1_v[pl.ds(idx_b, 1), :], (16, D))
    xc, rs = _center(jnp.where(sub == 0, xa, xb))
    gate_r = jax.nn.sigmoid(router(xc, rs))
    hb = (xc * rs * rows_of(4, 16) + rows_of(3, 16)).astype(BF)
    wait("wu", "wd")
    for t in range(NTILE - 1):
        out_copy(t, 0).wait()
        out_copy(t, 1).wait()

    def slab(idx):
        start = pl.multiple_of((idx // 16) * 16, 16)
        x1 = x1_v[pl.ds(start, 16), :]
        return start, block_out(x1, *_center(x1))

    slabs = [slab(idx_a), slab(idx_b)]
    g = _dot(hb, wg_v[...], NN)
    u = _dot(hb, wu_v[...], NN)
    act = (g * jax.nn.sigmoid(g) * u).astype(BF)
    y = _dot(act, wd_v[:, pl.ds(0, D)], NN) * (gate_r * rows_of(5, 16))

    fixes = []
    for slot, (start, o) in enumerate(slabs):
        o = o + jnp.where(sub + start == idx_a, y[0:1], 0.0) + jnp.where(sub + start == idx_b, y[1:2], 0.0)
        slab_v[slot] = o.astype(BF)
        fixes.append(pltpu.make_async_copy(slab_v.at[slot], out_hbm.at[pl.ds(start, 16)], osems.at[slot]))
    out_copy(NTILE - 1, 0).wait()
    out_copy(NTILE - 1, 1).wait()
    fixes[0].start()

    @pl.when(idx_a // 16 != idx_b // 16)
    def _():
        fixes[1].start()
        fixes[1].wait()

    fixes[0].wait()
    mark(None)


def make(flags=None, **cfg):
    cfg = dict(dict(tie=False, vmod=32, chain3=1, ws=(3, 3, 2), n0=11, bs=((0, 2), (0, 2)),
                    quota=(0, 0, 0, 0, 2, 4, 6, 6, 6, 6, 6, 6, 6, 4, 4, 4),
                    kslots={0: (), 2: (4, 5), 3: (3, 4, 5), 4: (1, 2, 3, 4), 5: (1, 2, 3, 4, 5), 6: (0, 1, 2, 3, 4, 5)},
                    nks=(32, 32, 32, 32), mstep=8, ks=(1, 2, 3, 4)), **cfg)
    if cfg.get("ev", False):
        flags = dict(flags or {}, XLA_TPU_EVENLY_DISTRIBUTE_CRITICAL_NODES=True)
    pad = cfg.get("pad", 128)

    def run(A_x, A_wqkv, A_w_phi, A_wo, B_x, B_w_r, B_w_gate, B_w_up, B_w_down, c, w_mod):
        del B_x
        any_spec = pl.BlockSpec(memory_space=pl.ANY)
        scratch = [
            pltpu.VMEM((S, D), BF), pltpu.VMEM((3 * NCH, D, 256), BF), pltpu.VMEM((H, DH, DH), BF),
            pltpu.VMEM((D, D), BF), pltpu.VMEM((8, 128), BF),
            pltpu.VMEM((D, F), BF), pltpu.VMEM((D, F), BF), pltpu.VMEM((F, D + pad), BF),
            pltpu.VMEM((1, D), BF), pltpu.VMEM((6, D, D + pad), BF),
            pltpu.VMEM((NCH, 7, 256, DHALF), BF), pltpu.VMEM((NCH, 7, 64, DHALF), I32),
            pltpu.VMEM((7, DHALF // 2, DHALF), I32),
            pltpu.VMEM((NTILE, 4, TH, D), BF), pltpu.VMEM((NTILE, 7, TH, DHALF), BF), pltpu.VMEM((S, D), F32), pltpu.VMEM((T, D), F32),
            pltpu.VMEM((H // 2, 64, 128), F32), pltpu.VMEM((H // 2, 128, 128), F32),
            pltpu.VMEM((H // 2, 80, 128), BF),
            pltpu.VMEM((10, 8, D), F32), pltpu.VMEM((D, 128), F32), pltpu.VMEM((S + D, 128), F32), pltpu.VMEM((2, 16, D), BF), pltpu.SemaphoreType.REGULAR,
            pltpu.SemaphoreType.DMA((40,)), pltpu.SemaphoreType.DMA((2 * NTILE,)),
        ]
        out = pl.pallas_call(
            functools.partial(_kernel, cfg=cfg),
            out_shape=jax.ShapeDtypeStruct((S, D), BF),
            in_specs=[any_spec] * 10,
            out_specs=any_spec,
            scratch_shapes=scratch,
            compiler_params=pltpu.CompilerParams(vmem_limit_bytes=120 * 2**20, flags=flags),
            name="fused_block",
        )(A_x.reshape(S, D), A_wqkv, A_w_phi, A_wo, B_w_r.reshape(8, 128), B_w_gate, B_w_up, B_w_down, c, w_mod)
        return out.reshape(1, S, D)
    return run


_run = make(**dict())


@jax.jit
def pallas_adaLN_cond__linear_kernel_hedgehog__moe_arch_mod__prompt_kernel(
    A_x: jax.Array,
    A_wqkv: jax.Array,
    A_w_phi: jax.Array,
    A_wo: jax.Array,
    B_x: jax.Array,
    B_w_r: jax.Array,
    B_w_gate: jax.Array,
    B_w_up: jax.Array,
    B_w_down: jax.Array,
    c: jax.Array,
    w_mod: jax.Array,
):
    return _run(A_x, A_wqkv, A_w_phi, A_wo, B_x, B_w_r, B_w_gate, B_w_up, B_w_down, c, w_mod)
```

```python
import functools

import jax
import jax.numpy as jnp
from jax import lax
from jax.experimental import pallas as pl
from jax.experimental.pallas import tpu as pltpu

S, D, H, DH, F = 2048, 1024, 32, 32, 3584
T = 512
TH = T // 2
DHALF = D // 2
NTILE = S // T
NCH = D // 256
LOG2E = 1.4426950408889634
NN = (((1,), (0,)), ((), ()))
NT = (((1,), (1,)), ((), ()))
TN = (((0,), (0,)), ((), ()))
BF = jnp.bfloat16
F32 = jnp.float32
I32 = jnp.int32


def _dot(a, b, dims):
    return lax.dot_general(a, b, dims, preferred_element_type=F32)


def _recip(x):
    return pltpu.reciprocal(x, approx=False, full_range=False)


def _center(x, order=None):
    s = jnp.sum(x, axis=-1, keepdims=True)
    if order is not None:
        s = order.after(s)
    xc = x - s * (1.0 / D)
    rs = lax.rsqrt(jnp.sum(xc * xc, axis=-1, keepdims=True) * (1.0 / D) + 1e-5)
    if order is not None:
        order.link = rs
    return xc, rs


def _pair_reduce(x, op):
    r = x[0:8]
    for i in range(1, 8):
        r = op(r, x[8 * i:8 * i + 8])
    r = op(r, pltpu.roll(r, 4, 0))
    return op(r, pltpu.roll(r, 2, 0))


def _tile8(r, n):
    return jnp.concatenate([r] * n, axis=0)


def _hedgehog(p):
    mx = _tile8(_pair_reduce(p, jnp.maximum), 8)
    mn = _tile8(_pair_reduce(p, jnp.minimum), 8)
    ep = jnp.exp2(p - mx)
    en = jnp.exp2(mn - p)
    rp = _tile8(_recip(_pair_reduce(ep, jnp.add)), 8)
    rn = _tile8(_recip(_pair_reduce(en, jnp.add)), 8)
    return jnp.concatenate([ep * rp, en * rn], axis=0)


def _hedgehog_scaled(p):
    mx = _tile8(_pair_reduce(p, jnp.maximum), 8)
    mn = _tile8(_pair_reduce(p, jnp.minimum), 8)
    ep = jnp.exp2(p - mx)
    en = jnp.exp2(mn - p)
    sp = _pair_reduce(ep, jnp.add)
    ratio = _tile8(sp * _recip(_pair_reduce(en, jnp.add)), 8)
    return jnp.concatenate([ep, en * ratio], axis=0), sp


def _lhs_terms(a11, a12, a21, a22):
    return (a11 + a22, a21 + a22, a11, a22, a11 + a12, a21 - a11, a12 - a22)


def _rhs_terms(b11, b12, b21, b22):
    return (b11 + b22, b11, b12 - b22, b21 - b11, b22, b11 + b12, b21 + b22)


def _block_product(product, fill, lower_done=None):
    m0 = product(0)
    fill(0, m0)
    m1 = product(1)
    fill(1, m1)
    c22 = m0 - m1
    m3 = product(3)
    fill(2, m3)
    c21 = m1 + m3
    c11 = m0 + m3
    m2 = product(2)
    fill(3, m2)
    c22 = c22 + m2
    m5 = product(5)
    fill(4, m5)
    lower = jnp.concatenate([c21, c22 + m5], axis=1)
    if lower_done is not None:
        lower_done(lower)
    m4 = product(4)
    fill(5, m4)
    c12 = m2 + m4
    c11 = c11 - m4
    m6 = product(6)
    fill(6, m6)
    return jnp.concatenate([c11 + m6, c12], axis=1), lower


def _merge_top2(a, b):
    def ahead(v, i, w, j):
        return (v > w) | ((v == w) & (i < j))

    first = ahead(a[0], a[2], b[0], b[2])
    lose_v, lose_i = jnp.where(first, b[0], a[0]), jnp.where(first, b[2], a[2])
    next_v, next_i = jnp.where(first, a[1], b[1]), jnp.where(first, a[3], b[3])
    second = ahead(lose_v, lose_i, next_v, next_i)
    return (jnp.where(first, a[0], b[0]), jnp.where(second, lose_v, next_v),
            jnp.where(first, a[2], b[2]), jnp.where(second, lose_i, next_i))


def _pack(x):
    return pltpu.bitcast(x.astype(BF), I32)


def _unpack(x):
    return pltpu.bitcast(x, BF)


class _Order:
    def __init__(self, never):
        self.never = never
        self.link = None
        self.release = None

    def after(self, v):
        for dep in (self.link, self.release):
            if dep is not None:
                probe = self.never[:v.shape[0], :v.shape[1]]
                v = jnp.where(probe != probe, dep[:v.shape[0], :v.shape[1]], v)
        return v


def _kernel(x_hbm, wqkv_hbm, wphi_hbm, wo_hbm, wr_hbm, wg_hbm, wu_hbm, wd_hbm, c_hbm, wmod_hbm,
            out_hbm,
            x_v, wqkv_v, wphi_v, wo_v, wr_v, wg_v, wu_v, wd_v, c_v, wmod_v,
            wkv_c, wq_c, wo_c, hc_v, oc_v, x1_v, xn_v, kv_acc, z_acc, kvT, mod_v, sb_v, bias_v, slab_v, idle_sem,
            sems, osems, *, cfg):
    R1, R2, RB = cfg.get("R1", 16), cfg.get("R2", 16), cfg.get("RB", 32)

    def col(ref, j, w=D):
        return ref.at[:, pl.ds(j * w, w)]

    def x_copy(t):
        return ("x%d" % t, x_hbm.at[pl.ds(t * T, T)], x_v.at[pl.ds(t * T, T)])

    def w_copy(name, j, c):
        return ("%s%d" % (name, c), col(wqkv_hbm, j * NCH + c, 256), wqkv_v.at[j * NCH + c])

    def mod_copy(name, j):
        return (name, col(wmod_hbm, j), wmod_v.at[j, :, pl.ds(0, D)])

    def scale_copy(d, k):
        rows = pl.ds(k * DHALF, DHALF)
        return ("ca%d%d" % (d, k), wmod_hbm.at[rows, pl.ds(D + d * DHALF, DHALF)],
                wmod_v.at[1, rows, pl.ds(d * DHALF, DHALF)])

    order = [("c", c_hbm, c_v), x_copy(0), ("wphi", wphi_hbm, wphi_v),
             w_copy("wk", 1, 0), w_copy("wv", 2, 0), *[scale_copy(d, k) for d in range(2) for k in range(2)],
             w_copy("wk", 1, 1), w_copy("wv", 2, 1), w_copy("wk", 1, 2), w_copy("wv", 2, 2),
             w_copy("wk", 1, 3), w_copy("wv", 2, 3), x_copy(1), mod_copy("sa", 0), x_copy(2), x_copy(3)]
    order += [w_copy("wq", 0, c) for c in range(NCH)]
    order += [("wr", wr_hbm, wr_v), ("wo", wo_hbm, wo_v), mod_copy("ga", 2), mod_copy("sb", 3), mod_copy("cb", 4), mod_copy("gb", 5),
              ("wg", wg_hbm, wg_v), ("wu", wu_hbm, wu_v), ("wd", wd_hbm, wd_v.at[:, pl.ds(0, D)])]
    copies = {}
    for i, (name, src, dst) in enumerate(order):
        copies[name] = pltpu.make_async_copy(src, dst, sems.at[i])
        copies[name].start()

    waited, started = set(), []

    scope = []

    def mark(name):
        if cfg.get("marks"):
            if scope:
                scope.pop().__exit__(None, None, None)
            if name:
                scope.append(jax.named_scope(name))
                scope[0].__enter__()

    def wait(*names):
        mark("w_" + names[0])
        for name in names:
            copies[name].wait()
            waited.add(name)
        mark("r_" + names[0])


    wait("c", "x0")
    cf = c_v[...].astype(F32)
    never = jnp.broadcast_to(cf[:, 0:128], (32, 128))
    order1, order2, order3, order4 = [_Order(never) for _ in range(4)]
    sc = jnp.broadcast_to(cf * jax.nn.sigmoid(cf), (16, D)).astype(BF)

    def normalized(tok, n, order=None):
        xc, rs = _center(x_v[pl.ds(tok, n), :].astype(F32), order)
        return xc * rs

    for r0 in range(0, T, 32):
        xn_v[pl.ds(r0, 32), :] = normalized(r0, 32)

    wait("wphi")
    row = lax.broadcasted_iota(I32, (128, DH), 0)
    lane = lax.broadcasted_iota(I32, (128, DH), 1)
    expand = jnp.where(((row % 64) // 2) == lane, 1.0, 0.0).astype(BF)
    bdt = _dot(expand, wphi_v[...].reshape(H * DH, DH), NT)
    row = lax.broadcasted_iota(I32, (128, D), 0)
    lane = lax.broadcasted_iota(I32, (128, D), 1)
    bdt = jnp.where(2 * (row // 64) + (row % 2) == (lane % 128) // DH, bdt, 0.0).astype(BF)

    def mod_row(j):
        return _dot(sc, wmod_v[j, :, pl.ds(0, D)], NN)[0:8]

    def mod_part(j, n, half):
        part = _dot(sc[:, half * DHALF:(half + 1) * DHALF],
                    wmod_v[j, pl.ds(half * DHALF, DHALF), pl.ds(n * 128, 128)], NN)[0:8]
        if half == 0:
            mod_v[j, :, pl.ds(n * 128, 128)] = part
        else:
            mod_v[j, :, pl.ds(n * 128, 128)] += part

    for k0 in range(0, D, 128):
        sb_v[pl.ds(k0, 128), :] = jnp.broadcast_to(sc[0:1, k0:k0 + 128].astype(F32), (128, 128)).T

    partial_mod = {}

    def mod_piece(j, k0, nk):
        acc = partial_mod.pop(j, None)
        step = cfg.get("mstep", 16)
        for k in range(k0, k0 + nk, step):
            s_col = sb_v[pl.ds(k, step), :]
            if k == k0 and cfg.get("chain3"):
                s_col = order3.after(s_col)
            term = wmod_v[j, pl.ds(k, step), pl.ds(0, D)].astype(F32) * jnp.concatenate([s_col] * (D // 128), axis=1)
            if step == 16:
                term = term[0:8] + term[8:16]
            acc = term if acc is None else acc + term
        if cfg.get("chain3"):
            link = acc[:, 0:128]
            for _ in range(cfg["chain3"]):
                link = jnp.broadcast_to(jnp.max(link, axis=-1, keepdims=True), (8, 128))
            order3.link = jnp.concatenate([link, link], axis=0)
        if k0 + nk < D:
            partial_mod[j] = acc
        else:
            mod_v[j] = jnp.broadcast_to(jnp.sum(acc, axis=0, keepdims=True), (8, D))

    def finish_mod():
        wr = wr_v[...].astype(F32)
        wr_row = jnp.concatenate([jnp.broadcast_to(wr[j:j + 1, :], (8, 128)) for j in range(8)], axis=1)
        shift, scale, gate = mod_v[3], 1.0 + mod_v[4], mod_v[5]
        mod_v[4] = scale
        mod_v[6] = gate * scale
        mod_v[7] = gate * shift
        mod_v[8] = wr_row * scale
        mod_v[9] = jnp.broadcast_to(jnp.sum(wr_row * shift, axis=-1, keepdims=True), (8, D))

    def rows_of(j, n):
        return _tile8(mod_v[j], n // 8)

    VW, VO, VH = cfg.get("vw", 1), cfg.get("vo", 1), cfg.get("vh", 1)
    pieces = {}

    def put(key, value):
        pieces.setdefault(key, []).append(value.astype(BF))

    def get(key, axis=0):
        return jnp.concatenate(pieces[key], axis=axis)

    def h_term(t, i, r0=0, n=TH):
        return (t, i // 2, pl.ds(r0, n), pl.ds((i % 2) * DHALF, DHALF))

    def store_h_terms(t, r0, n, a, b):
        h1, h2 = a * rows_of(1, n), b * rows_of(1, n)
        terms = _rhs_terms(h1[:, :DHALF], h2[:, :DHALF], h1[:, DHALF:], h2[:, DHALF:])
        for i, term in enumerate(terms):
            if VH:
                put(("h", t, i), term)
            else:
                hc_v[h_term(t, i, r0, n)] = term.astype(BF)

    def ln1_piece(t, r0):
        second = order4 if t == 1 else order1
        store_h_terms(t, r0, R1, normalized(t * T + r0, R1, order1), normalized(t * T + TH + r0, R1, second))

    def store_lhs_terms(top, bot, dst, c, r0):
        terms = _lhs_terms(top[:, :DHALF], top[:, DHALF:], bot[:, :DHALF], bot[:, DHALF:])
        for i, term in enumerate(terms):
            if VW:
                put(("w", c, i, r0), term)
            else:
                dst[c, i, pl.ds(r0, 128), :] = term.astype(BF)

    def shift_bias(dst, w, order):
        shift = jnp.concatenate([order.after(mod_v[0, :, l:l + 128]) for l in range(0, D, 128)], axis=1)
        b = jnp.sum(w * _tile8(shift, w.shape[0] // 8), axis=-1, keepdims=True)
        order.link = jnp.broadcast_to(b, (w.shape[0], 128))
        bias_v[pl.ds(dst, w.shape[0]), :] = order.link

    def kv_bias(r0):
        shift_bias(r0, x1_v[pl.ds(r0, RB), :], order2)

    def keep_weights(c, r0, halves):
        for g in range(2):
            x1_v[pl.ds(c * 512 + g * 256 + r0, 128), :] = halves[g]

    def folded(j, c):
        halves = []
        for g in range(2):
            w = wqkv_v[j * NCH + c, :, g * 128:(g + 1) * 128]
            gg = 2 * c + g
            halves.append(_dot(bdt[:, gg * 128:(gg + 1) * 128], w, NT) * LOG2E)
        return halves

    def prep_k(c):
        halves = folded(1, c)
        store_lhs_terms(halves[0], halves[1], wkv_c, c, 0)
        keep_weights(c, 0, halves)

    def prep_q(c):
        halves = folded(0, c)
        for r0 in range(0, 128, 16):
            top, bot = [jnp.concatenate([order2.after(half[r0:r0 + 16, l:l + 128]) for l in range(0, D, 128)], axis=1)
                        if g == 0 and cfg.get("pq", 1) else half[r0:r0 + 16] for g, half in enumerate(halves)]
            terms = _lhs_terms(top[:, :DHALF], top[:, DHALF:], bot[:, :DHALF], bot[:, DHALF:])
            for i, term in enumerate(terms):
                if VW:
                    put(("q", c, i), term)
                else:
                    wq_c[c, i, pl.ds(r0 // 2, 8), :] = _pack(term)
            shift_bias(S + c * 256 + r0, top, _Order(never))
            shift_bias(S + c * 256 + 128 + r0, bot, order2 if cfg.get("pq", 1) else _Order(never))

    def prep_v(c):
        halves = [wqkv_v[2 * NCH + c, :, g * 128:(g + 1) * 128].T.astype(F32) for g in range(2)]
        store_lhs_terms(halves[0], halves[1], wkv_c, c, 128)
        keep_weights(c, 128, halves)

    def prep_wo(c, r0):
        def rows(r):
            w = wo_v[pl.ds(r, 16), :].astype(F32)
            return jnp.concatenate([order3.after(w[:, l:l + 128]) for l in range(0, D, 128)], axis=1)
        top, bot = rows(c * 256 + r0), wo_v[pl.ds(c * 256 + 128 + r0, 16), :].astype(F32)
        terms = _rhs_terms(top[:, :DHALF], top[:, DHALF:], bot[:, :DHALF], bot[:, DHALF:])
        for i, term in enumerate(terms):
            if VW:
                put(("wo", i), term)
            else:
                wo_c[i, pl.ds(c * 64 + r0 // 2, 8), :] = _pack(term)
        order3.link = jnp.broadcast_to(jnp.max(terms[0][:, 0:128], axis=-1, keepdims=True), (16, 128))

    stream = _Order(never)

    def behind_product(v):
        head = jnp.concatenate([stream.after(v[0:8, l:l + 128]) for l in range(0, T, 128)], axis=1)
        return jnp.concatenate([head, v[8:]], axis=0)

    def bias_rows(r0):
        return jnp.concatenate([bias_v[pl.ds(r0, 64), :]] * (T // 128), axis=1)

    def kv_pair(t, c, res, k):
        g, q = divmod(k, 2)
        pair = 4 * c + k
        r0 = c * 512 + g * 256 + q * 64
        phi = _hedgehog(res[g][q * 64:(q + 1) * 64] + bias_rows(r0))
        vt = behind_product(res[g][128 + q * 64:128 + (q + 1) * 64]).astype(BF)
        zs = phi[:, 0:128]
        for l in range(1, T // 128):
            zs = zs + phi[:, l * 128:(l + 1) * 128]
        kv = _dot(vt, phi.astype(BF), NT)
        if t > 0:
            zs = zs + z_acc[pair]
            kv = kv + kv_acc[pair]
        if t < NTILE - 1:
            z_acc[pair] = zs
            kv_acc[pair] = kv
        else:
            z = jnp.broadcast_to(jnp.sum(zs.T, axis=0, keepdims=True), (16, 128))
            kv = kv + bias_v[pl.ds(r0 + 128, 64), :] * _tile8(z[0:8], 8)
            row = lax.broadcasted_iota(I32, (80, 128), 0)
            lane = lax.broadcasted_iota(I32, (80, 128), 1)
            head = jnp.where(row < 64, row // DH, (row - 64) // 8)
            kvT[pair] = jnp.where(head == lane % 2, jnp.concatenate([kv, z], axis=0), 0.0).astype(BF)

    def q_pair(c, res, k):
        g, q = divmod(k, 2)
        pair = 4 * c + k
        even = (lax.broadcasted_iota(I32, (8, T), 0) % 2) == 0
        phi, scale = _hedgehog_scaled(res[g][q * 64:(q + 1) * 64] + bias_rows(S + pair * 64))
        if cfg.get("tq"):
            phi = behind_product(phi)
        nd = _dot(kvT[pair], phi.astype(BF), NN)
        swapped = pltpu.roll(scale, 1, 0)
        inv_a = _recip(nd[64:72] + 1e-6 * jnp.where(even, scale, swapped))
        inv_b = _recip(nd[72:80] + 1e-6 * jnp.where(even, swapped, scale))
        return nd[0:64] * jnp.concatenate([inv_a] * 4 + [inv_b] * 4, axis=0)

    held = {}

    def q_step(t, c, res, k):
        held[k] = q_pair(c, res, k)
        if k == 3:
            held["lower"] = jnp.concatenate([held.pop(2), held.pop(3)], axis=0).T
        if k == 1:
            o1, o2 = jnp.concatenate([held.pop(0), held.pop(1)], axis=0).T, held.pop("lower")
            for i, term in enumerate(_lhs_terms(o1[:TH], o2[:TH], o1[TH:], o2[TH:])):
                if VO:
                    put(("o", t, i), term)
                else:
                    oc_v[t, i, :, pl.ds(c * 128, 128)] = term.astype(BF)

    def residual(tok, attn):
        rows = pl.ds(tok, attn.shape[0])
        x1_v[rows, :] = x_v[rows, :].astype(F32) + rows_of(2, attn.shape[0]) * attn

    def block_out(x1, xc, rs):
        n = x1.shape[0]
        return xc * (rs * rows_of(6, n)) + (x1 + rows_of(7, n))

    def router(xc, rs):
        n = xc.shape[0]
        return jnp.sum(xc * rows_of(8, n), axis=-1, keepdims=True) * rs + rows_of(9, n)[:, 0:1]

    found = []

    def ln2_piece(tok, order):
        x1 = x1_v[pl.ds(tok, R2), :]
        xc, rs = _center(x1, order)
        t, r0 = divmod(tok, T)
        hc_v[t, r0 // TH, pl.ds(r0 % TH, R2), :] = block_out(x1, xc, rs).astype(BF)
        r = router(xc, rs)
        sub = lax.broadcasted_iota(I32, (8, 128), 0).astype(F32)
        ra, rb = jnp.broadcast_to(r[0:8], (8, 128)), jnp.broadcast_to(r[8:16], (8, 128))
        ia, ib = sub + float(tok), sub + float(tok + 8)
        first = ra >= rb
        found.append((jnp.where(first, ra, rb), jnp.where(first, rb, ra),
                      jnp.where(first, ia, ib), jnp.where(first, ib, ia)))
        if order is not None:
            found[:] = [_merge_top2(found[0], found[1])] if len(found) == 2 else found

    def out_copy(t, half):
        return pltpu.make_async_copy(hc_v.at[t, half], out_hbm.at[pl.ds(t * T + half * TH, TH)],
                                     osems.at[2 * t + half])

    def start_out(t):
        for half in range(2):
            out_copy(t, half).start()
        started.append(t)

    wait("wk0", "wv0")
    prep_k(0)
    prep_v(0)

    def first_terms(d, wanted):
        cols = pl.ds(d * DHALF, DHALF)
        scale = 1.0
        for k in range(2):
            wait("ca%d%d" % (d, k))
            scale = scale + _dot(sc[:, k * DHALF:(k + 1) * DHALF], wmod_v[1, pl.ds(k * DHALF, DHALF), cols], NN)[0:8]
        mod_v[1, :, cols] = scale

        def block(half, dd, r0):
            if dd > d:
                return None
            cc = pl.ds(dd * DHALF, DHALF)
            return xn_v[pl.ds(half * TH + r0, 64), cc] * _tile8(mod_v[1, :, cc], 8)

        for group in wanted:
            for r0 in range(0, TH, 64):
                b11, b12, b21, b22 = block(0, 0, r0), block(1, 0, r0), block(0, 1, r0), block(1, 1, r0)
                terms = _rhs_terms(b11, b12, b21, b22) if d else {1: b11, 5: b11 + b12}
                for i in group:
                    if VH:
                        put(("h", 0, i), terms[i])
                    else:
                        hc_v[h_term(0, i, r0, 64)] = terms[i].astype(BF)

    def h_operand(t, i):
        return get(("h", t, i)) if VH else hc_v[h_term(t, i)]

    def kv_product(t, c, i, part=None):
        rows = pl.ds(0, 256) if part is None else pl.ds(part * 128, 128)
        w = jnp.concatenate([get(("w", c, i, 0)), get(("w", c, i, 128))], axis=0) if VW else wkv_c[c, i, rows, :]
        return _dot(w, h_operand(t, i), NT)

    first_terms(0, ((1,), (5,)))
    head_start = {i: kv_product(0, 0, i) for i in (1, 5)}
    first_terms(1, cfg.get("tg", ((0,), (3, 2, 4, 6))))

    P = functools.partial

    def spread(slots, lo, hi, works):
        for n, work in enumerate(works):
            slots[lo + n * (hi - lo) // len(works)].append(work)

    steps = [("kv", t, c) for t in range(NTILE) for c in range(NCH)]
    steps += [("q", t, c) for t in range(NTILE) for c in range(NCH)]
    for t, sizes in enumerate(cfg["osplit"]):
        steps += [("o", t, (sum(sizes[:k]), n)) for k, n in enumerate(sizes)]
    if cfg.get("only"):
        steps = [steps[i] for i in cfg["only"]]
    mod_parts = [P(mod_part, j, n, half) for j in range(2, 6) for half in range(2) for n in range(8)]
    prev = None
    pending = []
    for step, (kind, t, c) in enumerate(steps):
        slots = [[] for _ in range(7)]
        lower_done = None
        if prev is not None:
            pkind, pt, pc, pres = prev
            if pkind == "kv":
                pending += [P(kv_pair, pt, pc, pres, k) for k in (2, 3, 0, 1)]
                n = len(pending) if cfg.get("only") or kind != "kv" else cfg["quota"][t * NCH + c]
                for slot in cfg["kslots"][n]:
                    slots[slot].append(pending.pop(0))
            elif pkind == "q":
                qs = cfg.get("qs", (0, 1, 3, 5))
                for slot, k in zip(qs, (2, 3, 0, 1)):
                    slots[slot].append(P(q_step, pt, pc, pres, k))
            else:
                tok = pt * T + pc[0]
                slots[0].append(P(residual, tok, pres[0]))
                lo, hi = cfg.get("l2a", (0, 4))
                group = _Order(never)
                spread(slots, lo, hi, [P(ln2_piece, tok + r0, group) for r0 in range(0, pc[1], R2)])
                if sum(pc) == TH:
                    slots[hi].append(P(start_out, pt))
        if kind == "kv":
            if t == 0 and c + 1 < NCH:
                names = (("wk1", "wv1"), ("wk2", "wv2", "wk3", "wv3"), ("x1",))[c]
                k = cfg["ws"][c]
                slots[k] += [P(wait, *names), P(prep_v, c + 1), P(prep_k, c + 1)]
            if (t, c) == (1, 0):
                slots[0] = [P(wait, "sa", "x2", "x3"), lambda: mod_v.__setitem__(0, mod_row(0))] + slots[0]
            if t == 1 and c < 2:
                for k in range(2):
                    first = (2 * c + k) * 512
                    at = cfg["bs"][c][k]
                    slots[at] += [P(kv_bias, r0) for r0 in range(first, first + 512, RB)]
            if t + 1 < NTILE:
                chunks = ((2, 3), (0, 1, 2, 3), (0, 1, 2, 3))[t]
                if c in chunks:
                    rows = list(range(0, TH, R1))
                    k = chunks.index(c)
                    mine = rows[k * len(rows) // len(chunks):(k + 1) * len(rows) // len(chunks)]
                    spread(slots, cfg["ws"][2] + 1 if (t, c) == (0, 2) else 0, 6, [P(ln1_piece, t + 1, r0) for r0 in mine])
            n = t * NCH + c - cfg["n0"]
            if n == 0:
                slots[0].insert(0, P(wait, "wq0", "wq1", "wq2", "wq3", "wr", "wo", "ga", "sb", "cb", "gb"))
                late = []
                for j in range(4):
                    for m in range(8):
                        k0 = m * 128
                        for nk in cfg["nks"]:
                            late.append(P(mod_piece, 2 + j, k0, nk))
                            k0 += nk
                        late.append(P(prep_wo, j, m * 16))
            if 0 <= n < NCH:
                slots[5].append(P(prep_q, n))
            if n >= 0:
                left = NTILE * NCH - cfg["n0"]
                spread(slots, 1, 7, late[n * len(late) // left:(n + 1) * len(late) // left])
        if (kind, t, c) == ("q", 0, 0):
            slots[0].insert(0, P(wait, "wg"))
            slots[6].append(finish_mod)
        if kind == "o":
            last = step == len(steps) - 1
            tok2 = t * T + TH + c[0]
            lower_done = P(residual, tok2)
            lo, hi = (5, 6) if last else cfg.get("l2b", (5, 7))
            group = _Order(never)
            spread(slots, lo, hi, [P(ln2_piece, tok2 + r0, None if last else group) for r0 in range(0, c[1], R2)])

        def fill(k, m, slots=slots):
            stream.release = m
            for work in slots[k]:
                work()

        if kind == "kv":
            if cfg.get("ksplit") and (t, c) != (0, 0):
                halves = [_block_product(P(kv_product, t, c, part=part),
                                         lambda k, m, part=part: fill((7 * part + k) // 2, m) if (7 * part + k) % 2 else None)
                          for part in range(2)]
                res = [jnp.concatenate([halves[0][g], halves[1][g]], axis=0) for g in range(2)]
            else:
                res = _block_product(lambda i: head_start.pop(i) if i in head_start else kv_product(t, c, i), fill)
        elif kind == "q":
            res = _block_product(lambda i: _dot(get(("q", c, i)) if VW else _unpack(wq_c[c, i]), h_operand(t, i), NT), fill)
        else:
            res = _block_product(
                lambda i: _dot(get(("o", t, i), 1)[c[0]:sum(c)] if VO else oc_v[t, i, pl.ds(*c), :],
                               get(("wo", i)) if VW else _unpack(wo_c[i]), NN), fill, lower_done)
        if kind == "kv" and c == NCH - 1:
            order1.link = None
        prev = (kind, t, c, res)

    if cfg.get("only"):
        for name in copies:
            if name not in waited:
                wait(name)
        a, b = prev[3]
        x1_v[0:128, 0:256] = a[0:128, 0:256] + b[0:128, 0:256] + a[0:128, 256:512] + b[0:128, 256:512]
        x1_v[128:136, 0:128] = sum(sum(f) for f in found) if found else jnp.zeros((8, 128), F32)
        z = pl.semaphore_read(idle_sem)
        x1_v[136:144, :] = mod_v[z]
        x1_v[144:160, 0:512] = oc_v[z, z, 0:16, :].astype(F32) + hc_v[z, z, 0:16, 0:512].astype(F32) + (
            wo_c[z, 0:16, :] + wq_c[z, z, 0:16, :] + wkv_c[z, z, 0:16, :]).astype(F32)
        x1_v[160:176, 0:128] = kvT[z, 0:16, :].astype(F32) + kv_acc[z, 0:16, :] + z_acc[z, 0:16, :]
        slab_v[0] = x1_v[pl.ds(pl.multiple_of(z * 16, 16), 16), :].astype(BF)
        cpy = pltpu.make_async_copy(slab_v.at[0], out_hbm.at[pl.ds(0, 16)], osems.at[0])
        cpy.start()
        cpy.wait()
        for t in started:
            out_copy(t, 0).wait()
            out_copy(t, 1).wait()
        return

    _, pt, pc, pres = prev
    tok = pt * T + pc[0]
    residual(tok, pres[0])
    for r0 in range(0, pc[1], R2):
        ln2_piece(tok + r0, None)
    start_out(pt)

    while len(found) > 1:
        found[:] = [_merge_top2(*found[k:k + 2]) if k + 1 < len(found) else found[k]
                    for k in range(0, len(found), 2)]
    m1, m2, i1, i2 = found[0]
    big = float(2 * S)
    best = jnp.max(m1, axis=0, keepdims=True)
    ia = jnp.min(jnp.where(m1 == best, i1, big), axis=0, keepdims=True)
    taken = i1 == ia
    cm = jnp.where(taken, m2, m1)
    ci = jnp.where(taken, i2, i1)
    second = jnp.max(cm, axis=0, keepdims=True)
    ib = jnp.min(jnp.where(cm == second, ci, big), axis=0, keepdims=True)
    idx_a = jnp.clip(ia.astype(I32)[0, 0], 0, S - 1)
    idx_b = jnp.clip(ib.astype(I32)[0, 0], 0, S - 1)

    sub = lax.broadcasted_iota(I32, (16, D), 0)
    xa = jnp.broadcast_to(x1_v[pl.ds(idx_a, 1), :], (16, D))
    xb = jnp.broadcast_to(x1_v[pl.ds(idx_b, 1), :], (16, D))
    xc, rs = _center(jnp.where(sub == 0, xa, xb))
    gate_r = jax.nn.sigmoid(router(xc, rs))
    hb = (xc * rs * rows_of(4, 16) + rows_of(3, 16)).astype(BF)
    wait("wu", "wd")
    for t in range(NTILE - 1):
        out_copy(t, 0).wait()
        out_copy(t, 1).wait()

    def slab(idx):
        start = pl.multiple_of((idx // 16) * 16, 16)
        x1 = x1_v[pl.ds(start, 16), :]
        return start, block_out(x1, *_center(x1))

    slabs = [slab(idx_a), slab(idx_b)]
    g = _dot(hb, wg_v[...], NN)
    u = _dot(hb, wu_v[...], NN)
    act = (g * jax.nn.sigmoid(g) * u).astype(BF)
    y = _dot(act, wd_v[:, pl.ds(0, D)], NN) * (gate_r * rows_of(5, 16))

    fixes = []
    for slot, (start, o) in enumerate(slabs):
        o = o + jnp.where(sub + start == idx_a, y[0:1], 0.0) + jnp.where(sub + start == idx_b, y[1:2], 0.0)
        slab_v[slot] = o.astype(BF)
        fixes.append(pltpu.make_async_copy(slab_v.at[slot], out_hbm.at[pl.ds(start, 16)], osems.at[slot]))
    out_copy(NTILE - 1, 0).wait()
    out_copy(NTILE - 1, 1).wait()
    fixes[0].start()

    @pl.when(idx_a // 16 != idx_b // 16)
    def _():
        fixes[1].start()
        fixes[1].wait()

    fixes[0].wait()
    mark(None)


def make(flags=None, **cfg):
    cfg = dict(dict(tie=False, vmod=32, chain3=1, ws=(3, 3, 2), osplit=((64,) * 4,) * 4, n0=10, bs=((1, 4), (0, 3)), RB=64, ev=1,
                    quota=(0, 0, 0, 0, 0, 3, 6, 6, 6, 6, 6, 6, 6, 5, 5, 5),
                    kslots={0: (), 2: (4, 5), 3: (3, 4, 5), 4: (1, 2, 3, 4), 5: (1, 2, 3, 4, 5), 6: (0, 1, 2, 3, 4, 5)},
                    nks=(32, 32, 32, 32), mstep=8, ks=(1, 2, 3, 4)), **cfg)
    if cfg.get("ev", False):
        flags = dict(flags or {}, XLA_TPU_EVENLY_DISTRIBUTE_CRITICAL_NODES=True)
    pad = cfg.get("pad", 128)

    def run(A_x, A_wqkv, A_w_phi, A_wo, B_x, B_w_r, B_w_gate, B_w_up, B_w_down, c, w_mod):
        del B_x
        any_spec = pl.BlockSpec(memory_space=pl.ANY)
        scratch = [
            pltpu.VMEM((S, D), BF), pltpu.VMEM((3 * NCH, D, 256), BF), pltpu.VMEM((H, DH, DH), BF),
            pltpu.VMEM((D, D), BF), pltpu.VMEM((8, 128), BF),
            pltpu.VMEM((D, F), BF), pltpu.VMEM((D, F), BF), pltpu.VMEM((F, D + pad), BF),
            pltpu.VMEM((1, D), BF), pltpu.VMEM((6, D, D + pad), BF),
            *([pltpu.VMEM((8, 128), I32)] * 3 if cfg.get("vw", 1) else [
                pltpu.VMEM((NCH, 7, 256, DHALF), BF), pltpu.VMEM((NCH, 7, 64, DHALF), I32),
                pltpu.VMEM((7, DHALF // 2, DHALF), I32)]),
            pltpu.VMEM((NTILE, 2 if cfg.get("vh", 1) else 4, TH, D), BF),
            pltpu.VMEM((8, 128) if cfg.get("vo", 1) else (NTILE, 7, TH, DHALF), BF), pltpu.VMEM((S, D), F32), pltpu.VMEM((T, D), F32),
            pltpu.VMEM((H // 2, 64, 128), F32), pltpu.VMEM((H // 2, 128, 128), F32),
            pltpu.VMEM((H // 2, 80, 128), BF),
            pltpu.VMEM((10, 8, D), F32), pltpu.VMEM((D, 128), F32), pltpu.VMEM((S + D, 128), F32), pltpu.VMEM((2, 16, D), BF), pltpu.SemaphoreType.REGULAR,
            pltpu.SemaphoreType.DMA((40,)), pltpu.SemaphoreType.DMA((2 * NTILE,)),
        ]
        out = pl.pallas_call(
            functools.partial(_kernel, cfg=cfg),
            out_shape=jax.ShapeDtypeStruct((S, D), BF),
            in_specs=[any_spec] * 10,
            out_specs=any_spec,
            scratch_shapes=scratch,
            compiler_params=pltpu.CompilerParams(vmem_limit_bytes=120 * 2**20, flags=flags),
            name="fused_block",
        )(A_x.reshape(S, D), A_wqkv, A_w_phi, A_wo, B_w_r.reshape(8, 128), B_w_gate, B_w_up, B_w_down, c, w_mod)
        return out.reshape(1, S, D)
    return run


_run = make(**dict())


@jax.jit
def pallas_adaLN_cond__linear_kernel_hedgehog__moe_arch_mod__prompt_kernel(
    A_x: jax.Array,
    A_wqkv: jax.Array,
    A_w_phi: jax.Array,
    A_wo: jax.Array,
    B_x: jax.Array,
    B_w_r: jax.Array,
    B_w_gate: jax.Array,
    B_w_up: jax.Array,
    B_w_down: jax.Array,
    c: jax.Array,
    w_mod: jax.Array,
):
    return _run(A_x, A_wqkv, A_w_phi, A_wo, B_x, B_w_r, B_w_gate, B_w_up, B_w_down, c, w_mod)
```

```python
import functools

import jax
import jax.numpy as jnp
from jax import lax
from jax.experimental import pallas as pl
from jax.experimental.pallas import tpu as pltpu

S, D, H, DH, F = 2048, 1024, 32, 32, 3584
T = 512
TH = T // 2
DHALF = D // 2
NTILE = S // T
NCH = D // 256
LOG2E = 1.4426950408889634
NN = (((1,), (0,)), ((), ()))
NT = (((1,), (1,)), ((), ()))
TN = (((0,), (0,)), ((), ()))
BF = jnp.bfloat16
F32 = jnp.float32
I32 = jnp.int32


def _dot(a, b, dims):
    return lax.dot_general(a, b, dims, preferred_element_type=F32)


def _recip(x):
    return pltpu.reciprocal(x, approx=False, full_range=False)


def _center(x, order=None):
    s = jnp.sum(x, axis=-1, keepdims=True)
    if order is not None:
        s = order.after(s)
    xc = x - s * (1.0 / D)
    rs = lax.rsqrt(jnp.sum(xc * xc, axis=-1, keepdims=True) * (1.0 / D) + 1e-5)
    if order is not None:
        order.link = rs
    return xc, rs


def _pair_reduce(x, op):
    r = x[0:8]
    for i in range(1, 8):
        r = op(r, x[8 * i:8 * i + 8])
    r = op(r, pltpu.roll(r, 4, 0))
    return op(r, pltpu.roll(r, 2, 0))


def _tile8(r, n):
    return jnp.concatenate([r] * n, axis=0)


def _hedgehog(p):
    mx = _tile8(_pair_reduce(p, jnp.maximum), 8)
    mn = _tile8(_pair_reduce(p, jnp.minimum), 8)
    ep = jnp.exp2(p - mx)
    en = jnp.exp2(mn - p)
    rp = _tile8(_recip(_pair_reduce(ep, jnp.add)), 8)
    rn = _tile8(_recip(_pair_reduce(en, jnp.add)), 8)
    return jnp.concatenate([ep * rp, en * rn], axis=0)


def _hedgehog_scaled(p):
    mx = _tile8(_pair_reduce(p, jnp.maximum), 8)
    mn = _tile8(_pair_reduce(p, jnp.minimum), 8)
    ep = jnp.exp2(p - mx)
    en = jnp.exp2(mn - p)
    sp = _pair_reduce(ep, jnp.add)
    ratio = _tile8(sp * _recip(_pair_reduce(en, jnp.add)), 8)
    return jnp.concatenate([ep, en * ratio], axis=0), sp


def _lhs_terms(a11, a12, a21, a22):
    return (a11 + a22, a21 + a22, a11, a22, a11 + a12, a21 - a11, a12 - a22)


def _rhs_terms(b11, b12, b21, b22):
    return (b11 + b22, b11, b12 - b22, b21 - b11, b22, b11 + b12, b21 + b22)


def _block_product(product, fill, lower_done=None):
    m0 = product(0)
    fill(0, m0)
    m1 = product(1)
    fill(1, m1)
    c22 = m0 - m1
    m3 = product(3)
    fill(2, m3)
    c21 = m1 + m3
    c11 = m0 + m3
    m2 = product(2)
    fill(3, m2)
    c22 = c22 + m2
    m5 = product(5)
    fill(4, m5)
    lower = jnp.concatenate([c21, c22 + m5], axis=1)
    if lower_done is not None:
        lower_done(lower)
    m4 = product(4)
    fill(5, m4)
    c12 = m2 + m4
    c11 = c11 - m4
    m6 = product(6)
    fill(6, m6)
    return jnp.concatenate([c11 + m6, c12], axis=1), lower


def _merge_top2(a, b):
    def ahead(v, i, w, j):
        return (v > w) | ((v == w) & (i < j))

    first = ahead(a[0], a[2], b[0], b[2])
    lose_v, lose_i = jnp.where(first, b[0], a[0]), jnp.where(first, b[2], a[2])
    next_v, next_i = jnp.where(first, a[1], b[1]), jnp.where(first, a[3], b[3])
    second = ahead(lose_v, lose_i, next_v, next_i)
    return (jnp.where(first, a[0], b[0]), jnp.where(second, lose_v, next_v),
            jnp.where(first, a[2], b[2]), jnp.where(second, lose_i, next_i))


def _pack(x):
    return pltpu.bitcast(x.astype(BF), I32)


def _unpack(x):
    return pltpu.bitcast(x, BF)


class _Order:
    def __init__(self, never):
        self.never = never
        self.link = None
        self.release = None

    def after(self, v):
        for dep in (self.link, self.release):
            if dep is not None:
                probe = self.never[:v.shape[0], :v.shape[1]]
                v = jnp.where(probe != probe, dep[:v.shape[0], :v.shape[1]], v)
        return v


def _kernel(x_hbm, wqkv_hbm, wphi_hbm, wo_hbm, wr_hbm, wg_hbm, wu_hbm, wd_hbm, c_hbm, wmod_hbm,
            out_hbm,
            x_v, wqkv_v, wphi_v, wo_v, wr_v, wg_v, wu_v, wd_v, c_v, wmod_v,
            wkv_c, wq_c, wo_c, hc_v, oc_v, x1_v, xn_v, kv_acc, z_acc, kvT, mod_v, sb_v, bias_v, slab_v, idle_sem,
            sems, osems, *, cfg):
    R1, R2, RB = cfg.get("R1", 16), cfg.get("R2", 16), cfg.get("RB", 32)

    def col(ref, j, w=D):
        return ref.at[:, pl.ds(j * w, w)]

    def x_copy(t):
        return ("x%d" % t, x_hbm.at[pl.ds(t * T, T)], x_v.at[pl.ds(t * T, T)])

    def w_copy(name, j, c):
        return ("%s%d" % (name, c), col(wqkv_hbm, j * NCH + c, 256), wqkv_v.at[j * NCH + c])

    def mod_copy(name, j):
        return (name, col(wmod_hbm, j), wmod_v.at[j, :, pl.ds(0, D)])

    def scale_copy(d, k):
        rows = pl.ds(k * DHALF, DHALF)
        return ("ca%d%d" % (d, k), wmod_hbm.at[rows, pl.ds(D + d * DHALF, DHALF)],
                wmod_v.at[1, rows, pl.ds(d * DHALF, DHALF)])

    order = [("c", c_hbm, c_v), x_copy(0), ("wphi", wphi_hbm, wphi_v),
             w_copy("wk", 1, 0), w_copy("wv", 2, 0), *[scale_copy(d, k) for d in range(2) for k in range(2)],
             w_copy("wk", 1, 1), w_copy("wv", 2, 1), w_copy("wk", 1, 2), w_copy("wv", 2, 2),
             w_copy("wk", 1, 3), w_copy("wv", 2, 3), x_copy(1), mod_copy("sa", 0), x_copy(2), x_copy(3)]
    order += [w_copy("wq", 0, c) for c in range(NCH)]
    order += [("wr", wr_hbm, wr_v), ("wo", wo_hbm, wo_v), mod_copy("ga", 2), mod_copy("sb", 3), mod_copy("cb", 4), mod_copy("gb", 5),
              ("wg", wg_hbm, wg_v), ("wu", wu_hbm, wu_v), ("wd", wd_hbm, wd_v.at[:, pl.ds(0, D)])]
    copies = {}
    for i, (name, src, dst) in enumerate(order):
        copies[name] = pltpu.make_async_copy(src, dst, sems.at[i])
        copies[name].start()

    waited, started = set(), []

    scope = []

    def mark(name):
        if cfg.get("marks"):
            if scope:
                scope.pop().__exit__(None, None, None)
            if name:
                scope.append(jax.named_scope(name))
                scope[0].__enter__()

    def wait(*names):
        mark("w_" + names[0])
        for name in names:
            copies[name].wait()
            waited.add(name)
        mark("r_" + names[0])


    wait("c", "x0")
    cf = c_v[...].astype(F32)
    never = jnp.broadcast_to(cf[:, 0:128], (32, 128))
    order1, order2, order3, order4 = [_Order(never) for _ in range(4)]
    sc = jnp.broadcast_to(cf * jax.nn.sigmoid(cf), (16, D)).astype(BF)

    def normalized(tok, n, order=None):
        xc, rs = _center(x_v[pl.ds(tok, n), :].astype(F32), order)
        return xc * rs

    for r0 in range(0, T, 32):
        xn_v[pl.ds(r0, 32), :] = normalized(r0, 32)

    wait("wphi")
    row = lax.broadcasted_iota(I32, (128, DH), 0)
    lane = lax.broadcasted_iota(I32, (128, DH), 1)
    expand = jnp.where(((row % 64) // 2) == lane, 1.0, 0.0).astype(BF)
    bdt = _dot(expand, wphi_v[...].reshape(H * DH, DH), NT)
    row = lax.broadcasted_iota(I32, (128, D), 0)
    lane = lax.broadcasted_iota(I32, (128, D), 1)
    bdt = jnp.where(2 * (row // 64) + (row % 2) == (lane % 128) // DH, bdt, 0.0).astype(BF)

    def mod_row(j):
        return _dot(sc, wmod_v[j, :, pl.ds(0, D)], NN)[0:8]

    def mod_part(j, n, half):
        part = _dot(sc[:, half * DHALF:(half + 1) * DHALF],
                    wmod_v[j, pl.ds(half * DHALF, DHALF), pl.ds(n * 128, 128)], NN)[0:8]
        if half == 0:
            mod_v[j, :, pl.ds(n * 128, 128)] = part
        else:
            mod_v[j, :, pl.ds(n * 128, 128)] += part

    for k0 in range(0, D, 128):
        sb_v[pl.ds(k0, 128), :] = jnp.broadcast_to(sc[0:1, k0:k0 + 128].astype(F32), (128, 128)).T

    partial_mod = {}

    def mod_piece(j, k0, nk):
        acc = partial_mod.pop(j, None)
        step = cfg.get("mstep", 16)
        for k in range(k0, k0 + nk, step):
            s_col = sb_v[pl.ds(k, step), :]
            if k == k0 and cfg.get("chain3"):
                s_col = order3.after(s_col)
            term = wmod_v[j, pl.ds(k, step), pl.ds(0, D)].astype(F32) * jnp.concatenate([s_col] * (D // 128), axis=1)
            if step == 16:
                term = term[0:8] + term[8:16]
            acc = term if acc is None else acc + term
        if cfg.get("chain3"):
            link = acc[:, 0:128]
            for _ in range(cfg["chain3"]):
                link = jnp.broadcast_to(jnp.max(link, axis=-1, keepdims=True), (8, 128))
            order3.link = jnp.concatenate([link, link], axis=0)
        if k0 + nk < D:
            partial_mod[j] = acc
        else:
            mod_v[j] = jnp.broadcast_to(jnp.sum(acc, axis=0, keepdims=True), (8, D))

    def finish_mod():
        wr = wr_v[...].astype(F32)
        wr_row = jnp.concatenate([jnp.broadcast_to(wr[j:j + 1, :], (8, 128)) for j in range(8)], axis=1)
        shift, scale, gate = mod_v[3], 1.0 + mod_v[4], mod_v[5]
        mod_v[4] = scale
        mod_v[6] = gate * scale
        mod_v[7] = gate * shift
        mod_v[8] = wr_row * scale
        mod_v[9] = jnp.broadcast_to(jnp.sum(wr_row * shift, axis=-1, keepdims=True), (8, D))

    def rows_of(j, n):
        return _tile8(mod_v[j], n // 8)

    VW, VO, VH = cfg.get("vw", 1), cfg.get("vo", 1), cfg.get("vh", 1)
    pieces = {}

    operands = {}

    def put(key, value, size, axis=0):
        parts = pieces.setdefault(key, [])
        parts.append(value)
        if sum(part.shape[axis] for part in parts) == size:
            operands[key] = jnp.concatenate(pieces.pop(key), axis=axis).astype(BF)

    def h_term(t, i, r0=0, n=TH):
        return (t, i // 2, pl.ds(r0, n), pl.ds((i % 2) * DHALF, DHALF))

    def store_h_terms(t, r0, n, a, b):
        h1, h2 = a * rows_of(1, n), b * rows_of(1, n)
        terms = _rhs_terms(h1[:, :DHALF], h2[:, :DHALF], h1[:, DHALF:], h2[:, DHALF:])
        for i, term in enumerate(terms):
            if VH:
                put(("h", t, i), term, TH)
            else:
                hc_v[h_term(t, i, r0, n)] = term.astype(BF)

    def ln1_piece(t, r0):
        second = order4 if t == 1 else order1
        store_h_terms(t, r0, R1, normalized(t * T + r0, R1, order1), normalized(t * T + TH + r0, R1, second))

    def store_lhs_terms(top, bot, dst, c, r0):
        terms = _lhs_terms(top[:, :DHALF], top[:, DHALF:], bot[:, :DHALF], bot[:, DHALF:])
        for i, term in enumerate(terms):
            if VW:
                put(("w", c, i), term, 256)
            else:
                dst[c, i, pl.ds(r0, 128), :] = term.astype(BF)

    def shift_bias(dst, w, order):
        shift = jnp.concatenate([order.after(mod_v[0, :, l:l + 128]) for l in range(0, D, 128)], axis=1)
        b = jnp.sum(w * _tile8(shift, w.shape[0] // 8), axis=-1, keepdims=True)
        order.link = jnp.broadcast_to(b, (w.shape[0], 128))
        bias_v[pl.ds(dst, w.shape[0]), :] = order.link

    def kv_bias(r0):
        shift_bias(r0, x1_v[pl.ds(r0, RB), :], order2)

    def keep_weights(c, r0, halves):
        for g in range(2):
            x1_v[pl.ds(c * 512 + g * 256 + r0, 128), :] = halves[g]

    def folded(j, c):
        halves = []
        for g in range(2):
            w = wqkv_v[j * NCH + c, :, g * 128:(g + 1) * 128]
            gg = 2 * c + g
            halves.append(_dot(bdt[:, gg * 128:(gg + 1) * 128], w, NT) * LOG2E)
        return halves

    def prep_k(c):
        halves = folded(1, c)
        store_lhs_terms(halves[0], halves[1], wkv_c, c, 0)
        keep_weights(c, 0, halves)

    def prep_q(c):
        halves = folded(0, c)
        for r0 in range(0, 128, 16):
            top, bot = [jnp.concatenate([order2.after(half[r0:r0 + 16, l:l + 128]) for l in range(0, D, 128)], axis=1)
                        if g == 0 and cfg.get("pq", 1) else half[r0:r0 + 16] for g, half in enumerate(halves)]
            terms = _lhs_terms(top[:, :DHALF], top[:, DHALF:], bot[:, :DHALF], bot[:, DHALF:])
            for i, term in enumerate(terms):
                if VW:
                    put(("q", c, i), term, 128)
                else:
                    wq_c[c, i, pl.ds(r0 // 2, 8), :] = _pack(term)
            shift_bias(S + c * 256 + r0, top, _Order(never))
            shift_bias(S + c * 256 + 128 + r0, bot, order2 if cfg.get("pq", 1) else _Order(never))

    def prep_v(c):
        halves = [wqkv_v[2 * NCH + c, :, g * 128:(g + 1) * 128].T.astype(F32) for g in range(2)]
        store_lhs_terms(halves[0], halves[1], wkv_c, c, 128)
        keep_weights(c, 128, halves)

    def prep_wo(c, r0):
        def rows(r):
            w = wo_v[pl.ds(r, 16), :].astype(F32)
            return jnp.concatenate([order3.after(w[:, l:l + 128]) for l in range(0, D, 128)], axis=1)
        top, bot = rows(c * 256 + r0), wo_v[pl.ds(c * 256 + 128 + r0, 16), :].astype(F32)
        terms = _rhs_terms(top[:, :DHALF], top[:, DHALF:], bot[:, :DHALF], bot[:, DHALF:])
        for i, term in enumerate(terms):
            if VW:
                put(("wo", i), term, DHALF)
            else:
                wo_c[i, pl.ds(c * 64 + r0 // 2, 8), :] = _pack(term)
        order3.link = jnp.broadcast_to(jnp.max(terms[0][:, 0:128], axis=-1, keepdims=True), (16, 128))

    stream = _Order(never)

    def behind_product(v):
        head = jnp.concatenate([stream.after(v[0:8, l:l + 128]) for l in range(0, T, 128)], axis=1)
        return jnp.concatenate([head, v[8:]], axis=0)

    def bias_rows(r0):
        return jnp.concatenate([bias_v[pl.ds(r0, 64), :]] * (T // 128), axis=1)

    def kv_pair(t, c, res, k):
        g, q = divmod(k, 2)
        pair = 4 * c + k
        r0 = c * 512 + g * 256 + q * 64
        phi = _hedgehog(res[g][128 + q * 64:128 + (q + 1) * 64] + bias_rows(r0))
        vt = behind_product(res[g][q * 64:(q + 1) * 64]).astype(BF)
        zs = phi[:, 0:128]
        for l in range(1, T // 128):
            zs = zs + phi[:, l * 128:(l + 1) * 128]
        kv = _dot(vt, phi.astype(BF), NT)
        if t > 0:
            zs = zs + z_acc[pair]
            kv = kv + kv_acc[pair]
        if t < NTILE - 1:
            z_acc[pair] = zs
            kv_acc[pair] = kv
        else:
            z = jnp.broadcast_to(jnp.sum(zs.T, axis=0, keepdims=True), (16, 128))
            kv = kv + bias_v[pl.ds(r0 + 128, 64), :] * _tile8(z[0:8], 8)
            row = lax.broadcasted_iota(I32, (80, 128), 0)
            lane = lax.broadcasted_iota(I32, (80, 128), 1)
            head = jnp.where(row < 64, row // DH, (row - 64) // 8)
            kvT[pair] = jnp.where(head == lane % 2, jnp.concatenate([kv, z], axis=0), 0.0).astype(BF)

    def q_pair(c, res, k):
        g, q = divmod(k, 2)
        pair = 4 * c + k
        even = (lax.broadcasted_iota(I32, (8, T), 0) % 2) == 0
        phi, scale = _hedgehog_scaled(res[g][q * 64:(q + 1) * 64] + bias_rows(S + pair * 64))
        if cfg.get("tq"):
            phi = behind_product(phi)
        nd = _dot(kvT[pair], phi.astype(BF), NN)
        swapped = pltpu.roll(scale, 1, 0)
        inv_a = _recip(nd[64:72] + 1e-6 * jnp.where(even, scale, swapped))
        inv_b = _recip(nd[72:80] + 1e-6 * jnp.where(even, swapped, scale))
        return nd[0:64] * jnp.concatenate([inv_a] * 4 + [inv_b] * 4, axis=0)

    held = {}

    def q_step(t, c, res, k):
        held[k] = q_pair(c, res, k)
        if k == 3:
            held["lower"] = jnp.concatenate([held.pop(2), held.pop(3)], axis=0).T
        if k == 1:
            o1, o2 = jnp.concatenate([held.pop(0), held.pop(1)], axis=0).T, held.pop("lower")
            for i, term in enumerate(_lhs_terms(o1[:TH], o2[:TH], o1[TH:], o2[TH:])):
                if VO:
                    for r0, n in (step[2] for step in steps if step[:2] == ("o", t)):
                        put(("o", t, i, r0), term[r0:r0 + n], DHALF, 1)
                else:
                    oc_v[t, i, :, pl.ds(c * 128, 128)] = term.astype(BF)

    def residual(tok, attn):
        rows = pl.ds(tok, attn.shape[0])
        x1_v[rows, :] = x_v[rows, :].astype(F32) + rows_of(2, attn.shape[0]) * attn

    def block_out(x1, xc, rs):
        n = x1.shape[0]
        return xc * (rs * rows_of(6, n)) + (x1 + rows_of(7, n))

    def router(xc, rs):
        n = xc.shape[0]
        return jnp.sum(xc * rows_of(8, n), axis=-1, keepdims=True) * rs + rows_of(9, n)[:, 0:1]

    found = []

    def ln2_piece(tok, order):
        x1 = x1_v[pl.ds(tok, R2), :]
        xc, rs = _center(x1, order)
        t, r0 = divmod(tok, T)
        hc_v[t, r0 // TH, pl.ds(r0 % TH, R2), :] = block_out(x1, xc, rs).astype(BF)
        r = router(xc, rs)
        sub = lax.broadcasted_iota(I32, (8, 128), 0).astype(F32)
        ra, rb = jnp.broadcast_to(r[0:8], (8, 128)), jnp.broadcast_to(r[8:16], (8, 128))
        ia, ib = sub + float(tok), sub + float(tok + 8)
        first = ra >= rb
        found.append((jnp.where(first, ra, rb), jnp.where(first, rb, ra),
                      jnp.where(first, ia, ib), jnp.where(first, ib, ia)))
        if order is not None:
            found[:] = [_merge_top2(found[0], found[1])] if len(found) == 2 else found

    def out_copy(t, half):
        return pltpu.make_async_copy(hc_v.at[t, half], out_hbm.at[pl.ds(t * T + half * TH, TH)],
                                     osems.at[2 * t + half])

    def start_out(t):
        for half in range(2):
            out_copy(t, half).start()
        started.append(t)

    wait("wk0", "wv0")
    prep_v(0)
    prep_k(0)

    def first_terms(d, wanted):
        cols = pl.ds(d * DHALF, DHALF)
        scale = 1.0
        for k in range(2):
            wait("ca%d%d" % (d, k))
            scale = scale + _dot(sc[:, k * DHALF:(k + 1) * DHALF], wmod_v[1, pl.ds(k * DHALF, DHALF), cols], NN)[0:8]
        mod_v[1, :, cols] = scale

        def block(half, dd, r0):
            if dd > d:
                return None
            cc = pl.ds(dd * DHALF, DHALF)
            return xn_v[pl.ds(half * TH + r0, 64), cc] * _tile8(mod_v[1, :, cc], 8)

        for group in wanted:
            for r0 in range(0, TH, 64):
                b11, b12, b21, b22 = block(0, 0, r0), block(1, 0, r0), block(0, 1, r0), block(1, 1, r0)
                terms = _rhs_terms(b11, b12, b21, b22) if d else {1: b11, 5: b11 + b12}
                for i in group:
                    if VH:
                        put(("h", 0, i), terms[i], TH)
                    else:
                        hc_v[h_term(0, i, r0, 64)] = terms[i].astype(BF)

    def h_operand(t, i):
        return operands["h", t, i] if VH else hc_v[h_term(t, i)]

    def kv_product(t, c, i, part=None):
        rows = pl.ds(0, 256) if part is None else pl.ds(part * 128, 128)
        w = operands["w", c, i] if VW else wkv_c[c, i, rows, :]
        return _dot(w, h_operand(t, i), NT)

    first_terms(0, ((1,), (5,)))
    head_start = {i: kv_product(0, 0, i) for i in (1, 5)}
    first_terms(1, cfg.get("tg", ((0,), (3, 2, 4, 6))))

    P = functools.partial

    def spread(slots, lo, hi, works):
        for n, work in enumerate(works):
            slots[lo + n * (hi - lo) // len(works)].append(work)

    steps = [("kv", t, c) for t in range(NTILE) for c in range(NCH)]
    steps += [("q", t, c) for t in range(NTILE) for c in range(NCH)]
    for t, sizes in enumerate(cfg["osplit"]):
        steps += [("o", t, (sum(sizes[:k]), n)) for k, n in enumerate(sizes)]
    if cfg.get("only"):
        steps = [steps[i] for i in cfg["only"]]
    mod_parts = [P(mod_part, j, n, half) for j in range(2, 6) for half in range(2) for n in range(8)]
    prev = None
    pending = []
    for step, (kind, t, c) in enumerate(steps):
        slots = [[] for _ in range(7)]
        lower_done = None
        if prev is not None:
            pkind, pt, pc, pres = prev
            if pkind == "kv":
                pending += [P(kv_pair, pt, pc, pres, k) for k in (2, 3, 0, 1)]
                n = len(pending) if cfg.get("only") or kind != "kv" else cfg["quota"][t * NCH + c]
                for slot in cfg["kslots"][n]:
                    slots[slot].append(pending.pop(0))
            elif pkind == "q":
                qs = cfg.get("qs", (0, 1, 3, 5))
                for slot, k in zip(qs, (2, 3, 0, 1)):
                    slots[slot].append(P(q_step, pt, pc, pres, k))
            else:
                tok = pt * T + pc[0]
                slots[0].append(P(residual, tok, pres[0]))
                lo, hi = cfg.get("l2a", (0, 4))
                group = _Order(never)
                spread(slots, lo, hi, [P(ln2_piece, tok + r0, group) for r0 in range(0, pc[1], R2)])
                if sum(pc) == TH:
                    slots[hi].append(P(start_out, pt))
        if kind == "kv":
            if t == 0 and c + 1 < NCH:
                names = (("wk1", "wv1"), ("wk2", "wv2", "wk3", "wv3"), ("x1",))[c]
                k = cfg["ws"][c]
                slots[k] += [P(wait, *names), P(prep_v, c + 1), P(prep_k, c + 1)]
            if (t, c) == (1, 0):
                slots[0] = [P(wait, "sa", "x2", "x3"), lambda: mod_v.__setitem__(0, mod_row(0))] + slots[0]
            if t == 1 and c < 2:
                for k in range(2):
                    first = (2 * c + k) * 512
                    at = cfg["bs"][c][k]
                    slots[at] += [P(kv_bias, r0) for r0 in range(first, first + 512, RB)]
            if t + 1 < NTILE:
                chunks = ((2, 3), (0, 1, 2, 3), (0, 1, 2, 3))[t]
                if c in chunks:
                    rows = list(range(0, TH, R1))
                    k = chunks.index(c)
                    mine = rows[k * len(rows) // len(chunks):(k + 1) * len(rows) // len(chunks)]
                    spread(slots, cfg["ws"][2] + 1 if (t, c) == (0, 2) else 0, 6, [P(ln1_piece, t + 1, r0) for r0 in mine])
        n = step - cfg["n0"]
        if n == 0:
            slots[0].insert(0, P(wait, "wq0", "wq1", "wq2", "wq3", "wr", "wo", "ga", "sb", "cb", "gb"))
            late = []
            for j in range(4):
                for m in range(8):
                    k0 = m * 128
                    for nk in cfg["nks"]:
                        late.append(P(mod_piece, 2 + j, k0, nk))
                        k0 += nk
                    late.append(P(prep_wo, j, m * 16))
        if 0 <= n - cfg.get("nq", 0) < NCH:
            slots[5].append(P(prep_q, n - cfg.get("nq", 0)))
        left = cfg["n1"] - cfg["n0"]
        if 0 <= n < left:
            spread(slots, 1, 7, late[n * len(late) // left:(n + 1) * len(late) // left])
        if n == left:
            slots[0].insert(0, P(wait, "wg"))
            slots[6].append(finish_mod)
        if kind == "o":
            last = step == len(steps) - 1
            tok2 = t * T + TH + c[0]
            lower_done = P(residual, tok2)
            lo, hi = (5, 6) if last else cfg.get("l2b", (5, 7))
            group = _Order(never)
            spread(slots, lo, hi, [P(ln2_piece, tok2 + r0, None if last else group) for r0 in range(0, c[1], R2)])

        def fill(k, m, slots=slots):
            stream.release = m
            for work in slots[k]:
                work()

        if kind == "kv":
            if cfg.get("ksplit") and (t, c) != (0, 0):
                halves = [_block_product(P(kv_product, t, c, part=part),
                                         lambda k, m, part=part: fill((7 * part + k) // 2, m) if (7 * part + k) % 2 else None)
                          for part in range(2)]
                res = [jnp.concatenate([halves[0][g], halves[1][g]], axis=0) for g in range(2)]
            else:
                res = _block_product(lambda i: head_start.pop(i) if i in head_start else kv_product(t, c, i), fill)
        elif kind == "q":
            res = _block_product(lambda i: _dot(operands["q", c, i] if VW else _unpack(wq_c[c, i]), h_operand(t, i), NT), fill)
        else:
            res = _block_product(
                lambda i: _dot(operands["o", t, i, c[0]] if VO else oc_v[t, i, pl.ds(*c), :],
                               operands["wo", i] if VW else _unpack(wo_c[i]), NN), fill, lower_done)
        if kind == "kv" and c == NCH - 1:
            order1.link = None
        prev = (kind, t, c, res)

    if cfg.get("only"):
        for name in copies:
            if name not in waited:
                wait(name)
        a, b = prev[3]
        x1_v[0:128, 0:256] = a[0:128, 0:256] + b[0:128, 0:256] + a[0:128, 256:512] + b[0:128, 256:512]
        x1_v[128:136, 0:128] = sum(sum(f) for f in found) if found else jnp.zeros((8, 128), F32)
        z = pl.semaphore_read(idle_sem)
        x1_v[136:144, :] = mod_v[z]
        x1_v[144:160, 0:512] = oc_v[z, z, 0:16, :].astype(F32) + hc_v[z, z, 0:16, 0:512].astype(F32) + (
            wo_c[z, 0:16, :] + wq_c[z, z, 0:16, :] + wkv_c[z, z, 0:16, :]).astype(F32)
        x1_v[160:176, 0:128] = kvT[z, 0:16, :].astype(F32) + kv_acc[z, 0:16, :] + z_acc[z, 0:16, :]
        slab_v[0] = x1_v[pl.ds(pl.multiple_of(z * 16, 16), 16), :].astype(BF)
        cpy = pltpu.make_async_copy(slab_v.at[0], out_hbm.at[pl.ds(0, 16)], osems.at[0])
        cpy.start()
        cpy.wait()
        for t in started:
            out_copy(t, 0).wait()
            out_copy(t, 1).wait()
        return

    _, pt, pc, pres = prev
    tok = pt * T + pc[0]
    residual(tok, pres[0])
    for r0 in range(0, pc[1], R2):
        ln2_piece(tok + r0, None)
    start_out(pt)

    while len(found) > 1:
        found[:] = [_merge_top2(*found[k:k + 2]) if k + 1 < len(found) else found[k]
                    for k in range(0, len(found), 2)]
    m1, m2, i1, i2 = found[0]
    big = float(2 * S)
    best = jnp.max(m1, axis=0, keepdims=True)
    ia = jnp.min(jnp.where(m1 == best, i1, big), axis=0, keepdims=True)
    taken = i1 == ia
    cm = jnp.where(taken, m2, m1)
    ci = jnp.where(taken, i2, i1)
    second = jnp.max(cm, axis=0, keepdims=True)
    ib = jnp.min(jnp.where(cm == second, ci, big), axis=0, keepdims=True)
    idx_a = jnp.clip(ia.astype(I32)[0, 0], 0, S - 1)
    idx_b = jnp.clip(ib.astype(I32)[0, 0], 0, S - 1)

    sub = lax.broadcasted_iota(I32, (16, D), 0)
    xa = jnp.broadcast_to(x1_v[pl.ds(idx_a, 1), :], (16, D))
    xb = jnp.broadcast_to(x1_v[pl.ds(idx_b, 1), :], (16, D))
    xc, rs = _center(jnp.where(sub == 0, xa, xb))
    gate_r = jax.nn.sigmoid(router(xc, rs))
    hb = (xc * rs * rows_of(4, 16) + rows_of(3, 16)).astype(BF)
    wait("wu", "wd")
    for t in range(NTILE - 1):
        out_copy(t, 0).wait()
        out_copy(t, 1).wait()

    def slab(idx):
        start = pl.multiple_of((idx // 16) * 16, 16)
        x1 = x1_v[pl.ds(start, 16), :]
        return start, block_out(x1, *_center(x1))

    slabs = [slab(idx_a), slab(idx_b)]
    g = _dot(hb, wg_v[...], NN)
    u = _dot(hb, wu_v[...], NN)
    act = (g * jax.nn.sigmoid(g) * u).astype(BF)
    y = _dot(act, wd_v[:, pl.ds(0, D)], NN) * (gate_r * rows_of(5, 16))

    fixes = []
    for slot, (start, o) in enumerate(slabs):
        o = o + jnp.where(sub + start == idx_a, y[0:1], 0.0) + jnp.where(sub + start == idx_b, y[1:2], 0.0)
        slab_v[slot] = o.astype(BF)
        fixes.append(pltpu.make_async_copy(slab_v.at[slot], out_hbm.at[pl.ds(start, 16)], osems.at[slot]))
    out_copy(NTILE - 1, 0).wait()
    out_copy(NTILE - 1, 1).wait()
    fixes[0].start()

    @pl.when(idx_a // 16 != idx_b // 16)
    def _():
        fixes[1].start()
        fixes[1].wait()

    fixes[0].wait()
    mark(None)


def make(flags=None, **cfg):
    cfg = dict(dict(tie=False, vmod=32, chain3=1, ws=(3, 3, 2), osplit=((64,) * 4,) * 4, n0=10, n1=16, bs=((1, 4), (0, 3)), RB=64, ev=1,
                    quota=(0, 0, 0, 0, 0, 3, 6, 6, 6, 6, 6, 6, 6, 5, 5, 5),
                    kslots={0: (), 2: (4, 5), 3: (3, 4, 5), 4: (1, 2, 3, 4), 5: (1, 2, 3, 4, 5), 6: (0, 1, 2, 3, 4, 5)},
                    nks=(32, 32, 32, 32), mstep=8, ks=(1, 2, 3, 4)), **cfg)
    if cfg.get("ev", False):
        flags = dict(flags or {}, XLA_TPU_EVENLY_DISTRIBUTE_CRITICAL_NODES=True)
    pad = cfg.get("pad", 128)

    def run(A_x, A_wqkv, A_w_phi, A_wo, B_x, B_w_r, B_w_gate, B_w_up, B_w_down, c, w_mod):
        del B_x
        any_spec = pl.BlockSpec(memory_space=pl.ANY)
        scratch = [
            pltpu.VMEM((S, D), BF), pltpu.VMEM((3 * NCH, D, 256), BF), pltpu.VMEM((H, DH, DH), BF),
            pltpu.VMEM((D, D), BF), pltpu.VMEM((8, 128), BF),
            pltpu.VMEM((D, F), BF), pltpu.VMEM((D, F), BF), pltpu.VMEM((F, D + pad), BF),
            pltpu.VMEM((1, D), BF), pltpu.VMEM((6, D, D + pad), BF),
            *([pltpu.VMEM((8, 128), I32)] * 3 if cfg.get("vw", 1) else [
                pltpu.VMEM((NCH, 7, 256, DHALF), BF), pltpu.VMEM((NCH, 7, 64, DHALF), I32),
                pltpu.VMEM((7, DHALF // 2, DHALF), I32)]),
            pltpu.VMEM((NTILE, 2 if cfg.get("vh", 1) else 4, TH, D), BF),
            pltpu.VMEM((8, 128) if cfg.get("vo", 1) else (NTILE, 7, TH, DHALF), BF), pltpu.VMEM((S, D), F32), pltpu.VMEM((T, D), F32),
            pltpu.VMEM((H // 2, 64, 128), F32), pltpu.VMEM((H // 2, 128, 128), F32),
            pltpu.VMEM((H // 2, 80, 128), BF),
            pltpu.VMEM((10, 8, D), F32), pltpu.VMEM((D, 128), F32), pltpu.VMEM((S + D, 128), F32), pltpu.VMEM((2, 16, D), BF), pltpu.SemaphoreType.REGULAR,
            pltpu.SemaphoreType.DMA((40,)), pltpu.SemaphoreType.DMA((2 * NTILE,)),
        ]
        out = pl.pallas_call(
            functools.partial(_kernel, cfg=cfg),
            out_shape=jax.ShapeDtypeStruct((S, D), BF),
            in_specs=[any_spec] * 10,
            out_specs=any_spec,
            scratch_shapes=scratch,
            compiler_params=pltpu.CompilerParams(vmem_limit_bytes=120 * 2**20, flags=flags),
            name="fused_block",
        )(A_x.reshape(S, D), A_wqkv, A_w_phi, A_wo, B_w_r.reshape(8, 128), B_w_gate, B_w_up, B_w_down, c, w_mod)
        return out.reshape(1, S, D)
    return run


_run = make(**dict())


@jax.jit
def pallas_adaLN_cond__linear_kernel_hedgehog__moe_arch_mod__prompt_kernel(
    A_x: jax.Array,
    A_wqkv: jax.Array,
    A_w_phi: jax.Array,
    A_wo: jax.Array,
    B_x: jax.Array,
    B_w_r: jax.Array,
    B_w_gate: jax.Array,
    B_w_up: jax.Array,
    B_w_down: jax.Array,
    c: jax.Array,
    w_mod: jax.Array,
):
    return _run(A_x, A_wqkv, A_w_phi, A_wo, B_x, B_w_r, B_w_gate, B_w_up, B_w_down, c, w_mod)
```

```python
import functools

import jax
import jax.numpy as jnp
from jax import lax
from jax.experimental import pallas as pl
from jax.experimental.pallas import tpu as pltpu

S, D, H, DH, F = 2048, 1024, 32, 32, 3584
T = 512
TH = T // 2
DHALF = D // 2
NTILE = S // T
NCH = D // 256
OROWS = 64
LROWS = 16
LANE_PAD = 128
LOG2E = 1.4426950408889634
NN = (((1,), (0,)), ((), ()))
NT = (((1,), (1,)), ((), ()))
BF = jnp.bfloat16
F32 = jnp.float32
I32 = jnp.int32

KV_QUOTA = (0, 0, 0, 0, 0, 3, 6, 6, 6, 6, 6, 6, 6, 5, 5, 5)
KV_SLOTS = {0: (), 3: (3, 4, 5), 4: (1, 2, 3, 4), 5: (1, 2, 3, 4, 5), 6: (0, 1, 2, 3, 4, 5)}
LATE_FIRST, LATE_LAST = 12, 18


def _dot(a, b, dims):
    return lax.dot_general(a, b, dims, preferred_element_type=F32)


def _recip(x):
    return pltpu.reciprocal(x, approx=False, full_range=False)


def _tile8(r, n):
    return jnp.concatenate([r] * n, axis=0)


class _Order:
    def __init__(self, probe):
        self.probe = probe
        self.link = None

    def after(self, v):
        if self.link is None:
            return v
        rows, lanes = v.shape[0], min(v.shape[1], 128)
        probe, link = self.probe[:rows, :lanes], self.link[:rows, :lanes]
        return jnp.concatenate([jnp.where(probe != probe, link, v[:, l:l + lanes])
                                for l in range(0, v.shape[1], lanes)], axis=1)


def _center(x, order=None):
    s = jnp.sum(x, axis=-1, keepdims=True)
    if order is not None:
        s = order.after(s)
    xc = x - s * (1.0 / D)
    rs = lax.rsqrt(jnp.sum(xc * xc, axis=-1, keepdims=True) * (1.0 / D) + 1e-5)
    if order is not None:
        order.link = rs
    return xc, rs


def _pair_reduce(x, op):
    r = x[0:8]
    for i in range(1, 8):
        r = op(r, x[8 * i:8 * i + 8])
    r = op(r, pltpu.roll(r, 4, 0))
    return op(r, pltpu.roll(r, 2, 0))


def _pair_exps(p):
    mx = _tile8(_pair_reduce(p, jnp.maximum), 8)
    mn = _tile8(_pair_reduce(p, jnp.minimum), 8)
    return jnp.exp2(p - mx), jnp.exp2(mn - p)


def _hedgehog(p):
    ep, en = _pair_exps(p)
    rp = _tile8(_recip(_pair_reduce(ep, jnp.add)), 8)
    rn = _tile8(_recip(_pair_reduce(en, jnp.add)), 8)
    return jnp.concatenate([ep * rp, en * rn], axis=0)


def _hedgehog_scaled(p):
    ep, en = _pair_exps(p)
    sp = _pair_reduce(ep, jnp.add)
    ratio = _tile8(sp * _recip(_pair_reduce(en, jnp.add)), 8)
    return jnp.concatenate([ep, en * ratio], axis=0), sp


def _lhs_terms(a11, a12, a21, a22):
    return (a11 + a22, a21 + a22, a11, a22, a11 + a12, a21 - a11, a12 - a22)


def _rhs_terms(b11, b12, b21, b22):
    return (b11 + b22, b11, b12 - b22, b21 - b11, b22, b11 + b12, b21 + b22)


def _quadrants(top, bottom):
    return top[:, :DHALF], top[:, DHALF:], bottom[:, :DHALF], bottom[:, DHALF:]


def _block_product(product, fill, lower_done=None):
    m0 = product(0)
    fill(0, m0)
    m1 = product(1)
    fill(1, m1)
    c22 = m0 - m1
    m3 = product(3)
    fill(2, m3)
    c21 = m1 + m3
    c11 = m0 + m3
    m2 = product(2)
    fill(3, m2)
    c22 = c22 + m2
    m5 = product(5)
    fill(4, m5)
    lower = jnp.concatenate([c21, c22 + m5], axis=1)
    if lower_done is not None:
        lower_done(lower)
    m4 = product(4)
    fill(5, m4)
    c12 = m2 + m4
    c11 = c11 - m4
    m6 = product(6)
    fill(6, m6)
    return jnp.concatenate([c11 + m6, c12], axis=1), lower


def _merge_top2(a, b):
    def ahead(v, i, w, j):
        return (v > w) | ((v == w) & (i < j))

    first = ahead(a[0], a[2], b[0], b[2])
    lose_v, lose_i = jnp.where(first, b[0], a[0]), jnp.where(first, b[2], a[2])
    next_v, next_i = jnp.where(first, a[1], b[1]), jnp.where(first, a[3], b[3])
    second = ahead(lose_v, lose_i, next_v, next_i)
    return (jnp.where(first, a[0], b[0]), jnp.where(second, lose_v, next_v),
            jnp.where(first, a[2], b[2]), jnp.where(second, lose_i, next_i))


def _kernel(x_hbm, wqkv_hbm, wphi_hbm, wo_hbm, wr_hbm, wg_hbm, wu_hbm, wd_hbm, c_hbm, wmod_hbm,
            out_hbm,
            x_v, wqkv_v, wphi_v, wo_v, wr_v, wg_v, wu_v, wd_v, c_v, wmod_v,
            out_v, x1_v, xn_v, kv_acc, z_acc, kv_v, mod_v, sc_v, bias_v, gate_v, slab_v,
            in_sems, out_sems):
    def x_copy(t):
        return ("x%d" % t, x_hbm.at[pl.ds(t * T, T)], x_v.at[pl.ds(t * T, T)])

    def w_copy(name, j, c):
        return ("%s%d" % (name, c), wqkv_hbm.at[:, pl.ds((j * NCH + c) * 256, 256)], wqkv_v.at[j * NCH + c])

    def mod_copy(name, j):
        return (name, wmod_hbm.at[:, pl.ds(j * D, D)], wmod_v.at[j, :, pl.ds(0, D)])

    def scale_copy(d, k):
        rows = pl.ds(k * DHALF, DHALF)
        return ("ca%d%d" % (d, k), wmod_hbm.at[rows, pl.ds(D + d * DHALF, DHALF)],
                wmod_v.at[1, rows, pl.ds(d * DHALF, DHALF)])

    queue = [("c", c_hbm, c_v), x_copy(0), ("wphi", wphi_hbm, wphi_v), w_copy("wk", 1, 0), w_copy("wv", 2, 0)]
    queue += [scale_copy(d, k) for d in range(2) for k in range(2)]
    for c in range(1, NCH):
        queue += [w_copy("wk", 1, c), w_copy("wv", 2, c)]
    queue += [x_copy(1), mod_copy("sa", 0), x_copy(2), x_copy(3)]
    queue += [w_copy("wq", 0, c) for c in range(NCH)]
    queue += [("wr", wr_hbm, wr_v), ("wo", wo_hbm, wo_v),
              mod_copy("ga", 2), mod_copy("sb", 3), mod_copy("cb", 4), mod_copy("gb", 5),
              ("wg", wg_hbm, wg_v), ("wu", wu_hbm, wu_v), ("wd", wd_hbm, wd_v.at[:, pl.ds(0, D)])]
    copies = {}
    for i, (name, src, dst) in enumerate(queue):
        copies[name] = pltpu.make_async_copy(src, dst, in_sems.at[i])
        copies[name].start()

    def wait(*names):
        for name in names:
            copies[name].wait()

    wait("c", "x0")
    cf = c_v[...].astype(F32)
    probe = jnp.broadcast_to(cf[:, 0:128], (64, 128))
    norm_order, norm_order2, bias_order, late_order, stream = [_Order(probe) for _ in range(5)]
    sc = jnp.broadcast_to(cf * jax.nn.sigmoid(cf), (16, D)).astype(BF)

    def normalized(tok, n, order=None):
        xc, rs = _center(x_v[pl.ds(tok, n), :].astype(F32), order)
        return xc * rs

    for r0 in range(0, T, 32):
        xn_v[pl.ds(r0, 32), :] = normalized(r0, 32)

    wait("wphi")
    row = lax.broadcasted_iota(I32, (128, DH), 0)
    lane = lax.broadcasted_iota(I32, (128, DH), 1)
    expand = jnp.where(((row % 64) // 2) == lane, 1.0, 0.0).astype(BF)
    phi_t = _dot(expand, wphi_v[...].reshape(H * DH, DH), NT)
    row = lax.broadcasted_iota(I32, (128, D), 0)
    lane = lax.broadcasted_iota(I32, (128, D), 1)
    phi_t = jnp.where(2 * (row // 64) + (row % 2) == (lane % 128) // DH, phi_t, 0.0).astype(BF)

    for k0 in range(0, D, 128):
        sc_v[pl.ds(k0, 128), :] = jnp.broadcast_to(sc[0:1, k0:k0 + 128].astype(F32), (128, 128)).T

    partial_mod = {}

    def mod_piece(j, k0, nk):
        acc = partial_mod.pop(j, None)
        for k in range(k0, k0 + nk, 8):
            s_col = sc_v[pl.ds(k, 8), :]
            if k == k0:
                s_col = late_order.after(s_col)
            term = wmod_v[j, pl.ds(k, 8), pl.ds(0, D)].astype(F32) * jnp.concatenate([s_col] * (D // 128), axis=1)
            acc = term if acc is None else acc + term
        link = jnp.broadcast_to(jnp.max(acc[:, 0:128], axis=-1, keepdims=True), (8, 128))
        late_order.link = jnp.concatenate([link, link], axis=0)
        if k0 + nk < D:
            partial_mod[j] = acc
        else:
            mod_v[j] = jnp.broadcast_to(jnp.sum(acc, axis=0, keepdims=True), (8, D))

    def first_shift():
        mod_v[0] = _dot(sc, wmod_v[0, :, pl.ds(0, D)], NN)[0:8]

    def finish_mod():
        wr = wr_v[...].astype(F32)
        wr_row = jnp.concatenate([jnp.broadcast_to(wr[j:j + 1, :], (8, 128)) for j in range(8)], axis=1)
        shift, scale, gate = mod_v[3], 1.0 + mod_v[4], mod_v[5]
        mod_v[4] = scale
        mod_v[6] = gate * scale
        mod_v[7] = gate * shift
        mod_v[8] = wr_row * scale
        mod_v[9] = jnp.broadcast_to(jnp.sum(wr_row * shift, axis=-1, keepdims=True), (8, D))

    def rows_of(j, n):
        return _tile8(mod_v[j], n // 8)

    pieces, operands = {}, {}

    def put(key, value, size, axis=0):
        parts = pieces.setdefault(key, [])
        parts.append(value)
        if sum(part.shape[axis] for part in parts) == size:
            operands[key] = jnp.concatenate(pieces.pop(key), axis=axis).astype(BF)

    def ln1_piece(t, r0):
        a = normalized(t * T + r0, LROWS, norm_order)
        b = normalized(t * T + TH + r0, LROWS, norm_order2 if t == 1 else norm_order)
        h1, h2 = a * rows_of(1, LROWS), b * rows_of(1, LROWS)
        for i, term in enumerate(_rhs_terms(h1[:, :DHALF], h2[:, :DHALF], h1[:, DHALF:], h2[:, DHALF:])):
            put(("h", t, i), term, TH)

    def shift_bias(dst, w, order):
        b = jnp.sum(w * _tile8(order.after(mod_v[0]), w.shape[0] // 8), axis=-1, keepdims=True)
        order.link = jnp.broadcast_to(b, (w.shape[0], 128))
        bias_v[pl.ds(dst, w.shape[0]), :] = order.link

    def kv_bias(r0):
        shift_bias(r0, x1_v[pl.ds(r0, 64), :], bias_order)

    def folded(j, c):
        halves = []
        for g in range(2):
            w = wqkv_v[j * NCH + c, :, g * 128:(g + 1) * 128]
            group = 2 * c + g
            halves.append(_dot(phi_t[:, group * 128:(group + 1) * 128], w, NT) * LOG2E)
        return halves

    def put_kv_weights(c, r0, halves):
        for i, term in enumerate(_lhs_terms(*_quadrants(*halves))):
            put(("w", c, i), term, 256)
        for g in range(2):
            x1_v[pl.ds(c * 512 + g * 256 + r0, 128), :] = halves[g]

    def prep_kv(c):
        put_kv_weights(c, 128, [wqkv_v[2 * NCH + c, :, g * 128:(g + 1) * 128].T.astype(F32) for g in range(2)])
        put_kv_weights(c, 0, folded(1, c))

    def prep_q(c):
        halves = folded(0, c)
        for r0 in range(0, 128, 16):
            top, bottom = bias_order.after(halves[0][r0:r0 + 16]), halves[1][r0:r0 + 16]
            for i, term in enumerate(_lhs_terms(*_quadrants(top, bottom))):
                put(("q", c, i), term, 128)
            shift_bias(S + c * 256 + r0, top, _Order(probe))
            shift_bias(S + c * 256 + 128 + r0, bottom, bias_order)

    def prep_wo(c, r0):
        top = late_order.after(wo_v[pl.ds(c * 256 + r0, 16), :].astype(F32))
        bottom = wo_v[pl.ds(c * 256 + 128 + r0, 16), :].astype(F32)
        terms = _rhs_terms(*_quadrants(top, bottom))
        for i, term in enumerate(terms):
            put(("wo", i), term, DHALF)
        late_order.link = jnp.broadcast_to(jnp.max(terms[0][:, 0:128], axis=-1, keepdims=True), (16, 128))

    def bias_rows(r0):
        return jnp.concatenate([bias_v[pl.ds(r0, 64), :]] * (T // 128), axis=1)

    def kv_pair(t, c, res, k):
        g, q = divmod(k, 2)
        pair = 4 * c + k
        r0 = c * 512 + g * 256 + q * 64
        phi = _hedgehog(res[g][128 + q * 64:128 + (q + 1) * 64] + bias_rows(r0))
        vt = res[g][q * 64:(q + 1) * 64]
        vt = jnp.concatenate([stream.after(vt[0:8]), vt[8:]], axis=0).astype(BF)
        zs = phi[:, 0:128]
        for l in range(128, T, 128):
            zs = zs + phi[:, l:l + 128]
        kv = _dot(vt, phi.astype(BF), NT)
        if t > 0:
            zs = zs + z_acc[pair]
            kv = kv + kv_acc[pair]
        if t < NTILE - 1:
            z_acc[pair] = zs
            kv_acc[pair] = kv
        else:
            z = jnp.broadcast_to(jnp.sum(zs.T, axis=0, keepdims=True), (16, 128))
            kv = kv + bias_v[pl.ds(r0 + 128, 64), :] * _tile8(z[0:8], 8)
            row = lax.broadcasted_iota(I32, (80, 128), 0)
            lane = lax.broadcasted_iota(I32, (80, 128), 1)
            head = jnp.where(row < 64, row // DH, (row - 64) // 8)
            kv_v[pair] = jnp.where(head == lane % 2, jnp.concatenate([kv, z], axis=0), 0.0).astype(BF)

    held = {}

    def q_pair(t, c, res, k):
        g, q = divmod(k, 2)
        pair = 4 * c + k
        even = (lax.broadcasted_iota(I32, (8, T), 0) % 2) == 0
        phi, scale = _hedgehog_scaled(res[g][q * 64:(q + 1) * 64] + bias_rows(S + pair * 64))
        nd = _dot(kv_v[pair], phi.astype(BF), NN)
        swapped = pltpu.roll(scale, 1, 0)
        inv_a = _recip(nd[64:72] + 1e-6 * jnp.where(even, scale, swapped))
        inv_b = _recip(nd[72:80] + 1e-6 * jnp.where(even, swapped, scale))
        held[k] = nd[0:64] * jnp.concatenate([inv_a] * 4 + [inv_b] * 4, axis=0)
        if k == 3:
            held["lower"] = jnp.concatenate([held.pop(2), held.pop(3)], axis=0).T
        if k == 1:
            o1, o2 = jnp.concatenate([held.pop(0), held.pop(1)], axis=0).T, held.pop("lower")
            for i, term in enumerate(_lhs_terms(o1[:TH], o2[:TH], o1[TH:], o2[TH:])):
                for r0 in range(0, TH, OROWS):
                    put(("o", t, i, r0), term[r0:r0 + OROWS], DHALF, 1)

    def residual(tok, attn):
        rows = pl.ds(tok, OROWS)
        x1_v[rows, :] = x_v[rows, :].astype(F32) + rows_of(2, OROWS) * attn

    def block_out(x1, xc, rs):
        return xc * (rs * rows_of(6, LROWS)) + (x1 + rows_of(7, LROWS))

    def router(xc, rs):
        return jnp.sum(xc * rows_of(8, LROWS), axis=-1, keepdims=True) * rs + rows_of(9, LROWS)[:, 0:1]

    found = []

    def ln2_piece(tok, order):
        x1 = x1_v[pl.ds(tok, LROWS), :]
        xc, rs = _center(x1, order)
        out_v[tok // TH, pl.ds(tok % TH, LROWS), :] = block_out(x1, xc, rs).astype(BF)
        r = router(xc, rs)
        sub = lax.broadcasted_iota(I32, (8, 128), 0).astype(F32)
        ra, rb = jnp.broadcast_to(r[0:8], (8, 128)), jnp.broadcast_to(r[8:16], (8, 128))
        ia, ib = sub + float(tok), sub + float(tok + 8)
        first = ra >= rb
        found.append((jnp.where(first, ra, rb), jnp.where(first, rb, ra),
                      jnp.where(first, ia, ib), jnp.where(first, ib, ia)))
        if order is not None and len(found) == 2:
            found[:] = [_merge_top2(*found)]

    def select():
        while len(found) > 1:
            found[:] = [_merge_top2(*found[k:k + 2]) if k + 1 < len(found) else found[k]
                        for k in range(0, len(found), 2)]
        m1, m2, i1, i2 = found[0]
        big = float(2 * S)
        best = jnp.max(m1, axis=0, keepdims=True)
        ia = jnp.min(jnp.where(m1 == best, i1, big), axis=0, keepdims=True)
        taken = i1 == ia
        cm = jnp.where(taken, m2, m1)
        ci = jnp.where(taken, i2, i1)
        second = jnp.max(cm, axis=0, keepdims=True)
        ib = jnp.min(jnp.where(cm == second, ci, big), axis=0, keepdims=True)
        idx_a = jnp.clip(ia.astype(I32)[0, 0], 0, S - 1)
        idx_b = jnp.clip(ib.astype(I32)[0, 0], 0, S - 1)
        xa = jnp.broadcast_to(x1_v[pl.ds(idx_a, 1), :], (LROWS, D))
        xb = jnp.broadcast_to(x1_v[pl.ds(idx_b, 1), :], (LROWS, D))
        xc, rs = _center(jnp.where(lax.broadcasted_iota(I32, (LROWS, D), 0) == 0, xa, xb))
        rows = xc * rs * rows_of(4, LROWS) + rows_of(3, LROWS)
        return idx_a, idx_b, jax.nn.sigmoid(router(xc, rs)), rows

    def out_copy(k):
        return pltpu.make_async_copy(out_v.at[k], out_hbm.at[pl.ds(k * TH, TH)], out_sems.at[k])

    def start_out(t):
        out_copy(2 * t).start()
        out_copy(2 * t + 1).start()

    wait("wk0", "wv0")
    prep_kv(0)

    def first_terms(d, groups):
        cols = pl.ds(d * DHALF, DHALF)
        scale = 1.0
        for k in range(2):
            wait("ca%d%d" % (d, k))
            scale = scale + _dot(sc[:, k * DHALF:(k + 1) * DHALF], wmod_v[1, pl.ds(k * DHALF, DHALF), cols], NN)[0:8]
        mod_v[1, :, cols] = scale

        def block(half, dd, r0):
            cc = pl.ds(dd * DHALF, DHALF)
            return xn_v[pl.ds(half * TH + r0, 64), cc] * _tile8(mod_v[1, :, cc], 8)

        for group in groups:
            for r0 in range(0, TH, 64):
                b11, b12 = block(0, 0, r0), block(1, 0, r0)
                terms = _rhs_terms(b11, b12, block(0, 1, r0), block(1, 1, r0)) if d else {1: b11, 5: b11 + b12}
                for i in group:
                    put(("h", 0, i), terms[i], TH)

    def kv_product(t, c, i):
        return _dot(operands["w", c, i], operands["h", t, i], NT)

    first_terms(0, ((1,), (5,)))
    head_start = {i: kv_product(0, 0, i) for i in (1, 5)}
    first_terms(1, ((0,), (3, 2, 4, 6)))

    P = functools.partial

    def spread(slots, lo, hi, works):
        for n, work in enumerate(works):
            slots[lo + n * (hi - lo) // len(works)].append(work)

    steps = [("kv", t, c) for t in range(NTILE) for c in range(NCH)]
    steps += [("q", t, c) for t in range(NTILE) for c in range(NCH)]
    steps += [("o", t, r0) for t in range(NTILE) for r0 in range(0, TH, OROWS)]
    late = []
    for j in range(NCH):
        for m in range(8):
            late += [P(mod_piece, 2 + j, m * 128 + k0, 32) for k0 in range(0, 128, 32)]
            late.append(P(prep_wo, j, m * 16))
    prev, pending, guess = None, [], []
    for step, (kind, t, c) in enumerate(steps):
        slots = [[] for _ in range(7)]
        lower_done = None
        if prev is not None:
            pkind, pt, pc, pres = prev
            if pkind == "kv":
                pending += [P(kv_pair, pt, pc, pres, k) for k in (2, 3, 0, 1)]
                for slot in KV_SLOTS[KV_QUOTA[step] if kind == "kv" else len(pending)]:
                    slots[slot].append(pending.pop(0))
            elif pkind == "q":
                for slot, k in zip((0, 1, 3, 5), (2, 3, 0, 1)):
                    slots[slot].append(P(q_pair, pt, pc, pres, k))
            else:
                tok, order = pt * T + pc, _Order(probe)
                slots[0].append(P(residual, tok, pres[0]))
                spread(slots, 0, 4, [P(ln2_piece, tok + r0, order) for r0 in range(0, OROWS, LROWS)])
                if pc + OROWS == TH:
                    slots[4].append(P(start_out, pt))
        if kind == "kv":
            if t == 0 and c + 1 < NCH:
                slot, names = ((3, ("wk1", "wv1")), (3, ("wk2", "wv2", "wk3", "wv3")), (2, ("x1",)))[c]
                slots[slot] += [P(wait, *names), P(prep_kv, c + 1)]
            if (t, c) == (1, 0):
                slots[0] = [P(wait, "sa", "x2", "x3"), first_shift] + slots[0]
            if t == 1 and c < 2:
                for k, slot in enumerate(((1, 4), (0, 3))[c]):
                    first = (2 * c + k) * 512
                    slots[slot] += [P(kv_bias, r0) for r0 in range(first, first + 512, 64)]
            chunks = (2, 3) if t == 0 else (0, 1, 2, 3)
            if t + 1 < NTILE and c in chunks:
                n = TH // len(chunks)
                first = chunks.index(c) * n
                spread(slots, 3 if (t, c) == (0, 2) else 0, 6,
                       [P(ln1_piece, t + 1, r0) for r0 in range(first, first + n, LROWS)])
        n, span = step - LATE_FIRST, LATE_LAST - LATE_FIRST
        if n == 0:
            slots[0].insert(0, P(wait, "wq0", "wq1", "wq2", "wq3", "wr", "wo", "ga", "sb", "cb", "gb"))
        if 0 <= n < NCH:
            slots[5].append(P(prep_q, n))
        if 0 <= n < span:
            spread(slots, 1, 7, late[n * len(late) // span:(n + 1) * len(late) // span])
        if n == span:
            slots[0].insert(0, P(wait, "wg"))
            slots[6].append(finish_mod)
        if kind == "o":
            last = step == len(steps) - 1
            if last:
                slots[5].append(lambda: guess.extend(select()))
            tok, order = t * T + TH + c, None if last else _Order(probe)
            lower_done = P(residual, tok)
            spread(slots, 5, 6 if last else 7, [P(ln2_piece, tok + r0, order) for r0 in range(0, OROWS, LROWS)])

        def fill(k, m):
            stream.link = m
            for work in slots[k]:
                work()

        if kind == "kv":
            res = _block_product(lambda i: head_start.pop(i) if i in head_start else kv_product(t, c, i), fill)
            if c == NCH - 1:
                norm_order.link = None
        elif kind == "q":
            res = _block_product(lambda i: _dot(operands["q", c, i], operands["h", t, i], NT), fill)
        else:
            res = _block_product(lambda i: _dot(operands["o", t, i, c], operands["wo", i], NN), fill, lower_done)
        prev = (kind, t, c, res)

    gate_v[...] = _dot(stream.after(guess[3]).astype(BF), wg_v[...], NN)
    _, pt, pc, pres = prev
    tok = pt * T + pc
    residual(tok, pres[0])
    for r0 in range(0, OROWS, LROWS):
        ln2_piece(tok + r0, None)
    start_out(pt)

    idx_a, idx_b, gate_r, rows = select()
    rows = rows.astype(BF)
    sub = lax.broadcasted_iota(I32, (LROWS, D), 0)

    def slab(idx):
        start = pl.multiple_of((idx // LROWS) * LROWS, LROWS)
        x1 = x1_v[pl.ds(start, LROWS), :]
        return start, block_out(x1, *_center(x1))

    slabs = [slab(idx_a), slab(idx_b)]

    @pl.when((idx_a != guess[0]) | (idx_b != guess[1]))
    def _():
        gate_v[...] = _dot(rows, wg_v[...], NN)

    wait("wu", "wd")
    g = gate_v[...]
    u = _dot(rows, wu_v[...], NN)
    act = (g * jax.nn.sigmoid(g) * u).astype(BF)
    y = _dot(act, wd_v[:, pl.ds(0, D)], NN) * (gate_r * rows_of(5, LROWS))

    fixes = []
    for slot, (start, o) in enumerate(slabs):
        o = o + jnp.where(sub + start == idx_a, y[0:1], 0.0) + jnp.where(sub + start == idx_b, y[1:2], 0.0)
        slab_v[slot] = o.astype(BF)
        fixes.append(pltpu.make_async_copy(slab_v.at[slot], out_hbm.at[pl.ds(start, LROWS)], out_sems.at[slot]))
    for k in range(2 * NTILE):
        out_copy(k).wait()
    fixes[0].start()

    @pl.when(idx_a // LROWS != idx_b // LROWS)
    def _():
        fixes[1].start()
        fixes[1].wait()

    fixes[0].wait()


@jax.jit
def pallas_adaLN_cond__linear_kernel_hedgehog__moe_arch_mod__prompt_kernel(
    A_x: jax.Array,
    A_wqkv: jax.Array,
    A_w_phi: jax.Array,
    A_wo: jax.Array,
    B_x: jax.Array,
    B_w_r: jax.Array,
    B_w_gate: jax.Array,
    B_w_up: jax.Array,
    B_w_down: jax.Array,
    c: jax.Array,
    w_mod: jax.Array,
):
    del B_x
    any_spec = pl.BlockSpec(memory_space=pl.ANY)
    scratch = [
        pltpu.VMEM((S, D), BF),
        pltpu.VMEM((3 * NCH, D, 256), BF),
        pltpu.VMEM((H, DH, DH), BF),
        pltpu.VMEM((D, D), BF),
        pltpu.VMEM((8, 128), BF),
        pltpu.VMEM((D, F), BF),
        pltpu.VMEM((D, F), BF),
        pltpu.VMEM((F, D + LANE_PAD), BF),
        pltpu.VMEM((1, D), BF),
        pltpu.VMEM((6, D, D + LANE_PAD), BF),
        pltpu.VMEM((2 * NTILE, TH, D), BF),
        pltpu.VMEM((S, D), F32),
        pltpu.VMEM((T, D), F32),
        pltpu.VMEM((H // 2, 64, 128), F32),
        pltpu.VMEM((H // 2, 128, 128), F32),
        pltpu.VMEM((H // 2, 80, 128), BF),
        pltpu.VMEM((10, 8, D), F32),
        pltpu.VMEM((D, 128), F32),
        pltpu.VMEM((S + D, 128), F32),
        pltpu.VMEM((LROWS, F), F32),
        pltpu.VMEM((2, LROWS, D), BF),
        pltpu.SemaphoreType.DMA((40,)),
        pltpu.SemaphoreType.DMA((2 * NTILE,)),
    ]
    out = pl.pallas_call(
        _kernel,
        out_shape=jax.ShapeDtypeStruct((S, D), BF),
        in_specs=[any_spec] * 10,
        out_specs=any_spec,
        scratch_shapes=scratch,
        compiler_params=pltpu.CompilerParams(
            vmem_limit_bytes=120 * 2**20,
            flags={"XLA_TPU_EVENLY_DISTRIBUTE_CRITICAL_NODES": True},
        ),
        name="fused_block",
    )(A_x.reshape(S, D), A_wqkv, A_w_phi, A_wo, B_w_r.reshape(8, 128), B_w_gate, B_w_up, B_w_down, c, w_mod)
    return out.reshape(1, S, D)
```

```python
import functools

import jax
import jax.numpy as jnp
from jax import lax
from jax.experimental import pallas as pl
from jax.experimental.pallas import tpu as pltpu

S, D, H, DH, F = 2048, 1024, 32, 32, 3584
T = 512
TH = T // 2
DHALF = D // 2
NTILE = S // T
NCH = D // 256
OROWS = 64
LROWS = 16
LANE_PAD = 128
QMAIN = 56
LOG2E = 1.4426950408889634
NN = (((1,), (0,)), ((), ()))
NT = (((1,), (1,)), ((), ()))
BF = jnp.bfloat16
F32 = jnp.float32
I32 = jnp.int32

KV_QUOTA = (0, 0, 0, 0, 0, 3, 5, 7, 7, 7, 7, 7, 5, 4, 4, 4)
KV_SLOTS = {0: (), 3: (3, 4, 5), 4: (1, 2, 3, 4), 5: (1, 2, 3, 4, 5), 7: (0, 1, 2, 3, 4, 5, 6)}
LATE_FIRST, LATE_LAST = 12, 18


def _dot(a, b, dims):
    return lax.dot_general(a, b, dims, preferred_element_type=F32)


def _recip(x):
    return pltpu.reciprocal(x, approx=False, full_range=False)


def _tile8(r, n):
    return jnp.concatenate([r] * n, axis=0)


class _Order:
    def __init__(self, probe):
        self.probe = probe
        self.link = None

    def after(self, v):
        if self.link is None:
            return v
        rows, lanes = v.shape[0], min(v.shape[1], 128)
        probe, link = self.probe[:rows, :lanes], self.link[:rows, :lanes]
        return jnp.concatenate([jnp.where(probe != probe, link, v[:, l:l + lanes])
                                for l in range(0, v.shape[1], lanes)], axis=1)


def _center(x, order=None):
    s = jnp.sum(x, axis=-1, keepdims=True)
    if order is not None:
        s = order.after(s)
    xc = x - s * (1.0 / D)
    rs = lax.rsqrt(jnp.sum(xc * xc, axis=-1, keepdims=True) * (1.0 / D) + 1e-5)
    if order is not None:
        order.link = rs
    return xc, rs


def _pair_reduce(x, op):
    r = x[0:8]
    for i in range(1, 8):
        r = op(r, x[8 * i:8 * i + 8])
    r = op(r, pltpu.roll(r, 4, 0))
    return op(r, pltpu.roll(r, 2, 0))


def _pair_exps(p):
    mx = _tile8(_pair_reduce(p, jnp.maximum), 8)
    mn = _tile8(_pair_reduce(p, jnp.minimum), 8)
    return jnp.exp2(p - mx), jnp.exp2(mn - p)


def _hedgehog(p):
    ep, en = _pair_exps(p)
    rp = _tile8(_recip(_pair_reduce(ep, jnp.add)), 8)
    rn = _tile8(_recip(_pair_reduce(en, jnp.add)), 8)
    return jnp.concatenate([ep * rp, en * rn], axis=0)


def _hedgehog_scaled(p):
    ep, en = _pair_exps(p)
    sp = _pair_reduce(ep, jnp.add)
    ratio = _tile8(sp * _recip(_pair_reduce(en, jnp.add)), 8)
    return jnp.concatenate([ep, en * ratio], axis=0), sp


def _minus_last_feature(w):
    last = jnp.where(lax.broadcasted_iota(I32, (8, w.shape[1]), 0) >= 6, w[56:64], 0.0)
    last = last + pltpu.roll(last, 2, 0)
    last = last + pltpu.roll(last, 4, 0)
    return w - _tile8(last, 8)


def _shifted(x, shift):
    return pltpu.roll(x, shift % 8, 0) if shift % 8 else x


def _pack_tails(tails):
    sub = lax.broadcasted_iota(I32, tails[0].shape, 0)
    packed = []
    for r0 in range(0, 48, 8):
        p, q = r0 // 6, (r0 + 7) // 6
        packed.append(jnp.where(sub < 6 * q - r0, _shifted(tails[p], 6 * p), _shifted(tails[q], 6 * q)))
    return jnp.concatenate(packed, axis=0)


def _unpack_tail(packed, p):
    lo, hi = 6 * p // 8 * 8, (6 * p + 5) // 8 * 8
    sub = lax.broadcasted_iota(I32, (8, packed.shape[1]), 0)
    rows = _shifted(packed[lo:lo + 8], -6 * p)
    if hi != lo:
        rows = jnp.where(sub < hi - 6 * p, rows, _shifted(packed[hi:hi + 8], -6 * p))
    return jnp.where(sub < 6, rows, 0.0)


def _lhs_terms(a11, a12, a21, a22):
    return (a11 + a22, a21 + a22, a11, a22, a11 + a12, a21 - a11, a12 - a22)


def _rhs_terms(b11, b12, b21, b22):
    return (b11 + b22, b11, b12 - b22, b21 - b11, b22, b11 + b12, b21 + b22)


def _quadrants(top, bottom):
    return top[:, :DHALF], top[:, DHALF:], bottom[:, :DHALF], bottom[:, DHALF:]


def _block_product(product, fill, lower_done=None):
    m0 = product(0)
    fill(0, m0)
    m1 = product(1)
    fill(1, m1)
    c22 = m0 - m1
    m3 = product(3)
    fill(2, m3)
    c21 = m1 + m3
    c11 = m0 + m3
    m2 = product(2)
    fill(3, m2)
    c22 = c22 + m2
    m5 = product(5)
    fill(4, m5)
    lower = jnp.concatenate([c21, c22 + m5], axis=1)
    if lower_done is not None:
        lower_done(lower)
    m4 = product(4)
    fill(5, m4)
    c12 = m2 + m4
    c11 = c11 - m4
    m6 = product(6)
    fill(6, m6)
    return jnp.concatenate([c11 + m6, c12], axis=1), lower


def _merge_top2(a, b):
    def ahead(v, i, w, j):
        return (v > w) | ((v == w) & (i < j))

    first = ahead(a[0], a[2], b[0], b[2])
    lose_v, lose_i = jnp.where(first, b[0], a[0]), jnp.where(first, b[2], a[2])
    next_v, next_i = jnp.where(first, a[1], b[1]), jnp.where(first, a[3], b[3])
    second = ahead(lose_v, lose_i, next_v, next_i)
    return (jnp.where(first, a[0], b[0]), jnp.where(second, lose_v, next_v),
            jnp.where(first, a[2], b[2]), jnp.where(second, lose_i, next_i))


def _kernel(x_hbm, wqkv_hbm, wphi_hbm, wo_hbm, wr_hbm, wg_hbm, wu_hbm, wd_hbm, c_hbm, wmod_hbm,
            out_hbm,
            x_v, wqkv_v, wphi_v, wo_v, wr_v, wg_v, wu_v, wd_v, c_v, wmod_v,
            out_v, x1_v, xn_v, kv_acc, z_acc, kv_v, mod_v, sc_v, bias_v, gate_v, slab_v,
            in_sems, out_sems):
    def x_copy(t):
        return ("x%d" % t, x_hbm.at[pl.ds(t * T, T)], x_v.at[pl.ds(t * T, T)])

    def w_copy(name, j, c):
        return ("%s%d" % (name, c), wqkv_hbm.at[:, pl.ds((j * NCH + c) * 256, 256)], wqkv_v.at[j * NCH + c])

    def mod_copy(name, j):
        return (name, wmod_hbm.at[:, pl.ds(j * D, D)], wmod_v.at[j, :, pl.ds(0, D)])

    def scale_copy(d, k):
        rows = pl.ds(k * DHALF, DHALF)
        return ("ca%d%d" % (d, k), wmod_hbm.at[rows, pl.ds(D + d * DHALF, DHALF)],
                wmod_v.at[1, rows, pl.ds(d * DHALF, DHALF)])

    queue = [("c", c_hbm, c_v), x_copy(0), ("wphi", wphi_hbm, wphi_v), w_copy("wk", 1, 0), w_copy("wv", 2, 0)]
    queue += [scale_copy(d, k) for d in range(2) for k in range(2)]
    for c in range(1, NCH):
        queue += [w_copy("wk", 1, c), w_copy("wv", 2, c)]
    queue += [x_copy(1), mod_copy("sa", 0), x_copy(2), x_copy(3)]
    queue += [w_copy("wq", 0, c) for c in range(NCH)]
    queue += [("wr", wr_hbm, wr_v), ("wo", wo_hbm, wo_v),
              mod_copy("ga", 2), mod_copy("sb", 3), mod_copy("cb", 4), mod_copy("gb", 5),
              ("wg", wg_hbm, wg_v), ("wu", wu_hbm, wu_v), ("wd", wd_hbm, wd_v.at[:, pl.ds(0, D)])]
    copies = {}
    for i, (name, src, dst) in enumerate(queue):
        copies[name] = pltpu.make_async_copy(src, dst, in_sems.at[i])
        copies[name].start()

    def wait(*names):
        for name in names:
            copies[name].wait()

    wait("c", "x0")
    cf = c_v[...].astype(F32)
    probe = jnp.broadcast_to(cf[:, 0:128], (64, 128))
    norm_order, norm_order2, bias_order, late_order, stream = [_Order(probe) for _ in range(5)]
    sc = jnp.broadcast_to(cf * jax.nn.sigmoid(cf), (16, D)).astype(BF)

    def normalized(tok, n, order=None):
        xc, rs = _center(x_v[pl.ds(tok, n), :].astype(F32), order)
        return xc * rs

    for r0 in range(0, T, 32):
        xn_v[pl.ds(r0, 32), :] = normalized(r0, 32)

    wait("wphi")
    row = lax.broadcasted_iota(I32, (128, DH), 0)
    lane = lax.broadcasted_iota(I32, (128, DH), 1)
    expand = jnp.where(((row % 64) // 2) == lane, 1.0, 0.0).astype(BF)
    phi_t = _dot(expand, wphi_v[...].reshape(H * DH, DH), NT)
    row = lax.broadcasted_iota(I32, (128, D), 0)
    lane = lax.broadcasted_iota(I32, (128, D), 1)
    phi_t = jnp.where(2 * (row // 64) + (row % 2) == (lane % 128) // DH, phi_t, 0.0).astype(BF)

    for k0 in range(0, D, 128):
        sc_v[pl.ds(k0, 128), :] = jnp.broadcast_to(sc[0:1, k0:k0 + 128].astype(F32), (128, 128)).T

    partial_mod = {}

    def mod_piece(j, k0, nk):
        acc = partial_mod.pop(j, None)
        for k in range(k0, k0 + nk, 8):
            s_col = sc_v[pl.ds(k, 8), :]
            if k == k0:
                s_col = late_order.after(s_col)
            term = wmod_v[j, pl.ds(k, 8), pl.ds(0, D)].astype(F32) * jnp.concatenate([s_col] * (D // 128), axis=1)
            acc = term if acc is None else acc + term
        link = jnp.broadcast_to(jnp.max(acc[:, 0:128], axis=-1, keepdims=True), (8, 128))
        late_order.link = jnp.concatenate([link, link], axis=0)
        if k0 + nk < D:
            partial_mod[j] = acc
        else:
            mod_v[j] = jnp.broadcast_to(jnp.sum(acc, axis=0, keepdims=True), (8, D))

    def first_shift():
        mod_v[0] = _dot(sc, wmod_v[0, :, pl.ds(0, D)], NN)[0:8]

    def finish_mod():
        wr = wr_v[...].astype(F32)
        wr_row = jnp.concatenate([jnp.broadcast_to(wr[j:j + 1, :], (8, 128)) for j in range(8)], axis=1)
        shift, scale, gate = mod_v[3], 1.0 + mod_v[4], mod_v[5]
        mod_v[4] = scale
        mod_v[6] = gate * scale
        mod_v[7] = gate * shift
        mod_v[8] = wr_row * scale
        mod_v[9] = jnp.broadcast_to(jnp.sum(wr_row * shift, axis=-1, keepdims=True), (8, D))

    def rows_of(j, n):
        return _tile8(mod_v[j], n // 8)

    pieces, operands = {}, {}

    def put(key, value, size, axis=0):
        parts = pieces.setdefault(key, [])
        parts.append(value)
        if sum(part.shape[axis] for part in parts) == size:
            operands[key] = jnp.concatenate(pieces.pop(key), axis=axis).astype(BF)

    def ln1_piece(t, r0):
        a = normalized(t * T + r0, LROWS, norm_order)
        b = normalized(t * T + TH + r0, LROWS, norm_order2 if t == 1 else norm_order)
        h1, h2 = a * rows_of(1, LROWS), b * rows_of(1, LROWS)
        for i, term in enumerate(_rhs_terms(h1[:, :DHALF], h2[:, :DHALF], h1[:, DHALF:], h2[:, DHALF:])):
            put(("h", t, i), term, TH)

    def shift_bias(dst, w, order):
        b = jnp.sum(w * _tile8(order.after(mod_v[0]), w.shape[0] // 8), axis=-1, keepdims=True)
        order.link = jnp.broadcast_to(b, (w.shape[0], 128))
        bias_v[pl.ds(dst, w.shape[0]), :] = order.link

    def kv_bias(r0):
        shift_bias(r0, x1_v[pl.ds(r0, 64), :], bias_order)

    def folded(j, c):
        halves = []
        for g in range(2):
            w = wqkv_v[j * NCH + c, :, g * 128:(g + 1) * 128]
            group = 2 * c + g
            halves.append(_dot(phi_t[:, group * 128:(group + 1) * 128], w, NT) * LOG2E)
        return halves

    def put_kv_weights(c, r0, halves):
        for i, term in enumerate(_lhs_terms(*_quadrants(*halves))):
            put(("w", c, i), term, 256)
        for g in range(2):
            x1_v[pl.ds(c * 512 + g * 256 + r0, 128), :] = halves[g]

    def prep_kv(c):
        keys = folded(1, c)
        put_kv_weights(c, 128, [wqkv_v[2 * NCH + c, :, g * 128:(g + 1) * 128].astype(F32).T for g in range(2)])
        put_kv_weights(c, 0, keys)

    q_tails = []

    def prep_q(c):
        halves = folded(0, c)
        size = 2 * QMAIN + 48 * (c == 0)
        for q in range(2):
            top, bottom = [_minus_last_feature(half[q * 64:(q + 1) * 64]) for half in halves]
            for r0 in range(0, 64, 16):
                a, b = bias_order.after(top[r0:r0 + 16]), bottom[r0:r0 + 16]
                n = min(16, QMAIN - r0)
                for i, term in enumerate(_lhs_terms(*_quadrants(a[:n], b[:n]))):
                    put(("q", c, i), term, size)
                shift_bias(S + c * 256 + q * 64 + r0, a, _Order(probe))
                shift_bias(S + c * 256 + 128 + q * 64 + r0, b, bias_order)
            q_tails.append((top[QMAIN:], bottom[QMAIN:]))
        if c == NCH - 1:
            for i, term in enumerate(_lhs_terms(*_quadrants(*[_pack_tails(tails) for tails in zip(*q_tails)]))):
                put(("q", 0, i), term, 2 * QMAIN + 48)

    def prep_wo(c, r0):
        top = late_order.after(wo_v[pl.ds(c * 256 + r0, 16), :].astype(F32))
        bottom = wo_v[pl.ds(c * 256 + 128 + r0, 16), :].astype(F32)
        terms = _rhs_terms(*_quadrants(top, bottom))
        for i, term in enumerate(terms):
            put(("wo", i), term, DHALF)
        late_order.link = jnp.broadcast_to(jnp.max(terms[0][:, 0:128], axis=-1, keepdims=True), (16, 128))

    def bias_rows(r0):
        return jnp.concatenate([bias_v[pl.ds(r0, 64), :]] * (T // 128), axis=1)

    def kv_pair(t, c, res, k):
        g, q = divmod(k, 2)
        pair = 4 * c + k
        r0 = c * 512 + g * 256 + q * 64
        phi = _hedgehog(res[g][128 + q * 64:128 + (q + 1) * 64] + bias_rows(r0))
        vt = res[g][q * 64:(q + 1) * 64]
        vt = jnp.concatenate([stream.after(vt[0:8]), vt[8:]], axis=0).astype(BF)
        zs = phi[:, 0:128]
        for l in range(128, T, 128):
            zs = zs + phi[:, l:l + 128]
        kv = _dot(vt, phi.astype(BF), NT)
        if t > 0:
            zs = zs + z_acc[pair]
            kv = kv + kv_acc[pair]
        if t < NTILE - 1:
            z_acc[pair] = zs
            kv_acc[pair] = kv
        else:
            z = jnp.broadcast_to(jnp.sum(zs.T, axis=0, keepdims=True), (16, 128))
            kv = kv + bias_v[pl.ds(r0 + 128, 64), :] * _tile8(z[0:8], 8)
            row = lax.broadcasted_iota(I32, (80, 128), 0)
            lane = lax.broadcasted_iota(I32, (80, 128), 1)
            head = jnp.where(row < 64, row // DH, (row - 64) // 8)
            kv_v[pair] = jnp.where(head == lane % 2, jnp.concatenate([kv, z], axis=0), 0.0).astype(BF)

    held = {}

    def q_pair(t, c, res, k):
        g, q = divmod(k, 2)
        pair = 4 * c + k
        even = (lax.broadcasted_iota(I32, (8, T), 0) % 2) == 0
        if c == 0:
            held["tail", g] = res[g][2 * QMAIN:]
        logits = jnp.concatenate([res[g][q * QMAIN:(q + 1) * QMAIN], _unpack_tail(held["tail", g], 2 * c + q)], axis=0)
        phi, scale = _hedgehog_scaled(logits + bias_rows(S + pair * 64))
        nd = _dot(kv_v[pair], phi.astype(BF), NN)
        swapped = pltpu.roll(scale, 1, 0)
        inv_a = _recip(nd[64:72] + 1e-6 * jnp.where(even, scale, swapped))
        inv_b = _recip(nd[72:80] + 1e-6 * jnp.where(even, swapped, scale))
        held[k] = nd[0:64] * jnp.concatenate([inv_a] * 4 + [inv_b] * 4, axis=0)
        if k == 3:
            held["lower"] = jnp.concatenate([held.pop(2), held.pop(3)], axis=0).T
        if k == 1:
            o1, o2 = jnp.concatenate([held.pop(0), held.pop(1)], axis=0).T, held.pop("lower")
            for i, term in enumerate(_lhs_terms(o1[:TH], o2[:TH], o1[TH:], o2[TH:])):
                for r0 in range(0, TH, OROWS):
                    put(("o", t, i, r0), term[r0:r0 + OROWS], DHALF, 1)

    def residual(tok, attn):
        rows = pl.ds(tok, OROWS)
        x1_v[rows, :] = x_v[rows, :].astype(F32) + rows_of(2, OROWS) * attn

    def block_out(x1, xc, rs):
        return xc * (rs * rows_of(6, LROWS)) + (x1 + rows_of(7, LROWS))

    def router(xc, rs):
        return jnp.sum(xc * rows_of(8, LROWS), axis=-1, keepdims=True) * rs + rows_of(9, LROWS)[:, 0:1]

    found = []

    def ln2_piece(tok, order):
        x1 = x1_v[pl.ds(tok, LROWS), :]
        xc, rs = _center(x1, order)
        out_v[tok // TH, pl.ds(tok % TH, LROWS), :] = block_out(x1, xc, rs).astype(BF)
        r = router(xc, rs)
        sub = lax.broadcasted_iota(I32, (8, 128), 0).astype(F32)
        ra, rb = jnp.broadcast_to(r[0:8], (8, 128)), jnp.broadcast_to(r[8:16], (8, 128))
        ia, ib = sub + float(tok), sub + float(tok + 8)
        first = ra >= rb
        found.append((jnp.where(first, ra, rb), jnp.where(first, rb, ra),
                      jnp.where(first, ia, ib), jnp.where(first, ib, ia)))
        if order is not None and len(found) == 2:
            found[:] = [_merge_top2(*found)]

    def select():
        while len(found) > 1:
            found[:] = [_merge_top2(*found[k:k + 2]) if k + 1 < len(found) else found[k]
                        for k in range(0, len(found), 2)]
        m1, m2, i1, i2 = found[0]
        big = float(2 * S)
        best = jnp.max(m1, axis=0, keepdims=True)
        ia = jnp.min(jnp.where(m1 == best, i1, big), axis=0, keepdims=True)
        taken = i1 == ia
        cm = jnp.where(taken, m2, m1)
        ci = jnp.where(taken, i2, i1)
        second = jnp.max(cm, axis=0, keepdims=True)
        ib = jnp.min(jnp.where(cm == second, ci, big), axis=0, keepdims=True)
        idx_a = jnp.clip(ia.astype(I32)[0, 0], 0, S - 1)
        idx_b = jnp.clip(ib.astype(I32)[0, 0], 0, S - 1)
        xa = jnp.broadcast_to(x1_v[pl.ds(idx_a, 1), :], (LROWS, D))
        xb = jnp.broadcast_to(x1_v[pl.ds(idx_b, 1), :], (LROWS, D))
        xc, rs = _center(jnp.where(lax.broadcasted_iota(I32, (LROWS, D), 0) == 0, xa, xb))
        rows = xc * rs * rows_of(4, LROWS) + rows_of(3, LROWS)
        return idx_a, idx_b, jax.nn.sigmoid(router(xc, rs)), rows

    def out_copy(k):
        return pltpu.make_async_copy(out_v.at[k], out_hbm.at[pl.ds(k * TH, TH)], out_sems.at[k])

    def start_out(t):
        out_copy(2 * t).start()
        out_copy(2 * t + 1).start()

    wait("wk0", "wv0")
    prep_kv(0)

    def first_terms(d, groups):
        cols = pl.ds(d * DHALF, DHALF)
        scale = 1.0
        for k in range(2):
            wait("ca%d%d" % (d, k))
            scale = scale + _dot(sc[:, k * DHALF:(k + 1) * DHALF], wmod_v[1, pl.ds(k * DHALF, DHALF), cols], NN)[0:8]
        mod_v[1, :, cols] = scale

        def block(half, dd, r0):
            cc = pl.ds(dd * DHALF, DHALF)
            return xn_v[pl.ds(half * TH + r0, 64), cc] * _tile8(mod_v[1, :, cc], 8)

        for group in groups:
            for r0 in range(0, TH, 64):
                b11, b12 = block(0, 0, r0), block(1, 0, r0)
                terms = _rhs_terms(b11, b12, block(0, 1, r0), block(1, 1, r0)) if d else {1: b11, 5: b11 + b12}
                for i in group:
                    put(("h", 0, i), terms[i], TH)

    def kv_product(t, c, i):
        return _dot(operands["w", c, i], operands["h", t, i], NT)

    first_terms(0, ((1,), (5,)))
    head_start = {i: kv_product(0, 0, i) for i in (1, 5)}
    first_terms(1, ((0,), (3, 2, 4, 6)))

    P = functools.partial

    def spread(slots, lo, hi, works):
        for n, work in enumerate(works):
            slots[lo + n * (hi - lo) // len(works)].append(work)

    steps = [("kv", t, c) for t in range(NTILE) for c in range(NCH)]
    steps += [("q", t, c) for t in range(NTILE) for c in range(NCH)]
    steps += [("o", t, r0) for t in range(NTILE) for r0 in range(0, TH, OROWS)]
    late = []
    for j in range(NCH):
        for m in range(8):
            late += [P(mod_piece, 2 + j, m * 128 + k0, 32) for k0 in range(0, 128, 32)]
            late.append(P(prep_wo, j, m * 16))
    prev, pending, guess = None, [], []
    for step, (kind, t, c) in enumerate(steps):
        slots = [[] for _ in range(7)]
        lower_done = None
        if prev is not None:
            pkind, pt, pc, pres = prev
            if pkind == "kv":
                pending += [P(kv_pair, pt, pc, pres, k) for k in (2, 3, 0, 1)]
                for slot in KV_SLOTS[KV_QUOTA[step] if kind == "kv" else len(pending)]:
                    slots[slot].append(pending.pop(0))
            elif pkind == "q":
                for slot, k in zip((1, 2, 4, 5), (2, 3, 0, 1)):
                    slots[slot].append(P(q_pair, pt, pc, pres, k))
            else:
                tok, order = pt * T + pc, _Order(probe)
                slots[0].append(P(residual, tok, pres[0]))
                spread(slots, 0, 4, [P(ln2_piece, tok + r0, order) for r0 in range(0, OROWS, LROWS)])
                if pc + OROWS == TH:
                    slots[4].append(P(start_out, pt))
        if kind == "kv":
            if t == 0 and c + 1 < NCH:
                slot, names = ((4, ("wk1", "wv1")), (4, ("wk2", "wv2", "wk3", "wv3")), (3, ("x1",)))[c]
                slots[slot] += [P(wait, *names), P(prep_kv, c + 1)]
            if (t, c) == (1, 0):
                slots[0] = [P(wait, "sa", "x2", "x3"), first_shift] + slots[0]
            if t == 1 and c < 2:
                for k, slot in enumerate(((1, 4), (0, 3))[c]):
                    first = (2 * c + k) * 512
                    slots[slot] += [P(kv_bias, r0) for r0 in range(first, first + 512, 64)]
            chunks = (2, 3) if t == 0 else (0, 1, 2, 3)
            if t + 1 < NTILE and c in chunks:
                n = TH // len(chunks)
                first = chunks.index(c) * n
                spread(slots, 4 if (t, c) == (0, 2) else 0, 6,
                       [P(ln1_piece, t + 1, r0) for r0 in range(first, first + n, LROWS)])
        n, span = step - LATE_FIRST, LATE_LAST - LATE_FIRST
        if n == 0:
            slots[0].insert(0, P(wait, "wq0", "wq1", "wq2", "wq3", "wr", "wo", "ga", "sb", "cb", "gb"))
        if 0 <= n < NCH:
            slots[5].append(P(prep_q, n))
        if 0 <= n < span:
            spread(slots, 1, 7, late[n * len(late) // span:(n + 1) * len(late) // span])
        if n == span:
            slots[0].insert(0, P(wait, "wg"))
            slots[6].append(finish_mod)
        if kind == "o":
            last = step == len(steps) - 1
            if last:
                slots[5].append(lambda: guess.extend(select()))
            tok, order = t * T + TH + c, None if last else _Order(probe)
            lower_done = P(residual, tok)
            spread(slots, 5, 6 if last else 7, [P(ln2_piece, tok + r0, order) for r0 in range(0, OROWS, LROWS)])

        def fill(k, m):
            stream.link = m
            for work in slots[k]:
                work()

        if kind == "kv":
            res = _block_product(lambda i: head_start.pop(i) if i in head_start else kv_product(t, c, i), fill)
            if c == NCH - 1:
                norm_order.link = None
        elif kind == "q":
            res = _block_product(lambda i: _dot(operands["q", c, i], operands["h", t, i], NT), fill)
        else:
            res = _block_product(lambda i: _dot(operands["o", t, i, c], operands["wo", i], NN), fill, lower_done)
        prev = (kind, t, c, res)

    gate_v[...] = _dot(stream.after(guess[3]).astype(BF), wg_v[...], NN)
    _, pt, pc, pres = prev
    tok = pt * T + pc
    residual(tok, pres[0])
    for r0 in range(0, OROWS, LROWS):
        ln2_piece(tok + r0, None)
    start_out(pt)

    idx_a, idx_b, gate_r, rows = select()
    rows = rows.astype(BF)
    sub = lax.broadcasted_iota(I32, (LROWS, D), 0)

    def slab(idx):
        start = pl.multiple_of((idx // LROWS) * LROWS, LROWS)
        x1 = x1_v[pl.ds(start, LROWS), :]
        return start, block_out(x1, *_center(x1))

    slabs = [slab(idx_a), slab(idx_b)]

    @pl.when((idx_a != guess[0]) | (idx_b != guess[1]))
    def _():
        gate_v[...] = _dot(rows, wg_v[...], NN)

    wait("wu", "wd")
    g = gate_v[...]
    u = _dot(rows, wu_v[...], NN)
    act = (g * jax.nn.sigmoid(g) * u).astype(BF)
    y = _dot(act, wd_v[:, pl.ds(0, D)], NN) * (gate_r * rows_of(5, LROWS))

    fixes = []
    for slot, (start, o) in enumerate(slabs):
        o = o + jnp.where(sub + start == idx_a, y[0:1], 0.0) + jnp.where(sub + start == idx_b, y[1:2], 0.0)
        slab_v[slot] = o.astype(BF)
        fixes.append(pltpu.make_async_copy(slab_v.at[slot], out_hbm.at[pl.ds(start, LROWS)], out_sems.at[slot]))
    for k in range(2 * NTILE):
        out_copy(k).wait()
    fixes[0].start()

    @pl.when(idx_a // LROWS != idx_b // LROWS)
    def _():
        fixes[1].start()
        fixes[1].wait()

    fixes[0].wait()


@jax.jit
def pallas_adaLN_cond__linear_kernel_hedgehog__moe_arch_mod__prompt_kernel(
    A_x: jax.Array,
    A_wqkv: jax.Array,
    A_w_phi: jax.Array,
    A_wo: jax.Array,
    B_x: jax.Array,
    B_w_r: jax.Array,
    B_w_gate: jax.Array,
    B_w_up: jax.Array,
    B_w_down: jax.Array,
    c: jax.Array,
    w_mod: jax.Array,
):
    del B_x
    any_spec = pl.BlockSpec(memory_space=pl.ANY)
    scratch = [
        pltpu.VMEM((S, D), BF),
        pltpu.VMEM((3 * NCH, D, 256), BF),
        pltpu.VMEM((H, DH, DH), BF),
        pltpu.VMEM((D, D), BF),
        pltpu.VMEM((8, 128), BF),
        pltpu.VMEM((D, F), BF),
        pltpu.VMEM((D, F), BF),
        pltpu.VMEM((F, D + LANE_PAD), BF),
        pltpu.VMEM((1, D), BF),
        pltpu.VMEM((6, D, D + LANE_PAD), BF),
        pltpu.VMEM((2 * NTILE, TH, D), BF),
        pltpu.VMEM((S, D), F32),
        pltpu.VMEM((T, D), F32),
        pltpu.VMEM((H // 2, 64, 128), F32),
        pltpu.VMEM((H // 2, 128, 128), F32),
        pltpu.VMEM((H // 2, 80, 128), BF),
        pltpu.VMEM((10, 8, D), F32),
        pltpu.VMEM((D, 128), F32),
        pltpu.VMEM((S + D, 128), F32),
        pltpu.VMEM((LROWS, F), F32),
        pltpu.VMEM((2, LROWS, D), BF),
        pltpu.SemaphoreType.DMA((40,)),
        pltpu.SemaphoreType.DMA((2 * NTILE,)),
    ]
    out = pl.pallas_call(
        _kernel,
        out_shape=jax.ShapeDtypeStruct((S, D), BF),
        in_specs=[any_spec] * 10,
        out_specs=any_spec,
        scratch_shapes=scratch,
        compiler_params=pltpu.CompilerParams(
            vmem_limit_bytes=120 * 2**20,
            flags={"XLA_TPU_EVENLY_DISTRIBUTE_CRITICAL_NODES": True},
        ),
        name="fused_block",
    )(A_x.reshape(S, D), A_wqkv, A_w_phi, A_wo, B_w_r.reshape(8, 128), B_w_gate, B_w_up, B_w_down, c, w_mod)
    return out.reshape(1, S, D)
```
